```python
import jax
import jax.numpy as jnp

def _softmax(x, axis=-1):
    return jax.nn.softmax(x, axis=axis)
def _gelu(x):
    return jax.nn.gelu(x, approximate=True)
def _silu(x):
    return jax.nn.silu(x)
def _sigmoid(x):
    return jax.nn.sigmoid(x)
def _layernorm(x, axis=-1, eps=1e-5):
    m = jnp.mean(x, axis=axis, keepdims=True)
    v = jnp.var(x, axis=axis, keepdims=True)
    return (x - m) / jnp.sqrt(v + eps)
def _scatter_add(tgt, idx, src, axis=0):
    return tgt.at[idx].add(src)
def _segment_sum(src, seg, n):
    return jax.ops.segment_sum(src, seg, n)
class _Rng:
    def __init__(self, key):
        self._k = key
    def _next(self):
        self._k, sub = jax.random.split(self._k)
        return sub
    def normal(self, shape):
        return jax.random.normal(self._next(), shape, dtype=jnp.bfloat16)
    def randint(self, lo, hi, shape):
        return jax.random.randint(self._next(), shape, lo, hi, dtype=jnp.int32)
    def uniform(self, shape, lo=0.0, hi=1.0):
        return jax.random.uniform(self._next(), shape, jnp.bfloat16, lo, hi)
    def permutation(self, n):
        return jax.random.permutation(self._next(), n)


kernel_name = 'standalone__modern_conv_block_slak__vision'

def setup_inputs():
    _rng = _Rng(jax.random.key(int.from_bytes(__import__("os").urandom(4), "little")))
    _w = (lambda a: (lambda t: t.astype(jnp.bfloat16) if jnp.issubdtype(t.dtype, jnp.floating) else t)(jnp.asarray(a)))
    H = W = 384
    C = 384
    K = 1
    return {
        "x": _w((lambda *s: _rng.normal(s) * 0.05)(1, H, W, C)),
        "dw": _w((lambda *s: _rng.normal(s) * 0.05)(K, K, C)),
        "w1": _w((lambda *s: _rng.normal(s) * 0.05)(C, 4 * C)),
        "w2": _w((lambda *s: _rng.normal(s) * 0.05)(4 * C, C)),
        "grn_g": _w((lambda *s: _rng.normal(s) * 0.05)(4 * C)),
        "grn_b": _w((lambda *s: _rng.normal(s) * 0.05)(4 * C)),
    }

def reference(x, dw, w1, w2, grn_g, grn_b):
    B, H, W, C = x.shape
    K = dw.shape[0]
    pad = K // 2
    xp = jnp.pad(x, ((0,0),(pad,pad),(pad,pad),(0,0)))
    out = jnp.zeros_like(x)
    for i in range(K):
        for j in range(K):
            out = out + xp[:, i:i+H, j:j+W, :] * dw[i, j][None, None, None, :]
    h = _layernorm(out, axis=-1)
    h = _gelu(h @ w1)
    gx = jnp.sqrt((h * h).sum(axis=(1, 2), keepdims=True) + 1e-6)
    nx = gx / (gx.mean(axis=-1, keepdims=True) + 1e-6)
    h = grn_g[None, None, None, :] * (h * nx) + grn_b[None, None, None, :] + h
    return x + h @ w2
```

```python
import functools

import jax
import jax.numpy as jnp
import jax.experimental.pallas as pl
import jax.experimental.pallas.tpu as pltpu

F32 = jnp.float32
BF16 = jnp.bfloat16

_GELU_C0 = 0.7978845608028654
_GELU_C1 = 0.7978845608028654 * 0.044715


def _gelu_tanh(a):
    inner = a * (_GELU_C0 + _GELU_C1 * (a * a))
    ha = 0.5 * a
    return ha + ha * jnp.tanh(inner)


def _kernel(x_ref, dw_ref, w1_ref, w2_ref, g_ref, b_ref,
            o_ref, h_hbm,
            hbuf, ssq_ref, w2s_ref, bias_ref, sems,
            *, tm, nt, c, c4, cn, nbuf):
    p = pl.program_id(0)
    i = pl.program_id(1)

    def h_out_copy(slot, t):
        return pltpu.make_async_copy(
            hbuf.at[slot], h_hbm.at[pl.ds(t * tm, tm), :], sems.at[slot])

    def h_in_copy(slot, t):
        return pltpu.make_async_copy(
            h_hbm.at[pl.ds(t * tm, tm), :], hbuf.at[slot], sems.at[slot])

    @pl.when(p == 0)
    def _phase0():
        slot = i % nbuf

        @pl.when(i == 0)
        def _():
            ssq_ref[...] = jnp.zeros_like(ssq_ref)

        @pl.when(i >= nbuf)
        def _():
            h_out_copy(slot, i - nbuf).wait()

        y = x_ref[...].astype(F32) * dw_ref[...].astype(F32)
        m = jnp.mean(y, axis=-1, keepdims=True)
        yc = y - m
        v = jnp.mean(yc * yc, axis=-1, keepdims=True)
        xn = (yc * jax.lax.rsqrt(v + 1e-5)).astype(BF16)
        for j in range(c4 // cn):
            cs = slice(j * cn, (j + 1) * cn)
            a = jnp.dot(xn, w1_ref[:, cs], preferred_element_type=F32)
            gl = _gelu_tanh(a)
            sq = gl * gl
            ssq_ref[:, cs] += jnp.sum(sq.reshape(tm // 8, 8, cn), axis=0)
            hbuf[slot, :, cs] = gl.astype(BF16)
        h_out_copy(slot, i).start()

        @pl.when(i == nt - 1)
        def _():
            for k in range(nbuf):
                t = nt - nbuf + k
                h_out_copy(t % nbuf, t).wait()
            for k in range(nbuf - 1):
                h_in_copy(k, k).start()

    @pl.when(p == 1)
    def _phase1():
        slot = i % nbuf

        @pl.when(i == 0)
        def _():
            ssq = jnp.sum(ssq_ref[...], axis=0, keepdims=True)
            gx = jnp.sqrt(ssq + 1e-6)
            nx = gx / (jnp.mean(gx, axis=-1, keepdims=True) + 1e-6)
            s = 1.0 + g_ref[...].astype(F32) * nx
            s_t = jnp.transpose(jnp.broadcast_to(s, (128, c4)))
            for k in range(c // 128):
                ls = slice(k * 128, (k + 1) * 128)
                w2s_ref[:, ls] = (w2_ref[:, ls].astype(F32) * s_t).astype(BF16)
            b8 = jnp.broadcast_to(b_ref[...], (16, c4))
            bias_ref[...] = jnp.dot(b8, w2_ref[...], preferred_element_type=F32)[:8]

        @pl.when(i + nbuf - 1 < nt)
        def _():
            t = i + nbuf - 1
            h_in_copy(t % nbuf, t).start()

        h_in_copy(slot, i).wait()
        acc = jnp.dot(hbuf[slot], w2s_ref[...], preferred_element_type=F32)
        o_ref[...] = (x_ref[...].astype(F32) + acc + bias_ref[0:1, :]).astype(BF16)


def _build(n, c, c4, tm=1024, cn=256, nbuf=2, vmem_mb=100):
    nt = n // tm
    kern = functools.partial(_kernel, tm=tm, nt=nt, c=c, c4=c4, cn=cn, nbuf=nbuf)
    const = lambda p, i: (0, 0)
    return pl.pallas_call(
        kern,
        grid=(2, nt),
        in_specs=[
            pl.BlockSpec((tm, c), lambda p, i: (i, 0)),
            pl.BlockSpec((1, c), const),
            pl.BlockSpec((c, c4), const),
            pl.BlockSpec((c4, c), const),
            pl.BlockSpec((1, c4), const),
            pl.BlockSpec((1, c4), const),
        ],
        out_specs=[
            pl.BlockSpec((tm, c), lambda p, i: (i * p, 0)),
            pl.BlockSpec(memory_space=pl.ANY),
        ],
        out_shape=[
            jax.ShapeDtypeStruct((n, c), BF16),
            jax.ShapeDtypeStruct((n, c4), BF16),
        ],
        scratch_shapes=[
            pltpu.VMEM((nbuf, tm, c4), BF16),
            pltpu.VMEM((8, c4), F32),
            pltpu.VMEM((c4, c), BF16),
            pltpu.VMEM((8, c), F32),
            pltpu.SemaphoreType.DMA((nbuf,)),
        ],
        compiler_params=pltpu.CompilerParams(
            dimension_semantics=("arbitrary", "arbitrary"),
            vmem_limit_bytes=vmem_mb * 1024 * 1024,
        ),
    )


def _run(x, dw, w1, w2, grn_g, grn_b, **kw):
    b, hh, ww, c = x.shape
    c4 = w1.shape[1]
    n = b * hh * ww
    assert b == 1 and dw.shape[0] == 1 and dw.shape[1] == 1
    out, _ = _build(n, c, c4, **kw)(
        x.reshape(n, c), dw.reshape(1, c), w1, w2,
        grn_g.reshape(1, c4), grn_b.reshape(1, c4))
    return out.reshape(x.shape)


@jax.jit
def pallas_standalone__modern_conv_block_slak__vision_kernel(
    x: jax.Array,
    dw: jax.Array,
    w1: jax.Array,
    w2: jax.Array,
    grn_g: jax.Array,
    grn_b: jax.Array,
):
    return _run(x, dw, w1, w2, grn_g, grn_b)
```

```python
import functools

import jax
import jax.numpy as jnp
import jax.experimental.pallas as pl
import jax.experimental.pallas.tpu as pltpu

F32 = jnp.float32
BF16 = jnp.bfloat16
LANES = 128

_GELU_C0 = 0.7978845608028654
_GELU_C1 = 0.7978845608028654 * 0.044715


def _col(row, n):
    return jnp.transpose(jnp.broadcast_to(row, (LANES, n)))


def _kernel(x_ref, dw_ref, w1_ref, w2_ref, g_ref, b_ref,
            o_ref, h_hbm,
            hs, ssq_ref, w1s_ref, w2s_ref, bias_ref, sems,
            *, tm, nt, c, c4, cn, ring, npin, phases, rbs, rbs1):
    p = pl.program_id(0)
    i = pl.program_id(1)
    if phases == (1,):
        p = p + 1
    nj = c4 // LANES
    nk = c // LANES
    nspill = nt - npin - ring

    def tile_info(t):
        lo = (t * npin) // nt
        hi = ((t + 1) * npin) // nt
        pinned = hi > lo
        u = t - lo
        slot = jnp.where(pinned, ring + lo, u % ring)
        return pinned, u, slot

    def h_out_copy(slot, u):
        return pltpu.make_async_copy(hs.at[slot], h_hbm.at[u], sems.at[slot])

    def h_in_copy(slot, u):
        return pltpu.make_async_copy(h_hbm.at[u], hs.at[slot], sems.at[slot])

    @pl.when(p == 0)
    def _phase0():
        pinned, u, slot = tile_info(i)
        unpinned = jnp.logical_not(pinned)

        @pl.when(i == 0)
        def _():
            ssq_ref[...] = jnp.zeros_like(ssq_ref)
            dcol = _col(dw_ref[...].astype(F32), c)
            for j in range(nj):
                w = w1_ref[:, j * LANES:(j + 1) * LANES].astype(F32)
                w = w - jnp.mean(w, axis=0, keepdims=True)
                w1s_ref[j] = (w * dcol).astype(BF16)

        @pl.when(jnp.logical_and(unpinned, u >= ring))
        def _():
            h_out_copy(u % ring, u - ring).wait()

        dw = dw_ref[...].astype(F32)
        jb = cn // LANES
        for rb in range(tm // rbs):
            rs = slice(rb * rbs, (rb + 1) * rbs)
            x = x_ref[rs, :]
            y = x.astype(F32) * dw
            m = jnp.mean(y, axis=-1, keepdims=True)
            yc = y - m
            v = jnp.mean(yc * yc, axis=-1, keepdims=True)
            r = jax.lax.rsqrt(v + 1e-5)
            pr = _GELU_C0 * r
            qr = _GELU_C1 * (r * r * r)
            hr = 0.5 * r
            for jc in range(nj // jb):
                if jb == 1:
                    w = w1s_ref[jc]
                else:
                    w = jnp.concatenate([w1s_ref[jc * jb + k] for k in range(jb)], axis=1)
                acc = jnp.dot(x, w, preferred_element_type=F32)
                t = jnp.tanh(acc * (pr + qr * (acc * acc)))
                ha = hr * acc
                gl = ha + ha * t
                sq = jnp.sum((gl * gl).reshape(rbs // 8, 8, cn), axis=0)
                glb = gl.astype(BF16)
                for k in range(jb):
                    j = jc * jb + k
                    ls = slice(k * LANES, (k + 1) * LANES)
                    ssq_ref[j] += sq[:, ls]
                    hs[slot, j, rs, :] = glb[:, ls]

        @pl.when(jnp.logical_and(unpinned, u < nspill))
        def _():
            h_out_copy(u % ring, u).start()

    @pl.when(p == 1)
    def _phase1():
        pinned, u, slot = tile_info(nt - 1 - i)
        unpinned = jnp.logical_not(pinned)

        @pl.when(i == 0)
        def _():
            ssq = jnp.concatenate(
                [jnp.sum(ssq_ref[j], axis=0, keepdims=True) for j in range(nj)], axis=1)
            gx = jnp.sqrt(ssq + 1e-6)
            nx = gx / (jnp.mean(gx, axis=-1, keepdims=True) + 1e-6)
            s = 1.0 + g_ref[...].astype(F32) * nx
            s_t = _col(s, c4)
            for k in range(nk):
                ls = slice(k * LANES, (k + 1) * LANES)
                w2s_ref[k] = (w2_ref[:, ls].astype(F32) * s_t).astype(BF16)
            b8 = jnp.broadcast_to(b_ref[...], (16, c4))
            bias_ref[...] = jnp.dot(b8, w2_ref[...], preferred_element_type=F32)[:8]

        pinned_p, u_p, _ = tile_info(jnp.minimum(nt - i, nt - 1))

        @pl.when(jnp.logical_and(i > 0, jnp.logical_and(jnp.logical_not(pinned_p), u_p >= ring)))
        def _():
            h_in_copy(u_p % ring, u_p - ring).start()

        @pl.when(jnp.logical_and(unpinned, u < nspill))
        def _():
            h_in_copy(u % ring, u).wait()

        w2 = jnp.concatenate([w2s_ref[k] for k in range(nk)], axis=1)
        for rb in range(tm // rbs1):
            rs = slice(rb * rbs1, (rb + 1) * rbs1)
            h = jnp.concatenate([hs[slot, j, rs, :] for j in range(nj)], axis=1)
            acc = jnp.dot(h, w2, preferred_element_type=F32)
            o_ref[rs, :] = (x_ref[rs, :].astype(F32) + acc + bias_ref[0:1, :]).astype(BF16)


def _build(n, c, c4, tm=2048, cn=256, ring=3, npin=12, vmem_mb=124, phases=(0, 1),
           rbs=64, rbs1=None):
    nt = n // tm
    phases = tuple(phases)
    rbs1 = rbs1 or tm
    kern = functools.partial(_kernel, tm=tm, nt=nt, c=c, c4=c4, cn=cn, ring=ring,
                             npin=npin, phases=phases, rbs=rbs, rbs1=rbs1)
    const = lambda p, i: (0, 0)
    if phases == (1,):
        xmap = omap = lambda p, i: (nt - 1 - i, 0)
    else:
        xmap = lambda p, i: (i + p * (nt - 1 - 2 * i), 0)
        omap = lambda p, i: (nt - 1 - i * p, 0)
    nj = c4 // LANES
    once = pl.Buffered(1)
    return pl.pallas_call(
        kern,
        grid=(len(phases), nt),
        in_specs=[
            pl.BlockSpec((tm, c), xmap),
            pl.BlockSpec((1, c), const),
            pl.BlockSpec((c, c4), const, pipeline_mode=once),
            pl.BlockSpec((c4, c), const, pipeline_mode=once),
            pl.BlockSpec((1, c4), const),
            pl.BlockSpec((1, c4), const),
        ],
        out_specs=[
            pl.BlockSpec((tm, c), omap),
            pl.BlockSpec(memory_space=pl.ANY),
        ],
        out_shape=[
            jax.ShapeDtypeStruct((n, c), BF16),
            jax.ShapeDtypeStruct((nt - npin - ring, nj, tm, LANES), BF16),
        ],
        scratch_shapes=[
            pltpu.VMEM((ring + npin, nj, tm, LANES), BF16),
            pltpu.VMEM((nj, 8, LANES), F32),
            pltpu.VMEM((nj, c, LANES), BF16),
            pltpu.VMEM((c // LANES, c4, LANES), BF16),
            pltpu.VMEM((8, c), F32),
            pltpu.SemaphoreType.DMA((ring,)),
        ],
        compiler_params=pltpu.CompilerParams(
            dimension_semantics=("arbitrary", "arbitrary"),
            vmem_limit_bytes=vmem_mb * 1024 * 1024,
        ),
    )


def _run(x, dw, w1, w2, grn_g, grn_b, **kw):
    b, hh, ww, c = x.shape
    c4 = w1.shape[1]
    n = b * hh * ww
    assert b == 1 and dw.shape[0] == 1 and dw.shape[1] == 1
    out, _ = _build(n, c, c4, **kw)(
        x.reshape(n, c), dw.reshape(1, c), w1, w2,
        grn_g.reshape(1, c4), grn_b.reshape(1, c4))
    return out.reshape(x.shape)


@jax.jit
def pallas_standalone__modern_conv_block_slak__vision_kernel(
    x: jax.Array,
    dw: jax.Array,
    w1: jax.Array,
    w2: jax.Array,
    grn_g: jax.Array,
    grn_b: jax.Array,
):
    return _run(x, dw, w1, w2, grn_g, grn_b)
```

```python
import functools

import jax
import jax.numpy as jnp
import jax.experimental.pallas as pl
import jax.experimental.pallas.tpu as pltpu

F32 = jnp.float32
BF16 = jnp.bfloat16
U32 = jnp.uint32
LANES = 128

_GELU_C0 = 0.7978845608028654
_GELU_C1 = 0.7978845608028654 * 0.044715


def _col(row, n):
    return jnp.transpose(jnp.broadcast_to(row, (LANES, n)))


def _pack(v):
    return pltpu.bitcast(v, U32)


def _unpack(v):
    return pltpu.bitcast(v, BF16)


def _kernel(x_ref, dw_ref, w1_ref, w2_ref, g_ref, b_ref,
            o_ref, h_hbm,
            hs, ssq_ref, w1s_ref, w2s_ref, bias_ref, sems,
            *, tm, nt, c, c4, cn, ring, npin, phases, rbs, rbs1):
    p = pl.program_id(0)
    i = pl.program_id(1)
    if phases == (1,):
        p = p + 1
    nj = c4 // LANES
    nk = c // LANES
    nspill = nt - npin - ring

    def tile_info(t):
        lo = (t * npin) // nt
        hi = ((t + 1) * npin) // nt
        pinned = hi > lo
        u = t - lo
        slot = jnp.where(pinned, ring + lo, u % ring)
        return pinned, u, slot

    def h_out_copy(slot, u):
        return pltpu.make_async_copy(hs.at[slot], h_hbm.at[u], sems.at[slot])

    def h_in_copy(slot, u):
        return pltpu.make_async_copy(h_hbm.at[u], hs.at[slot], sems.at[slot])

    @pl.when(p == 0)
    def _phase0():
        pinned, u, slot = tile_info(i)
        unpinned = jnp.logical_not(pinned)

        @pl.when(i == 0)
        def _():
            ssq_ref[...] = jnp.zeros_like(ssq_ref)
            dcol = _col(dw_ref[...].astype(F32), c)
            for j in range(nj):
                w = w1_ref[:, j * LANES:(j + 1) * LANES].astype(F32)
                w = w - jnp.mean(w, axis=0, keepdims=True)
                w1s_ref[j] = _pack((w * dcol).astype(BF16))

        @pl.when(jnp.logical_and(unpinned, u >= ring))
        def _():
            h_out_copy(u % ring, u - ring).wait()

        dw = dw_ref[...].astype(F32)
        jb = cn // LANES
        for rb in range(tm // rbs):
            rs = slice(rb * rbs, (rb + 1) * rbs)
            xu = _pack(x_ref[rs, :])
            xf = jnp.concatenate(
                [pltpu.unpack_elementwise(xu, index=k, packed_dtype=BF16, unpacked_dtype=F32)
                 for k in range(2)], axis=0)
            x = xf.astype(BF16)
            y = xf * dw
            m = jnp.mean(y, axis=-1, keepdims=True)
            yc = y - m
            v = jnp.mean(yc * yc, axis=-1, keepdims=True)
            r = jax.lax.rsqrt(v + 1e-5)
            pr = _GELU_C0 * r
            qr = _GELU_C1 * (r * r * r)
            hr = 0.5 * r
            for jc in range(nj // jb):
                if jb == 1:
                    w = _unpack(w1s_ref[jc])
                else:
                    w = jnp.concatenate([_unpack(w1s_ref[jc * jb + k]) for k in range(jb)], axis=1)
                acc = jnp.dot(x, w, preferred_element_type=F32)
                t = jnp.tanh(acc * (pr + qr * (acc * acc)))
                ha = hr * acc
                gl = ha + ha * t
                sq = jnp.sum((gl * gl).reshape(rbs // 8, 8, cn), axis=0)
                hp = pltpu.pack_elementwise([gl[:rbs // 2], gl[rbs // 2:]], packed_dtype=BF16)
                for k in range(jb):
                    j = jc * jb + k
                    ls = slice(k * LANES, (k + 1) * LANES)
                    ssq_ref[j] += sq[:, ls]
                    hs[slot, j, rb * rbs // 2:(rb + 1) * rbs // 2, :] = hp[:, ls]

        @pl.when(jnp.logical_and(unpinned, u < nspill))
        def _():
            h_out_copy(u % ring, u).start()

    @pl.when(p == 1)
    def _phase1():
        pinned, u, slot = tile_info(nt - 1 - i)
        unpinned = jnp.logical_not(pinned)

        @pl.when(i == 0)
        def _():
            ssq = jnp.concatenate(
                [jnp.sum(ssq_ref[j], axis=0, keepdims=True) for j in range(nj)], axis=1)
            gx = jnp.sqrt(ssq + 1e-6)
            nx = gx / (jnp.mean(gx, axis=-1, keepdims=True) + 1e-6)
            s = 1.0 + g_ref[...].astype(F32) * nx
            s_t = _col(s, c4)
            for k in range(nk):
                ls = slice(k * LANES, (k + 1) * LANES)
                w2s_ref[k] = _pack((w2_ref[:, ls].astype(F32) * s_t).astype(BF16))
            b8 = jnp.broadcast_to(b_ref[...], (16, c4))
            bias_ref[...] = jnp.dot(b8, w2_ref[...], preferred_element_type=F32)[:8]

        pinned_p, u_p, _ = tile_info(jnp.minimum(nt - i, nt - 1))

        @pl.when(jnp.logical_and(i > 0, jnp.logical_and(jnp.logical_not(pinned_p), u_p >= ring)))
        def _():
            h_in_copy(u_p % ring, u_p - ring).start()

        @pl.when(jnp.logical_and(unpinned, u < nspill))
        def _():
            h_in_copy(u % ring, u).wait()

        w2 = jnp.concatenate([_unpack(w2s_ref[k]) for k in range(nk)], axis=1)
        for rb in range(tm // rbs1):
            rs = slice(rb * rbs1, (rb + 1) * rbs1)
            hrs = slice(rb * rbs1 // 2, (rb + 1) * rbs1 // 2)
            h = jnp.concatenate([_unpack(hs[slot, j, hrs, :]) for j in range(nj)], axis=1)
            acc = jnp.dot(h, w2, preferred_element_type=F32)
            o_ref[rs, :] = (x_ref[rs, :].astype(F32) + acc + bias_ref[0:1, :]).astype(BF16)


def _build(n, c, c4, tm=3072, cn=256, ring=3, npin=7, vmem_mb=124, phases=(0, 1),
           rbs=64, rbs1=None):
    nt = n // tm
    phases = tuple(phases)
    rbs1 = rbs1 or tm
    kern = functools.partial(_kernel, tm=tm, nt=nt, c=c, c4=c4, cn=cn, ring=ring,
                             npin=npin, phases=phases, rbs=rbs, rbs1=rbs1)
    const = lambda p, i: (0, 0)
    if phases == (1,):
        xmap = omap = lambda p, i: (nt - 1 - i, 0)
    else:
        xmap = lambda p, i: (i + p * (nt - 1 - 2 * i), 0)
        omap = lambda p, i: (nt - 1 - i * p, 0)
    nj = c4 // LANES
    once = pl.Buffered(1)
    return pl.pallas_call(
        kern,
        grid=(len(phases), nt),
        in_specs=[
            pl.BlockSpec((tm, c), xmap),
            pl.BlockSpec((1, c), const),
            pl.BlockSpec((c, c4), const, pipeline_mode=once),
            pl.BlockSpec((c4, c), const, pipeline_mode=once),
            pl.BlockSpec((1, c4), const),
            pl.BlockSpec((1, c4), const),
        ],
        out_specs=[
            pl.BlockSpec((tm, c), omap),
            pl.BlockSpec(memory_space=pl.ANY),
        ],
        out_shape=[
            jax.ShapeDtypeStruct((n, c), BF16),
            jax.ShapeDtypeStruct((nt - npin - ring, nj, tm // 2, LANES), U32),
        ],
        scratch_shapes=[
            pltpu.VMEM((ring + npin, nj, tm // 2, LANES), U32),
            pltpu.VMEM((nj, 8, LANES), F32),
            pltpu.VMEM((nj, c // 2, LANES), U32),
            pltpu.VMEM((c // LANES, c4 // 2, LANES), U32),
            pltpu.VMEM((8, c), F32),
            pltpu.SemaphoreType.DMA((ring,)),
        ],
        compiler_params=pltpu.CompilerParams(
            dimension_semantics=("arbitrary", "arbitrary"),
            vmem_limit_bytes=vmem_mb * 1024 * 1024,
        ),
    )


def _run(x, dw, w1, w2, grn_g, grn_b, **kw):
    b, hh, ww, c = x.shape
    c4 = w1.shape[1]
    n = b * hh * ww
    assert b == 1 and dw.shape[0] == 1 and dw.shape[1] == 1
    out, _ = _build(n, c, c4, **kw)(
        x.reshape(n, c), dw.reshape(1, c), w1, w2,
        grn_g.reshape(1, c4), grn_b.reshape(1, c4))
    return out.reshape(x.shape)


@jax.jit
def pallas_standalone__modern_conv_block_slak__vision_kernel(
    x: jax.Array,
    dw: jax.Array,
    w1: jax.Array,
    w2: jax.Array,
    grn_g: jax.Array,
    grn_b: jax.Array,
):
    return _run(x, dw, w1, w2, grn_g, grn_b)
```

```python
import functools

import jax
import jax.numpy as jnp
import jax.experimental.pallas as pl
import jax.experimental.pallas.tpu as pltpu

F32 = jnp.float32
BF16 = jnp.bfloat16
U32 = jnp.uint32
LANES = 128

_GELU_C0 = 0.7978845608028654
_GELU_C1 = 0.7978845608028654 * 0.044715
_LAM = _GELU_C1 ** (1.0 / 3.0)
_KAP = _GELU_C0 / _LAM
_HSCALE = 1.0 / (2.0 * _LAM)


def _col(row, n):
    return jnp.transpose(jnp.broadcast_to(row, (LANES, n)))


def _pack(v):
    return pltpu.bitcast(v, U32)


def _unpack(v):
    return pltpu.bitcast(v, BF16)


def _kernel(x_ref, dw_ref, w1_ref, w2_ref, g_ref, b_ref,
            o_ref, h_hbm,
            hs, ssq_ref, w1s_ref, w2s_ref, bias_ref, sems,
            *, tm, nt, c, c4, cn, ring, npin, phases, rbs, rbs1, st1, nodma, st0):
    p = pl.program_id(0)
    i = pl.program_id(1)
    if phases == (1,):
        p = p + 1
    nj = c4 // LANES
    nk = c // LANES
    nspill = nt - npin - ring

    def tile_info(t):
        lo = (t * npin) // nt
        hi = ((t + 1) * npin) // nt
        pinned = hi > lo
        u = t - lo
        slot = jnp.where(pinned, ring + lo, u % ring)
        return pinned, u, slot

    def h_out_copy(slot, u):
        return pltpu.make_async_copy(hs.at[slot], h_hbm.at[u], sems.at[slot])

    def h_in_copy(slot, u):
        return pltpu.make_async_copy(h_hbm.at[u], hs.at[slot], sems.at[slot])

    @pl.when(p == 0)
    def _phase0():
        pinned, u, slot = tile_info(i)
        unpinned = jnp.logical_not(pinned)

        @pl.when(i == 0)
        def _():
            ssq_ref[...] = jnp.zeros_like(ssq_ref)
            if not st0:
                dcol = _col(dw_ref[...].astype(F32), c)
                for j in range(nj):
                    w = w1_ref[:, j * LANES:(j + 1) * LANES].astype(F32)
                    w = w - jnp.mean(w, axis=0, keepdims=True)
                    w1s_ref[j] = _pack((w * dcol).astype(BF16))
            else:
                njh = nj // 2
                for j in range(njh):
                    cl = slice(j * LANES, (j + 1) * LANES)
                    cr = slice((njh + j) * LANES, (njh + j + 1) * LANES)
                    b11 = w1_ref[0:LANES, cl].astype(F32)
                    b12 = w1_ref[0:LANES, cr].astype(F32)
                    b21 = w1_ref[LANES:2 * LANES, cl].astype(F32)
                    b22 = w1_ref[LANES:2 * LANES, cr].astype(F32)
                    combos = [b11 + b22, b11, b12 - b22, b21 - b11, b22, b11 + b12, b21 + b22]
                    for q, t in enumerate(combos):
                        w1s_ref[q * njh + j] = _pack(t.astype(BF16))
                    w1s_ref[7 * njh + j] = _pack(w1_ref[2 * LANES:3 * LANES, cl])
                    w1s_ref[8 * njh + j] = _pack(w1_ref[2 * LANES:3 * LANES, cr])

        @pl.when(jnp.logical_and(unpinned, u >= ring))
        def _():
            h_out_copy(u % ring, u - ring).wait()

        dw = dw_ref[...].astype(F32)
        jb = cn // LANES
        dot = functools.partial(jnp.dot, preferred_element_type=F32)

        def gelu(b):
            return b * (1.0 + jnp.tanh(b * (b * b + _KAP)))

        def layernorm(xf):
            y = xf * dw
            yc = y - jnp.mean(y, axis=-1, keepdims=True)
            v = jnp.mean(yc * yc, axis=-1, keepdims=True)
            return yc * (_LAM * jax.lax.rsqrt(v + 1e-5))

        for rb in range(tm // rbs if st0 else 0):
            hh = rbs // 2
            njh = nj // 2
            xu = _pack(x_ref[rb * rbs:(rb + 1) * rbs, :])
            a1, a2 = [layernorm(pltpu.unpack_elementwise(
                xu, index=k, packed_dtype=BF16, unpacked_dtype=F32)) for k in range(2)]
            a11, a12, a13 = (a1[:, k * LANES:(k + 1) * LANES] for k in range(3))
            a21, a22, a23 = (a2[:, k * LANES:(k + 1) * LANES] for k in range(3))
            s1 = (a11 + a22).astype(BF16)
            s2 = (a21 + a22).astype(BF16)
            s5 = (a11 + a12).astype(BF16)
            s6 = (a21 - a11).astype(BF16)
            s7 = (a12 - a22).astype(BF16)
            s3 = a11.astype(BF16)
            s4 = a22.astype(BF16)
            kk = jnp.concatenate([a13, a23], axis=0).astype(BF16)
            qs = slice(rb * hh, (rb + 1) * hh)
            for jc in range(njh // jb):
                def wq(q):
                    ws = [_unpack(w1s_ref[q * njh + jc * jb + k]) for k in range(jb)]
                    return ws[0] if jb == 1 else jnp.concatenate(ws, axis=1)
                m1 = dot(s1, wq(0))
                m2 = dot(s2, wq(1))
                m3 = dot(s3, wq(2))
                m4 = dot(s4, wq(3))
                m5 = dot(s5, wq(4))
                m6 = dot(s6, wq(5))
                m7 = dot(s7, wq(6))
                kl = dot(kk, wq(7))
                kr = dot(kk, wq(8))
                g11 = gelu(m1 + m4 - m5 + m7 + kl[:hh])
                g12 = gelu(m3 + m5 + kr[:hh])
                g21 = gelu(m2 + m4 + kl[hh:])
                g22 = gelu(m1 - m2 + m3 + m6 + kr[hh:])
                for (gt, gb, j0) in ((g11, g21, jc * jb), (g12, g22, njh + jc * jb)):
                    sq = jnp.sum((gt * gt + gb * gb).reshape(hh // 8, 8, cn), axis=0)
                    hp = pltpu.pack_elementwise([gt, gb], packed_dtype=BF16)
                    for k in range(jb):
                        ls = slice(k * LANES, (k + 1) * LANES)
                        ssq_ref[j0 + k] += sq[:, ls]
                        hs[slot, j0 + k, qs, :] = hp[:, ls]

        for rb in range(0 if st0 else tm // rbs):
            rs = slice(rb * rbs, (rb + 1) * rbs)
            xu = _pack(x_ref[rs, :])
            xf = jnp.concatenate(
                [pltpu.unpack_elementwise(xu, index=k, packed_dtype=BF16, unpacked_dtype=F32)
                 for k in range(2)], axis=0)
            x = xf.astype(BF16)
            y = xf * dw
            m = jnp.mean(y, axis=-1, keepdims=True)
            yc = y - m
            v = jnp.mean(yc * yc, axis=-1, keepdims=True)
            r = jax.lax.rsqrt(v + 1e-5)
            pr = _GELU_C0 * r
            qr = _GELU_C1 * (r * r * r)
            hr = 0.5 * r
            for jc in range(nj // jb):
                if jb == 1:
                    w = _unpack(w1s_ref[jc])
                else:
                    w = jnp.concatenate([_unpack(w1s_ref[jc * jb + k]) for k in range(jb)], axis=1)
                acc = jnp.dot(x, w, preferred_element_type=F32)
                t = jnp.tanh(acc * (pr + qr * (acc * acc)))
                ha = hr * acc
                gl = ha + ha * t
                sq = jnp.sum((gl * gl).reshape(rbs // 8, 8, cn), axis=0)
                hp = pltpu.pack_elementwise([gl[:rbs // 2], gl[rbs // 2:]], packed_dtype=BF16)
                for k in range(jb):
                    j = jc * jb + k
                    ls = slice(k * LANES, (k + 1) * LANES)
                    ssq_ref[j] += sq[:, ls]
                    hs[slot, j, rb * rbs // 2:(rb + 1) * rbs // 2, :] = hp[:, ls]

        @pl.when(jnp.logical_and(unpinned, u < nspill))
        def _():
            h_out_copy(u % ring, u).start()

    @pl.when(p == 1)
    def _phase1():
        pinned, u, slot = tile_info(nt - 1 - i)
        unpinned = jnp.logical_not(pinned)

        @pl.when(i == 0)
        def _():
            ssq = jnp.concatenate(
                [jnp.sum(ssq_ref[j], axis=0, keepdims=True) for j in range(nj)], axis=1)
            if st0:
                ssq = ssq * (_HSCALE * _HSCALE)
            gx = jnp.sqrt(ssq + 1e-6)
            nx = gx / (jnp.mean(gx, axis=-1, keepdims=True) + 1e-6)
            s = 1.0 + g_ref[...].astype(F32) * nx
            if st0:
                s = s * _HSCALE
            s_t = _col(s, c4)
            if not st1:
                for k in range(nk):
                    ls = slice(k * LANES, (k + 1) * LANES)
                    w2s_ref[k] = _pack((w2_ref[:, ls].astype(F32) * s_t).astype(BF16))
            else:
                kh = c4 // 2
                ws = [w2_ref[:, k * LANES:(k + 1) * LANES].astype(F32) * s_t for k in range(nk)]
                b11, b21 = ws[0][:kh], ws[0][kh:]
                b12, b22 = ws[1][:kh], ws[1][kh:]
                combos = [b11 + b22, b11, b12 - b22, b21 - b11, b22, b11 + b12, b21 + b22]
                for q, t in enumerate(combos):
                    w2s_ref[q] = _pack(t.astype(BF16))
                w2s_ref[7] = _pack(ws[2][:kh].astype(BF16))
                w2s_ref[8] = _pack(ws[2][kh:].astype(BF16))
            b8 = jnp.broadcast_to(b_ref[...], (16, c4))
            bias_ref[...] = jnp.dot(b8, w2_ref[...], preferred_element_type=F32)[:8]

        pinned_p, u_p, _ = tile_info(jnp.minimum(nt - i, nt - 1))

        if not nodma:
            @pl.when(jnp.logical_and(i > 0, jnp.logical_and(jnp.logical_not(pinned_p), u_p >= ring)))
            def _():
                h_in_copy(u_p % ring, u_p - ring).start()

            @pl.when(jnp.logical_and(unpinned, u < nspill))
            def _():
                h_in_copy(u % ring, u).wait()

        if not st1:
            w2 = jnp.concatenate([_unpack(w2s_ref[k]) for k in range(nk)], axis=1)
            for rb in range(tm // rbs1):
                rs = slice(rb * rbs1, (rb + 1) * rbs1)
                hrs = slice(rb * rbs1 // 2, (rb + 1) * rbs1 // 2)
                h = jnp.concatenate([_unpack(hs[slot, j, hrs, :]) for j in range(nj)], axis=1)
                acc = jnp.dot(h, w2, preferred_element_type=F32)
                o_ref[rs, :] = (x_ref[rs, :].astype(F32) + acc + bias_ref[0:1, :]).astype(BF16)
        else:
            hh = rbs1 // 2
            njh = nj // 2
            dot = functools.partial(jnp.dot, preferred_element_type=F32)
            wq = lambda q: _unpack(w2s_ref[q])
            bias = bias_ref[0:1, :]
            for rb in range(tm // rbs1):
                r0 = rb * rbs1

                def blk(half, kk):
                    q0 = (r0 + half * hh) // 2
                    return jnp.concatenate(
                        [_unpack(hs[slot, kk * njh + j, q0:q0 + hh // 2, :]) for j in range(njh)],
                        axis=1)

                a11, a12, a21, a22 = blk(0, 0), blk(0, 1), blk(1, 0), blk(1, 1)
                f11, f12, f21, f22 = (a.astype(F32) for a in (a11, a12, a21, a22))
                m1 = dot((f11 + f22).astype(BF16), wq(0))
                m2 = dot((f21 + f22).astype(BF16), wq(1))
                m3 = dot(a11, wq(2))
                m4 = dot(a22, wq(3))
                m5 = dot((f11 + f12).astype(BF16), wq(4))
                m6 = dot((f21 - f11).astype(BF16), wq(5))
                m7 = dot((f12 - f22).astype(BF16), wq(6))
                c11 = m1 + m4 - m5 + m7
                c12 = m3 + m5
                c21 = m2 + m4
                c22 = m1 - m2 + m3 + m6
                w3 = jnp.concatenate([wq(7), wq(8)], axis=0)
                c13 = dot(jnp.concatenate([a11, a12], axis=1), w3)
                c23 = dot(jnp.concatenate([a21, a22], axis=1), w3)
                top = jnp.concatenate([c11, c12, c13], axis=1)
                bot = jnp.concatenate([c21, c22, c23], axis=1)
                rt = slice(r0, r0 + hh)
                rbm = slice(r0 + hh, r0 + 2 * hh)
                o_ref[rt, :] = (x_ref[rt, :].astype(F32) + top + bias).astype(BF16)
                o_ref[rbm, :] = (x_ref[rbm, :].astype(F32) + bot + bias).astype(BF16)


def _build(n, c, c4, tm=2048, cn=256, ring=3, npin=13, vmem_mb=124, phases=(0, 1),
           rbs=128, rbs1=512, st1=True, nodma=False, st0=True):
    nt = n // tm
    phases = tuple(phases)
    rbs1 = rbs1 or tm
    kern = functools.partial(_kernel, tm=tm, nt=nt, c=c, c4=c4, cn=cn, ring=ring,
                             npin=npin, phases=phases, rbs=rbs, rbs1=rbs1, st1=st1, nodma=nodma, st0=st0)
    const = lambda p, i: (0, 0)
    if phases == (1,):
        xmap = omap = lambda p, i: (nt - 1 - i, 0)
    else:
        xmap = lambda p, i: (i + p * (nt - 1 - 2 * i), 0)
        omap = lambda p, i: (nt - 1 - i * p, 0)
    nj = c4 // LANES
    once = pl.Buffered(1)
    return pl.pallas_call(
        kern,
        grid=(len(phases), nt),
        in_specs=[
            pl.BlockSpec((tm, c), xmap),
            pl.BlockSpec((1, c), const),
            pl.BlockSpec((c, c4), const, pipeline_mode=once),
            pl.BlockSpec((c4, c), const, pipeline_mode=once),
            pl.BlockSpec((1, c4), const),
            pl.BlockSpec((1, c4), const),
        ],
        out_specs=[
            pl.BlockSpec((tm, c), omap),
            pl.BlockSpec(memory_space=pl.ANY),
        ],
        out_shape=[
            jax.ShapeDtypeStruct((n, c), BF16),
            jax.ShapeDtypeStruct((nt - npin - ring, nj, tm // 2, LANES), U32),
        ],
        scratch_shapes=[
            pltpu.VMEM((ring + npin, nj, tm // 2, LANES), U32),
            pltpu.VMEM((nj, 8, LANES), F32),
            pltpu.VMEM((9 * nj // 2, LANES // 2, LANES) if st0 else (nj, c // 2, LANES), U32),
            pltpu.VMEM((9, c4 // 4, LANES) if st1 else (c // LANES, c4 // 2, LANES), U32),
            pltpu.VMEM((8, c), F32),
            pltpu.SemaphoreType.DMA((ring,)),
        ],
        compiler_params=pltpu.CompilerParams(
            dimension_semantics=("arbitrary", "arbitrary"),
            vmem_limit_bytes=vmem_mb * 1024 * 1024,
        ),
    )


def _run(x, dw, w1, w2, grn_g, grn_b, **kw):
    b, hh, ww, c = x.shape
    c4 = w1.shape[1]
    n = b * hh * ww
    assert b == 1 and dw.shape[0] == 1 and dw.shape[1] == 1
    out, _ = _build(n, c, c4, **kw)(
        x.reshape(n, c), dw.reshape(1, c), w1, w2,
        grn_g.reshape(1, c4), grn_b.reshape(1, c4))
    return out.reshape(x.shape)


@jax.jit
def pallas_standalone__modern_conv_block_slak__vision_kernel(
    x: jax.Array,
    dw: jax.Array,
    w1: jax.Array,
    w2: jax.Array,
    grn_g: jax.Array,
    grn_b: jax.Array,
):
    return _run(x, dw, w1, w2, grn_g, grn_b)
```

```python
import functools

import jax
import jax.numpy as jnp
import jax.experimental.pallas as pl
import jax.experimental.pallas.tpu as pltpu

F32 = jnp.float32
BF16 = jnp.bfloat16
U32 = jnp.uint32
LANES = 128

_GELU_C0 = 0.7978845608028654
_GELU_C1 = 0.7978845608028654 * 0.044715
_LAM = _GELU_C1 ** (1.0 / 3.0)
_KAP = _GELU_C0 / _LAM
_HSCALE = 1.0 / (2.0 * _LAM)


_HK_U = ((0, 0, 0, 1, -1, 0), (-1, 0, 0, 0, 0, 1), (1, 0, 0, -1, 0, 0), (-1, 0, 0, 0, 0, 0),
         (0, 0, -1, 0, 0, 1), (1, 0, 0, -1, 1, 0), (0, -1, 0, 0, 0, 0), (0, -1, 1, 0, 0, -1),
         (0, 1, -1, 0, 0, 0), (1, 0, -1, 0, 0, 0), (0, 0, 0, 0, -1, 0), (0, 0, 0, -1, 0, 1),
         (0, 1, -1, 0, -1, 1), (-1, 1, 0, 1, -1, 0), (0, 0, 0, 0, 0, 1))
_HK_V = ((0, 0, 1, 0, 0, 0, 0, 0, 0), (0, -1, 0, 0, 0, 0, 1, 0, 0), (1, 1, 0, 1, 0, 0, 0, 0, 0),
         (1, 0, -1, 0, 0, 0, 1, 0, 0), (0, 0, 0, 0, 1, 0, 1, 1, 0), (0, 0, 1, 1, 0, 0, 0, 0, 0),
         (0, 0, 0, -1, 0, 1, 0, 0, 1), (0, 0, 0, 0, -1, 0, 0, 0, -1), (0, 0, 0, 0, 0, 0, 0, 0, 1),
         (0, 0, 0, 0, 0, 0, 1, 0, 0), (0, 0, 1, 0, -1, 1, 0, 0, 0), (0, -1, 0, 0, 0, 0, 0, 0, 0),
         (0, 0, 0, 0, -1, 0, 0, 0, 0), (0, 0, 0, 1, 0, 0, 0, 0, 0), (0, -1, 0, 0, 0, 0, 0, -1, 1))
_HK_W = ((1, 0, 1, 1, 0, 1), (0, 1, 0, 1, 0, 0), (0, 0, 0, -1, 0, 0), (-1, 0, 0, -1, 0, 0),
         (0, -1, 0, 0, 0, 0), (1, 0, 1, 1, 0, 0), (0, 0, -1, 0, 0, 0), (0, 1, 0, 0, 1, 1),
         (0, -1, -1, 0, -1, -1), (-1, 1, 0, 0, 0, 0), (0, 0, 0, 0, 0, -1), (0, 0, 0, -1, 1, 0),
         (0, 0, 0, 0, 1, 1), (1, 0, 1, 0, 0, 0), (0, -1, 0, 0, -1, 0))


def _combos(rows, vals):
    vals = list(vals)
    rows = [{i: c for i, c in enumerate(r) if c} for r in rows]
    while True:
        cnt = {}
        for r in rows:
            ks = sorted(r)
            for ia, a in enumerate(ks):
                for b in ks[ia + 1:]:
                    key = (a, b, r[a] * r[b])
                    cnt[key] = cnt.get(key, 0) + 1
        if not cnt or max(cnt.values()) < 2:
            break
        a, b, sg = max(sorted(cnt), key=lambda k_: cnt[k_])
        vals.append(_lazy(lambda a=a, b=b, sg=sg: (
            _force(vals[a]) + _force(vals[b]) if sg > 0 else _force(vals[a]) - _force(vals[b]))))
        new = len(vals) - 1
        for r in rows:
            if a in r and b in r and r[a] * r[b] == sg:
                r[new] = r.pop(a)
                del r[b]
    out = []
    for r in rows:
        items = sorted(r.items(), key=lambda kv: -kv[1])
        sign = items[0][1]
        acc = _force(vals[items[0][0]])
        for idx, cf in items[1:]:
            acc = acc + _force(vals[idx]) if cf * sign > 0 else acc - _force(vals[idx])
        out.append((acc, sign))
    return out


class _lazy:
    def __init__(self, fn):
        self.fn, self.val = fn, None


def _force(v):
    if isinstance(v, _lazy):
        if v.val is None:
            v.val = v.fn()
        return v.val
    return v


_HK_USIGN = tuple(sg for _, sg in _combos(_HK_U, [1.0] * 6))


def _col(row, n):
    return jnp.transpose(jnp.broadcast_to(row, (LANES, n)))


def _pack(v):
    return pltpu.bitcast(v, U32)


def _unpack(v):
    return pltpu.bitcast(v, BF16)


def _kernel(x_ref, dw_ref, w1_ref, w2_ref, g_ref, b_ref,
            o_ref, h_hbm,
            hs, ssq_ref, w1s_ref, w2s_ref, bias_ref, sems,
            *, tm, nt, c, c4, cn, ring, npin, phases, rbs, rbs1, st1, nodma, st0):
    p = pl.program_id(0)
    i = pl.program_id(1)
    if phases == (1,):
        p = p + 1
    nj = c4 // LANES
    nk = c // LANES
    nspill = nt - npin - ring

    def tile_info(t):
        lo = (t * npin) // nt
        hi = ((t + 1) * npin) // nt
        pinned = hi > lo
        u = t - lo
        slot = jnp.where(pinned, ring + lo, u % ring)
        return pinned, u, slot

    def h_out_copy(slot, u):
        return pltpu.make_async_copy(hs.at[slot], h_hbm.at[u], sems.at[slot])

    def h_in_copy(slot, u):
        return pltpu.make_async_copy(h_hbm.at[u], hs.at[slot], sems.at[slot])

    @pl.when(p == 0)
    def _phase0():
        pinned, u, slot = tile_info(i)
        unpinned = jnp.logical_not(pinned)

        @pl.when(i == 0)
        def _():
            ssq_ref[...] = jnp.zeros_like(ssq_ref)
            if not st0:
                dcol = _col(dw_ref[...].astype(F32), c)
                for j in range(nj):
                    w = w1_ref[:, j * LANES:(j + 1) * LANES].astype(F32)
                    w = w - jnp.mean(w, axis=0, keepdims=True)
                    w1s_ref[j] = _pack((w * dcol).astype(BF16))
            else:
                njh = nj // 2
                for j in range(njh):
                    cl = slice(j * LANES, (j + 1) * LANES)
                    cr = slice((njh + j) * LANES, (njh + j + 1) * LANES)
                    b11 = w1_ref[0:LANES, cl].astype(F32)
                    b12 = w1_ref[0:LANES, cr].astype(F32)
                    b21 = w1_ref[LANES:2 * LANES, cl].astype(F32)
                    b22 = w1_ref[LANES:2 * LANES, cr].astype(F32)
                    combos = [b11 + b22, b11, b12 - b22, b21 - b11, b22, b11 + b12, b21 + b22]
                    for q, t in enumerate(combos):
                        w1s_ref[q * njh + j] = _pack(t.astype(BF16))
                    w1s_ref[7 * njh + j] = _pack(w1_ref[2 * LANES:3 * LANES, cl])
                    w1s_ref[8 * njh + j] = _pack(w1_ref[2 * LANES:3 * LANES, cr])

        @pl.when(jnp.logical_and(unpinned, u >= ring))
        def _():
            h_out_copy(u % ring, u - ring).wait()

        dw = dw_ref[...].astype(F32)
        jb = cn // LANES
        dot = functools.partial(jnp.dot, preferred_element_type=F32)

        def gelu(b):
            return b * (1.0 + jnp.tanh(b * (b * b + _KAP)))

        def layernorm(xf):
            y = xf * dw
            yc = y - jnp.mean(y, axis=-1, keepdims=True)
            v = jnp.mean(yc * yc, axis=-1, keepdims=True)
            return yc * (_LAM * jax.lax.rsqrt(v + 1e-5))

        for rb in range(tm // rbs if st0 else 0):
            hh = rbs // 2
            njh = nj // 2
            xu = _pack(x_ref[rb * rbs:(rb + 1) * rbs, :])
            a1, a2 = [layernorm(pltpu.unpack_elementwise(
                xu, index=k, packed_dtype=BF16, unpacked_dtype=F32)) for k in range(2)]
            a11, a12, a13 = (a1[:, k * LANES:(k + 1) * LANES] for k in range(3))
            a21, a22, a23 = (a2[:, k * LANES:(k + 1) * LANES] for k in range(3))
            s1 = (a11 + a22).astype(BF16)
            s2 = (a21 + a22).astype(BF16)
            s5 = (a11 + a12).astype(BF16)
            s6 = (a21 - a11).astype(BF16)
            s7 = (a12 - a22).astype(BF16)
            s3 = a11.astype(BF16)
            s4 = a22.astype(BF16)
            kk = jnp.concatenate([a13, a23], axis=0).astype(BF16)
            qs = slice(rb * hh, (rb + 1) * hh)
            for jc in range(njh // jb):
                def wq(q):
                    ws = [_unpack(w1s_ref[q * njh + jc * jb + k]) for k in range(jb)]
                    return ws[0] if jb == 1 else jnp.concatenate(ws, axis=1)
                m1 = dot(s1, wq(0))
                m2 = dot(s2, wq(1))
                m3 = dot(s3, wq(2))
                m4 = dot(s4, wq(3))
                m5 = dot(s5, wq(4))
                m6 = dot(s6, wq(5))
                m7 = dot(s7, wq(6))
                kl = dot(kk, wq(7))
                kr = dot(kk, wq(8))
                g11 = gelu(m1 + m4 - m5 + m7 + kl[:hh])
                g12 = gelu(m3 + m5 + kr[:hh])
                g21 = gelu(m2 + m4 + kl[hh:])
                g22 = gelu(m1 - m2 + m3 + m6 + kr[hh:])
                for (gt, gb, j0) in ((g11, g21, jc * jb), (g12, g22, njh + jc * jb)):
                    sq = jnp.sum((gt * gt + gb * gb).reshape(hh // 8, 8, cn), axis=0)
                    hp = pltpu.pack_elementwise([gt, gb], packed_dtype=BF16)
                    for k in range(jb):
                        ls = slice(k * LANES, (k + 1) * LANES)
                        ssq_ref[j0 + k] += sq[:, ls]
                        hs[slot, j0 + k, qs, :] = hp[:, ls]

        for rb in range(0 if st0 else tm // rbs):
            rs = slice(rb * rbs, (rb + 1) * rbs)
            xu = _pack(x_ref[rs, :])
            xf = jnp.concatenate(
                [pltpu.unpack_elementwise(xu, index=k, packed_dtype=BF16, unpacked_dtype=F32)
                 for k in range(2)], axis=0)
            x = xf.astype(BF16)
            y = xf * dw
            m = jnp.mean(y, axis=-1, keepdims=True)
            yc = y - m
            v = jnp.mean(yc * yc, axis=-1, keepdims=True)
            r = jax.lax.rsqrt(v + 1e-5)
            pr = _GELU_C0 * r
            qr = _GELU_C1 * (r * r * r)
            hr = 0.5 * r
            for jc in range(nj // jb):
                if jb == 1:
                    w = _unpack(w1s_ref[jc])
                else:
                    w = jnp.concatenate([_unpack(w1s_ref[jc * jb + k]) for k in range(jb)], axis=1)
                acc = jnp.dot(x, w, preferred_element_type=F32)
                t = jnp.tanh(acc * (pr + qr * (acc * acc)))
                ha = hr * acc
                gl = ha + ha * t
                sq = jnp.sum((gl * gl).reshape(rbs // 8, 8, cn), axis=0)
                hp = pltpu.pack_elementwise([gl[:rbs // 2], gl[rbs // 2:]], packed_dtype=BF16)
                for k in range(jb):
                    j = jc * jb + k
                    ls = slice(k * LANES, (k + 1) * LANES)
                    ssq_ref[j] += sq[:, ls]
                    hs[slot, j, rb * rbs // 2:(rb + 1) * rbs // 2, :] = hp[:, ls]

        @pl.when(jnp.logical_and(unpinned, u < nspill))
        def _():
            h_out_copy(u % ring, u).start()

    @pl.when(p == 1)
    def _phase1():
        pinned, u, slot = tile_info(nt - 1 - i)
        unpinned = jnp.logical_not(pinned)

        @pl.when(i == 0)
        def _():
            ssq = jnp.concatenate(
                [jnp.sum(ssq_ref[j], axis=0, keepdims=True) for j in range(nj)], axis=1)
            if st0:
                ssq = ssq * (_HSCALE * _HSCALE)
            gx = jnp.sqrt(ssq + 1e-6)
            nx = gx / (jnp.mean(gx, axis=-1, keepdims=True) + 1e-6)
            s = 1.0 + g_ref[...].astype(F32) * nx
            if st0:
                s = s * _HSCALE
            s_t = _col(s, c4)
            if st1 == 2:
                kb = c4 // 3
                ws = [w2_ref[:, k * LANES:(k + 1) * LANES].astype(F32) * s_t for k in range(nk)]
                bl = [ws[l][j * kb:(j + 1) * kb] for j in range(3) for l in range(3)]
                for q, (t, sg) in enumerate(_combos(_HK_V, bl)):
                    if sg * _HK_USIGN[q] < 0:
                        t = -t
                    w2s_ref[q] = _pack(t.astype(BF16))
            elif not st1:
                for k in range(nk):
                    ls = slice(k * LANES, (k + 1) * LANES)
                    w2s_ref[k] = _pack((w2_ref[:, ls].astype(F32) * s_t).astype(BF16))
            else:
                kh = c4 // 2
                ws = [w2_ref[:, k * LANES:(k + 1) * LANES].astype(F32) * s_t for k in range(nk)]
                b11, b21 = ws[0][:kh], ws[0][kh:]
                b12, b22 = ws[1][:kh], ws[1][kh:]
                combos = [b11 + b22, b11, b12 - b22, b21 - b11, b22, b11 + b12, b21 + b22]
                for q, t in enumerate(combos):
                    w2s_ref[q] = _pack(t.astype(BF16))
                w2s_ref[7] = _pack(ws[2][:kh].astype(BF16))
                w2s_ref[8] = _pack(ws[2][kh:].astype(BF16))
            b8 = jnp.broadcast_to(b_ref[...], (16, c4))
            bias_ref[...] = jnp.dot(b8, w2_ref[...], preferred_element_type=F32)[:8]

        pinned_p, u_p, _ = tile_info(jnp.minimum(nt - i, nt - 1))

        if not nodma:
            @pl.when(jnp.logical_and(i > 0, jnp.logical_and(jnp.logical_not(pinned_p), u_p >= ring)))
            def _():
                h_in_copy(u_p % ring, u_p - ring).start()

            @pl.when(jnp.logical_and(unpinned, u < nspill))
            def _():
                h_in_copy(u % ring, u).wait()

        if st1 == 2:
            hh = rbs1 // 2
            njk = nj // 3
            dot = functools.partial(jnp.dot, preferred_element_type=F32)
            bias = bias_ref[0:1, :]
            for rb in range(tm // rbs1):
                r0 = rb * rbs1
                raw = [jnp.concatenate(
                    [_unpack(hs[slot, kk * njk + j, (r0 + half * hh) // 2:(r0 + (half + 1) * hh) // 2, :])
                     for j in range(njk)], axis=1) for half in range(2) for kk in range(3)]
                flt = [_lazy(lambda a=a: a.astype(F32)) for a in raw]
                lhs = _combos(_HK_U, flt)
                ms = []
                for q, row in enumerate(_HK_U):
                    nzs = [ix for ix, cf in enumerate(row) if cf]
                    a = raw[nzs[0]] if len(nzs) == 1 else lhs[q][0].astype(BF16)
                    ms.append(dot(a, _unpack(w2s_ref[q])))
                cs = _combos([[w[o] for w in _HK_W] for o in range(6)], ms)
                for half in range(2):
                    rs = slice(r0 + half * hh, r0 + (half + 1) * hh)
                    for l in range(3):
                        cl = slice(l * LANES, (l + 1) * LANES)
                        val, sg = cs[half * 3 + l]
                        base = x_ref[rs, cl].astype(F32) + bias[:, cl]
                        o_ref[rs, cl] = (base + val if sg > 0 else base - val).astype(BF16)
        elif not st1:
            w2 = jnp.concatenate([_unpack(w2s_ref[k]) for k in range(nk)], axis=1)
            for rb in range(tm // rbs1):
                rs = slice(rb * rbs1, (rb + 1) * rbs1)
                hrs = slice(rb * rbs1 // 2, (rb + 1) * rbs1 // 2)
                h = jnp.concatenate([_unpack(hs[slot, j, hrs, :]) for j in range(nj)], axis=1)
                acc = jnp.dot(h, w2, preferred_element_type=F32)
                o_ref[rs, :] = (x_ref[rs, :].astype(F32) + acc + bias_ref[0:1, :]).astype(BF16)
        else:
            hh = rbs1 // 2
            njh = nj // 2
            dot = functools.partial(jnp.dot, preferred_element_type=F32)
            wq = lambda q: _unpack(w2s_ref[q])
            bias = bias_ref[0:1, :]
            for rb in range(tm // rbs1):
                r0 = rb * rbs1

                def blk(half, kk):
                    q0 = (r0 + half * hh) // 2
                    return jnp.concatenate(
                        [_unpack(hs[slot, kk * njh + j, q0:q0 + hh // 2, :]) for j in range(njh)],
                        axis=1)

                a11, a12, a21, a22 = blk(0, 0), blk(0, 1), blk(1, 0), blk(1, 1)
                f11, f12, f21, f22 = (a.astype(F32) for a in (a11, a12, a21, a22))
                m1 = dot((f11 + f22).astype(BF16), wq(0))
                m2 = dot((f21 + f22).astype(BF16), wq(1))
                m3 = dot(a11, wq(2))
                m4 = dot(a22, wq(3))
                m5 = dot((f11 + f12).astype(BF16), wq(4))
                m6 = dot((f21 - f11).astype(BF16), wq(5))
                m7 = dot((f12 - f22).astype(BF16), wq(6))
                c11 = m1 + m4 - m5 + m7
                c12 = m3 + m5
                c21 = m2 + m4
                c22 = m1 - m2 + m3 + m6
                w3 = jnp.concatenate([wq(7), wq(8)], axis=0)
                c13 = dot(jnp.concatenate([a11, a12], axis=1), w3)
                c23 = dot(jnp.concatenate([a21, a22], axis=1), w3)
                top = jnp.concatenate([c11, c12, c13], axis=1)
                bot = jnp.concatenate([c21, c22, c23], axis=1)
                rt = slice(r0, r0 + hh)
                rbm = slice(r0 + hh, r0 + 2 * hh)
                o_ref[rt, :] = (x_ref[rt, :].astype(F32) + top + bias).astype(BF16)
                o_ref[rbm, :] = (x_ref[rbm, :].astype(F32) + bot + bias).astype(BF16)


def _build(n, c, c4, tm=2048, cn=256, ring=3, npin=15, vmem_mb=128, phases=(0, 1),
           rbs=128, rbs1=128, st1=2, nodma=False, st0=True, xbuf=2, obuf=2):
    nt = n // tm
    phases = tuple(phases)
    rbs1 = rbs1 or tm
    kern = functools.partial(_kernel, tm=tm, nt=nt, c=c, c4=c4, cn=cn, ring=ring,
                             npin=npin, phases=phases, rbs=rbs, rbs1=rbs1, st1=st1, nodma=nodma, st0=st0)
    const = lambda p, i: (0, 0)
    if phases == (1,):
        xmap = omap = lambda p, i: (nt - 1 - i, 0)
    else:
        xmap = lambda p, i: (i + p * (nt - 1 - 2 * i), 0)
        omap = lambda p, i: (nt - 1 - i * p, 0)
    nj = c4 // LANES
    once = pl.Buffered(1)
    return pl.pallas_call(
        kern,
        grid=(len(phases), nt),
        in_specs=[
            pl.BlockSpec((tm, c), xmap, pipeline_mode=pl.Buffered(xbuf)),
            pl.BlockSpec((1, c), const),
            pl.BlockSpec((c, c4), const, pipeline_mode=once),
            pl.BlockSpec((c4, c), const, pipeline_mode=once),
            pl.BlockSpec((1, c4), const),
            pl.BlockSpec((1, c4), const),
        ],
        out_specs=[
            pl.BlockSpec((tm, c), omap, pipeline_mode=pl.Buffered(obuf)),
            pl.BlockSpec(memory_space=pl.ANY),
        ],
        out_shape=[
            jax.ShapeDtypeStruct((n, c), BF16),
            jax.ShapeDtypeStruct((nt - npin - ring, nj, tm // 2, LANES), U32),
        ],
        scratch_shapes=[
            pltpu.VMEM((ring + npin, nj, tm // 2, LANES), U32),
            pltpu.VMEM((nj, 8, LANES), F32),
            pltpu.VMEM((9 * nj // 2, LANES // 2, LANES) if st0 else (nj, c // 2, LANES), U32),
            pltpu.VMEM((15, c4 // 6, LANES) if st1 == 2 else (9, c4 // 4, LANES) if st1 else (c // LANES, c4 // 2, LANES), U32),
            pltpu.VMEM((8, c), F32),
            pltpu.SemaphoreType.DMA((ring,)),
        ],
        compiler_params=pltpu.CompilerParams(
            dimension_semantics=("arbitrary", "arbitrary"),
            vmem_limit_bytes=vmem_mb * 1024 * 1024,
        ),
    )


def _run(x, dw, w1, w2, grn_g, grn_b, **kw):
    b, hh, ww, c = x.shape
    c4 = w1.shape[1]
    n = b * hh * ww
    assert b == 1 and dw.shape[0] == 1 and dw.shape[1] == 1
    out, _ = _build(n, c, c4, **kw)(
        x.reshape(n, c), dw.reshape(1, c), w1, w2,
        grn_g.reshape(1, c4), grn_b.reshape(1, c4))
    return out.reshape(x.shape)


@jax.jit
def pallas_standalone__modern_conv_block_slak__vision_kernel(
    x: jax.Array,
    dw: jax.Array,
    w1: jax.Array,
    w2: jax.Array,
    grn_g: jax.Array,
    grn_b: jax.Array,
):
    return _run(x, dw, w1, w2, grn_g, grn_b)
```

```python
import functools
import math

import jax
import jax.numpy as jnp
import jax.experimental.pallas as pl
import jax.experimental.pallas.tpu as pltpu

F32 = jnp.float32
BF16 = jnp.bfloat16
U32 = jnp.uint32
LANES = 128

_GELU_C0 = 0.7978845608028654
_GELU_C1 = 0.7978845608028654 * 0.044715
_LAM = _GELU_C1 ** (1.0 / 3.0)
_KAP = _GELU_C0 / _LAM
_HSCALE = 1.0 / (2.0 * _LAM)
_LOG2E = 1.4426950408889634
_RS_C = math.log2(_LAM) + 0.5 * math.log2(384.0)


_HK_U = ((0, 0, 0, 1, -1, 0), (-1, 0, 0, 0, 0, 1), (1, 0, 0, -1, 0, 0), (-1, 0, 0, 0, 0, 0),
         (0, 0, -1, 0, 0, 1), (1, 0, 0, -1, 1, 0), (0, -1, 0, 0, 0, 0), (0, -1, 1, 0, 0, -1),
         (0, 1, -1, 0, 0, 0), (1, 0, -1, 0, 0, 0), (0, 0, 0, 0, -1, 0), (0, 0, 0, -1, 0, 1),
         (0, 1, -1, 0, -1, 1), (-1, 1, 0, 1, -1, 0), (0, 0, 0, 0, 0, 1))
_HK_V = ((0, 0, 1, 0, 0, 0, 0, 0, 0), (0, -1, 0, 0, 0, 0, 1, 0, 0), (1, 1, 0, 1, 0, 0, 0, 0, 0),
         (1, 0, -1, 0, 0, 0, 1, 0, 0), (0, 0, 0, 0, 1, 0, 1, 1, 0), (0, 0, 1, 1, 0, 0, 0, 0, 0),
         (0, 0, 0, -1, 0, 1, 0, 0, 1), (0, 0, 0, 0, -1, 0, 0, 0, -1), (0, 0, 0, 0, 0, 0, 0, 0, 1),
         (0, 0, 0, 0, 0, 0, 1, 0, 0), (0, 0, 1, 0, -1, 1, 0, 0, 0), (0, -1, 0, 0, 0, 0, 0, 0, 0),
         (0, 0, 0, 0, -1, 0, 0, 0, 0), (0, 0, 0, 1, 0, 0, 0, 0, 0), (0, -1, 0, 0, 0, 0, 0, -1, 1))
_HK_W = ((1, 0, 1, 1, 0, 1), (0, 1, 0, 1, 0, 0), (0, 0, 0, -1, 0, 0), (-1, 0, 0, -1, 0, 0),
         (0, -1, 0, 0, 0, 0), (1, 0, 1, 1, 0, 0), (0, 0, -1, 0, 0, 0), (0, 1, 0, 0, 1, 1),
         (0, -1, -1, 0, -1, -1), (-1, 1, 0, 0, 0, 0), (0, 0, 0, 0, 0, -1), (0, 0, 0, -1, 1, 0),
         (0, 0, 0, 0, 1, 1), (1, 0, 1, 0, 0, 0), (0, -1, 0, 0, -1, 0))


def _combos(rows, vals):
    vals = list(vals)
    rows = [{i: c for i, c in enumerate(r) if c} for r in rows]
    while True:
        cnt = {}
        for r in rows:
            ks = sorted(r)
            for ia, a in enumerate(ks):
                for b in ks[ia + 1:]:
                    key = (a, b, r[a] * r[b])
                    cnt[key] = cnt.get(key, 0) + 1
        if not cnt or max(cnt.values()) < 2:
            break
        a, b, sg = max(sorted(cnt), key=lambda k_: cnt[k_])
        vals.append(_lazy(lambda a=a, b=b, sg=sg: (
            _force(vals[a]) + _force(vals[b]) if sg > 0 else _force(vals[a]) - _force(vals[b]))))
        new = len(vals) - 1
        for r in rows:
            if a in r and b in r and r[a] * r[b] == sg:
                r[new] = r.pop(a)
                del r[b]
    out = []
    for r in rows:
        items = sorted(r.items(), key=lambda kv: -kv[1])
        sign = items[0][1]
        acc = _force(vals[items[0][0]])
        for idx, cf in items[1:]:
            acc = acc + _force(vals[idx]) if cf * sign > 0 else acc - _force(vals[idx])
        out.append((acc, sign))
    return out


class _lazy:
    def __init__(self, fn):
        self.fn, self.val = fn, None


def _force(v):
    if isinstance(v, _lazy):
        if v.val is None:
            v.val = v.fn()
        return v.val
    return v


_HK_USIGN = tuple(sg for _, sg in _combos(_HK_U, [1.0] * 6))


def _col(row, n):
    return jnp.transpose(jnp.broadcast_to(row, (LANES, n)))


def _pack(v):
    return pltpu.bitcast(v, U32)


def _unpack(v):
    return pltpu.bitcast(v, BF16)


_ORDER = ('klt m4 -m5 m1 m7', 'krt m3 m5', 'm4 klb m2', 'm1 m3 m6 -m2 krb')


def _kernel(x_hbm, dw_ref, w1_hbm, w2_hbm, g_ref, b_ref,
            o_hbm, h_hbm,
            hs, xb, sb0, ssq_ref, w1s_ref, w2s_ref, bias_ref, w1_ref, w2_ref,
            sem_h, sem_x, sem_o, sem_w,
            *, st, nu0, nu1, ns, c, c4, cn, ring, npin, xr, xd, rbs, rbs1, phases, nodma,
            lnpre, lnm, rsq, order, gform, kkcat, corder, lag, lnpos):
    nj = c4 // LANES
    njh = nj // 2
    njk = nj // 3
    nk = c // LANES
    nspill = ns - npin - ring
    dot = functools.partial(jnp.dot, preferred_element_type=F32)

    def tile_info(t):
        lo = (t * npin) // ns
        hi = ((t + 1) * npin) // ns
        unpinned = hi == lo
        u = t - lo
        slot = jnp.where(unpinned, u % ring, ring + lo)
        return unpinned, u, slot

    def h_out_copy(u):
        return pltpu.make_async_copy(hs.at[u % ring], h_hbm.at[u], sem_h.at[u % ring])

    def h_in_copy(u):
        return pltpu.make_async_copy(h_hbm.at[u], hs.at[u % ring], sem_h.at[u % ring])

    def x_copy(t, slot):
        return pltpu.make_async_copy(x_hbm.at[pl.ds(t * st, st), :], xb.at[slot], sem_x.at[slot])

    def o_copy(t, slot):
        return pltpu.make_async_copy(xb.at[slot], o_hbm.at[pl.ds(t * st, st), :], sem_o.at[slot])

    w1_copy = pltpu.make_async_copy(w1_hbm, w1_ref, sem_w.at[0])
    w2_copy = pltpu.make_async_copy(w2_hbm, w2_ref, sem_w.at[1])

    hh = rbs // 2

    def strassen_lhs(xslot, rb):
        dw = dw_ref[...].astype(F32)

        def scale(ss):
            if rsq == 0:
                return _LAM * jax.lax.rsqrt(ss * (1.0 / c) + 1e-5)
            return jnp.exp2(jnp.log(ss + c * 1e-5) * (-0.5 * _LOG2E) + _RS_C)

        def layernorm(xf):
            y = xf * dw
            if lnm == 0:
                yc = y - jnp.sum(y, axis=-1, keepdims=True) * (1.0 / c)
                return yc * scale(jnp.sum(yc * yc, axis=-1, keepdims=True))
            s1 = jnp.sum(y, axis=-1, keepdims=True)
            s2 = jnp.sum(y * y, axis=-1, keepdims=True)
            m = s1 * (1.0 / c)
            return (y - m) * scale(jnp.maximum(s2 - s1 * m, 0.0))

        xu = _pack(xb[xslot, rb * rbs:(rb + 1) * rbs, :])
        a1, a2 = [layernorm(pltpu.unpack_elementwise(
            xu, index=k, packed_dtype=BF16, unpacked_dtype=F32)) for k in range(2)]
        a11, a12, a13 = (a1[:, k * LANES:(k + 1) * LANES] for k in range(3))
        a21, a22, a23 = (a2[:, k * LANES:(k + 1) * LANES] for k in range(3))
        return [a11 + a22, a21 + a22, a11, a22, a11 + a12, a21 - a11, a12 - a22, a13, a23]

    def lhs_to_scratch(xslot):
        for q, t in enumerate(strassen_lhs(xslot, 0)):
            sb0[q] = _pack(t.astype(BF16))

    look = 1 if lnpre else 0
    w1_copy.start()
    if 0 in phases:
        for k in range(nu0 + look):
            x_copy(k, k).start()
    w2_copy.start()
    w1_copy.wait()
    ssq_ref[...] = jnp.zeros_like(ssq_ref)
    for j in range(njh):
        cl = slice(j * LANES, (j + 1) * LANES)
        cr = slice((njh + j) * LANES, (njh + j + 1) * LANES)
        b11 = w1_ref[0:LANES, cl].astype(F32)
        b12 = w1_ref[0:LANES, cr].astype(F32)
        b21 = w1_ref[LANES:2 * LANES, cl].astype(F32)
        b22 = w1_ref[LANES:2 * LANES, cr].astype(F32)
        combos = [b11 + b22, b11, b12 - b22, b21 - b11, b22, b11 + b12, b21 + b22]
        for q, t in enumerate(combos):
            w1s_ref[q * njh + j] = _pack(t.astype(BF16))
        w1s_ref[7 * njh + j] = _pack(w1_ref[2 * LANES:3 * LANES, cl])
        w1s_ref[8 * njh + j] = _pack(w1_ref[2 * LANES:3 * LANES, cr])
    if 0 in phases and lnpre:
        x_copy(0, 0).wait()
        lhs_to_scratch(0)

    def gelu(b):
        t = jnp.tanh(b * (b * b + _KAP))
        return b * (1.0 + t) if gform == 0 else b + b * t

    def phase0_block(blk, carry):
        jb = cn // LANES
        t0 = blk * nu0
        for su in range(nu0):
            tn = t0 + nu0 + look + su

            @pl.when(tn < ns)
            def _():
                x_copy(tn, tn % xr).start()

        for su in range(nu0):
            tw = t0 + look + su

            @pl.when(tw < ns)
            def _():
                x_copy(tw, tw % xr).wait()

        infos = [tile_info(t0 + su) for su in range(nu0)]
        for unpinned, u, _ in infos:
            @pl.when(jnp.logical_and(unpinned, u >= ring))
            def _():
                h_out_copy(u - ring).wait()

        nrb = st // rbs
        nch = njh // jb
        rbl = [(su, rb) for su in range(nu0) for rb in range(nrb)]
        lhs_cache = {}

        def get_lhs(k):
            if k not in lhs_cache:
                su, rb = rbl[k]
                if lnpre and k == 0:
                    ops = [_unpack(sb0[q]) for q in range(9)]
                else:
                    ops = [t.astype(BF16) for t in strassen_lhs((t0 + su) % xr, rb)]
                lhs_cache[k] = ops
            return lhs_cache[k]

        done = {}

        def finish(k, jc, cb, pre):
            done[(k, jc, cb)] = gelu(pre)
            for top, bot, j0 in ((0, 2, jc * jb), (1, 3, njh + jc * jb)):
                if cb in (top, bot) and (k, jc, top) in done and (k, jc, bot) in done:
                    gt, gb = done.pop((k, jc, top)), done.pop((k, jc, bot))
                    su, rb = rbl[k]
                    sq = jnp.sum((gt * gt + gb * gb).reshape(hh // 8, 8, cn), axis=0)
                    hp = pltpu.pack_elementwise([gt, gb], packed_dtype=BF16)
                    for kq in range(jb):
                        ls = slice(kq * LANES, (kq + 1) * LANES)
                        ssq_ref[j0 + kq] += sq[:, ls]
                        hs[infos[su][2], j0 + kq, rb * hh:(rb + 1) * hh, :] = hp[:, ls]

        queue = []
        for k in range(len(rbl)):
            for jc in range(nch):
                if jc == lnpos and k + 1 < len(rbl):
                    get_lhs(k + 1)
                s1, s2, s3, s4, s5, s6, s7, k1, k2 = get_lhs(k)

                def wq(q):
                    ws = [_unpack(w1s_ref[q * njh + jc * jb + kq]) for kq in range(jb)]
                    return ws[0] if jb == 1 else jnp.concatenate(ws, axis=1)

                prods = {}

                def prod(name):
                    if name not in prods:
                        if name[0] == 'm':
                            q = int(name[1]) - 1
                            prods[name] = dot((s1, s2, s3, s4, s5, s6, s7)[q], wq(q))
                        elif kkcat:
                            r = dot(jnp.concatenate([k1, k2], axis=0), wq(7 if name[1] == 'l' else 8))
                            prods[name[:2] + 't'], prods[name[:2] + 'b'] = r[:hh], r[hh:]
                        else:
                            prods[name] = dot(k1 if name[2] == 't' else k2,
                                              wq(7 if name[1] == 'l' else 8))
                    return prods[name]

                for cb in corder:
                    acc = None
                    for tok in order[cb].split():
                        v = prod(tok.lstrip('-'))
                        acc = v if acc is None else (acc - v if tok[0] == '-' else acc + v)
                    queue.append((k, jc, cb, acc))
                    if len(queue) > lag:
                        finish(*queue.pop(0))
        while queue:
            finish(*queue.pop(0))

        if lnpre:
            lhs_to_scratch(jnp.minimum(t0 + nu0, ns - 1) % xr)

        for unpinned, u, _ in infos:
            @pl.when(jnp.logical_and(unpinned, u < nspill))
            def _():
                h_out_copy(u).start()
        return carry

    if 0 in phases:
        jax.lax.fori_loop(0, ns // nu0, phase0_block, 0)

    if 1 in phases:
        for k in range(xd):
            x_copy(ns - 1 - k, k).start()
    w2_copy.wait()
    ssq = jnp.concatenate(
        [jnp.sum(ssq_ref[j], axis=0, keepdims=True) for j in range(nj)], axis=1)
    ssq = ssq * (_HSCALE * _HSCALE)
    gx = jnp.sqrt(ssq + 1e-6)
    nx = gx / (jnp.mean(gx, axis=-1, keepdims=True) + 1e-6)
    s = (1.0 + g_ref[...].astype(F32) * nx) * _HSCALE
    s_t = _col(s, c4)
    kb = c4 // 3
    ws = [w2_ref[:, k * LANES:(k + 1) * LANES].astype(F32) * s_t for k in range(nk)]
    bl = [ws[l][j * kb:(j + 1) * kb] for j in range(3) for l in range(3)]
    for q, (t, sg) in enumerate(_combos(_HK_V, bl)):
        if sg * _HK_USIGN[q] < 0:
            t = -t
        w2s_ref[q] = _pack(t.astype(BF16))
    b8 = jnp.broadcast_to(b_ref[...], (16, c4))
    bias_ref[...] = dot(b8, w2_ref[...])[:8]

    def phase1_block(blk, carry):
        hh1 = rbs1 // 2
        bias = bias_ref[0:1, :]
        i0 = blk * nu1
        for su in range(nu1):
            inx = i0 + su + xd

            @pl.when(jnp.logical_and(inx < ns, inx >= xr))
            def _():
                o_copy(ns - 1 - (inx - xr), inx % xr).wait()

            @pl.when(inx < ns)
            def _():
                x_copy(ns - 1 - inx, inx % xr).start()

        if not nodma:
            for su in range(nu1):
                ip = i0 - nu1 + su
                unp_p, u_p, _ = tile_info(ns - 1 - jnp.maximum(ip, 0))

                @pl.when(jnp.logical_and(ip >= 0, jnp.logical_and(unp_p, u_p >= ring)))
                def _():
                    h_in_copy(u_p - ring).start()

        infos = [tile_info(ns - 1 - (i0 + su)) for su in range(nu1)]
        for su in range(nu1):
            x_copy(ns - 1 - (i0 + su), (i0 + su) % xr).wait()
            if not nodma:
                unpinned, u, _ = infos[su]

                @pl.when(jnp.logical_and(unpinned, u < nspill))
                def _():
                    h_in_copy(u).wait()

        for su in range(nu1):
            slot = infos[su][2]
            xslot = (i0 + su) % xr
            for rb in range(st // rbs1):
                r0 = rb * rbs1
                raw = [jnp.concatenate(
                    [_unpack(hs[slot, kk * njk + j,
                                (r0 + half * hh1) // 2:(r0 + (half + 1) * hh1) // 2, :])
                     for j in range(njk)], axis=1) for half in range(2) for kk in range(3)]
                flt = [_lazy(lambda a=a: a.astype(F32)) for a in raw]
                lhs = _combos(_HK_U, flt)
                ms = []
                for q, row in enumerate(_HK_U):
                    nzs = [ix for ix, cf in enumerate(row) if cf]
                    a = raw[nzs[0]] if len(nzs) == 1 else lhs[q][0].astype(BF16)
                    ms.append(dot(a, _unpack(w2s_ref[q])))
                cs = _combos([[w[o] for w in _HK_W] for o in range(6)], ms)
                for half in range(2):
                    rs = slice(r0 + half * hh1, r0 + (half + 1) * hh1)
                    for l in range(3):
                        cl = slice(l * LANES, (l + 1) * LANES)
                        val, sg = cs[half * 3 + l]
                        base = xb[xslot, rs, cl].astype(F32) + bias[:, cl]
                        xb[xslot, rs, cl] = (base + val if sg > 0 else base - val).astype(BF16)

        for su in range(nu1):
            o_copy(ns - 1 - (i0 + su), (i0 + su) % xr).start()
        return carry

    if 1 in phases:
        jax.lax.fori_loop(0, ns // nu1, phase1_block, 0)
        for i in range(ns - xr, ns):
            o_copy(ns - 1 - i, i % xr).wait()
    else:
        o_copy(0, 0).start()
        o_copy(0, 0).wait()


def _build(n, c, c4, st=1024, nu0=2, nu1=1, cn=128, ring=4, npin=33, xr=5, xd=2, vmem_mb=128,
           phases=(0, 1), rbs=128, rbs1=128, nodma=False, lnpre=True, lnm=0, rsq=1, order=_ORDER, gform=0, kkcat=True, corder=(2, 0, 3, 1), lag=0, lnpos=99):
    ns = n // st
    phases = tuple(phases)
    assert xr >= 2 * nu0 + (1 if lnpre else 0) and xr >= xd + 2 * nu1 and xd >= nu1
    kern = functools.partial(_kernel, st=st, nu0=nu0, nu1=nu1, ns=ns, c=c, c4=c4, cn=cn,
                             ring=ring, npin=npin, xr=xr, xd=xd, rbs=rbs, rbs1=rbs1,
                             phases=phases, nodma=nodma, lnpre=lnpre, lnm=lnm, rsq=rsq,
                             order=tuple(order), gform=gform, kkcat=kkcat,
                             corder=tuple(corder), lag=lag, lnpos=lnpos)
    nj = c4 // LANES
    hbm = pl.BlockSpec(memory_space=pl.ANY)
    vmem = pl.BlockSpec(memory_space=pltpu.VMEM)
    return pl.pallas_call(
        kern,
        in_specs=[hbm, vmem, hbm, hbm, vmem, vmem],
        out_specs=[hbm, hbm],
        out_shape=[
            jax.ShapeDtypeStruct((n, c), BF16),
            jax.ShapeDtypeStruct((ns - npin - ring, nj, st // 2, LANES), U32),
        ],
        scratch_shapes=[
            pltpu.VMEM((ring + npin, nj, st // 2, LANES), U32),
            pltpu.VMEM((xr, st, c), BF16),
            pltpu.VMEM((9, rbs // 4, LANES), U32),
            pltpu.VMEM((nj, 8, LANES), F32),
            pltpu.VMEM((9 * nj // 2, LANES // 2, LANES), U32),
            pltpu.VMEM((15, c4 // 6, LANES), U32),
            pltpu.VMEM((8, c), F32),
            pltpu.VMEM((c, c4), BF16),
            pltpu.VMEM((c4, c), BF16),
            pltpu.SemaphoreType.DMA((ring,)),
            pltpu.SemaphoreType.DMA((xr,)),
            pltpu.SemaphoreType.DMA((xr,)),
            pltpu.SemaphoreType.DMA((2,)),
        ],
        compiler_params=pltpu.CompilerParams(
            vmem_limit_bytes=vmem_mb * 1024 * 1024,
        ),
    )


def _run(x, dw, w1, w2, grn_g, grn_b, **kw):
    b, hh, ww, c = x.shape
    c4 = w1.shape[1]
    n = b * hh * ww
    assert b == 1 and dw.shape[0] == 1 and dw.shape[1] == 1
    out, _ = _build(n, c, c4, **kw)(
        x.reshape(n, c), dw.reshape(1, c), w1, w2,
        grn_g.reshape(1, c4), grn_b.reshape(1, c4))
    return out.reshape(x.shape)


@jax.jit
def pallas_standalone__modern_conv_block_slak__vision_kernel(
    x: jax.Array,
    dw: jax.Array,
    w1: jax.Array,
    w2: jax.Array,
    grn_g: jax.Array,
    grn_b: jax.Array,
):
    return _run(x, dw, w1, w2, grn_g, grn_b)
```

```python
import functools
import math

import jax
import jax.numpy as jnp
import jax.experimental.pallas as pl
import jax.experimental.pallas.tpu as pltpu

F32 = jnp.float32
BF16 = jnp.bfloat16
U32 = jnp.uint32
LANES = 128

_GELU_C0 = 0.7978845608028654
_GELU_C1 = 0.7978845608028654 * 0.044715
_LAM = _GELU_C1 ** (1.0 / 3.0)
_KAP = _GELU_C0 / _LAM
_HSCALE = 1.0 / (2.0 * _LAM)
_LOG2E = 1.4426950408889634
_RS_C = math.log2(_LAM) + 0.5 * math.log2(384.0)


_HK_U = ((0, 0, 0, 1, -1, 0), (-1, 0, 0, 0, 0, 1), (1, 0, 0, -1, 0, 0), (-1, 0, 0, 0, 0, 0),
         (0, 0, -1, 0, 0, 1), (1, 0, 0, -1, 1, 0), (0, -1, 0, 0, 0, 0), (0, -1, 1, 0, 0, -1),
         (0, 1, -1, 0, 0, 0), (1, 0, -1, 0, 0, 0), (0, 0, 0, 0, -1, 0), (0, 0, 0, -1, 0, 1),
         (0, 1, -1, 0, -1, 1), (-1, 1, 0, 1, -1, 0), (0, 0, 0, 0, 0, 1))
_HK_V = ((0, 0, 1, 0, 0, 0, 0, 0, 0), (0, -1, 0, 0, 0, 0, 1, 0, 0), (1, 1, 0, 1, 0, 0, 0, 0, 0),
         (1, 0, -1, 0, 0, 0, 1, 0, 0), (0, 0, 0, 0, 1, 0, 1, 1, 0), (0, 0, 1, 1, 0, 0, 0, 0, 0),
         (0, 0, 0, -1, 0, 1, 0, 0, 1), (0, 0, 0, 0, -1, 0, 0, 0, -1), (0, 0, 0, 0, 0, 0, 0, 0, 1),
         (0, 0, 0, 0, 0, 0, 1, 0, 0), (0, 0, 1, 0, -1, 1, 0, 0, 0), (0, -1, 0, 0, 0, 0, 0, 0, 0),
         (0, 0, 0, 0, -1, 0, 0, 0, 0), (0, 0, 0, 1, 0, 0, 0, 0, 0), (0, -1, 0, 0, 0, 0, 0, -1, 1))
_HK_W = ((1, 0, 1, 1, 0, 1), (0, 1, 0, 1, 0, 0), (0, 0, 0, -1, 0, 0), (-1, 0, 0, -1, 0, 0),
         (0, -1, 0, 0, 0, 0), (1, 0, 1, 1, 0, 0), (0, 0, -1, 0, 0, 0), (0, 1, 0, 0, 1, 1),
         (0, -1, -1, 0, -1, -1), (-1, 1, 0, 0, 0, 0), (0, 0, 0, 0, 0, -1), (0, 0, 0, -1, 1, 0),
         (0, 0, 0, 0, 1, 1), (1, 0, 1, 0, 0, 0), (0, -1, 0, 0, -1, 0))


def _combos(rows, vals):
    vals = list(vals)
    rows = [{i: c for i, c in enumerate(r) if c} for r in rows]
    while True:
        cnt = {}
        for r in rows:
            ks = sorted(r)
            for ia, a in enumerate(ks):
                for b in ks[ia + 1:]:
                    key = (a, b, r[a] * r[b])
                    cnt[key] = cnt.get(key, 0) + 1
        if not cnt or max(cnt.values()) < 2:
            break
        a, b, sg = max(sorted(cnt), key=lambda k_: cnt[k_])
        vals.append(_lazy(lambda a=a, b=b, sg=sg: (
            _force(vals[a]) + _force(vals[b]) if sg > 0 else _force(vals[a]) - _force(vals[b]))))
        new = len(vals) - 1
        for r in rows:
            if a in r and b in r and r[a] * r[b] == sg:
                r[new] = r.pop(a)
                del r[b]
    out = []
    for r in rows:
        items = sorted(r.items(), key=lambda kv: -kv[1])
        sign = items[0][1]
        acc = _force(vals[items[0][0]])
        for idx, cf in items[1:]:
            acc = acc + _force(vals[idx]) if cf * sign > 0 else acc - _force(vals[idx])
        out.append((acc, sign))
    return out


class _lazy:
    def __init__(self, fn):
        self.fn, self.val = fn, None


def _force(v):
    if isinstance(v, _lazy):
        if v.val is None:
            v.val = v.fn()
        return v.val
    return v


_HK_USIGN = tuple(sg for _, sg in _combos(_HK_U, [1.0] * 6))


def _col(row, n):
    return jnp.transpose(jnp.broadcast_to(row, (LANES, n)))


def _pack(v):
    return pltpu.bitcast(v, U32)


def _unpack(v):
    return pltpu.bitcast(v, BF16)


_ORDER = ('klt m4 -m5 m1 m7', 'krt m3 m5', 'm4 klb m2', 'm1 m3 m6 -m2 krb')


def _kernel(x_hbm, dw_ref, w1_hbm, w2_hbm, g_ref, b_ref,
            o_hbm, h_hbm,
            hs, xb, sb0, ssq_ref, w1s_ref, w2s_ref, bias_ref, w1_ref, w2_ref,
            sem_h, sem_x, sem_o, sem_w,
            *, st, nu0, nu1, ns, c, c4, cn, ring, npin, xr, xd, rbs, rbs1, phases, nodma,
            lnpre, lnm, rsq, order, gform, kkcat, corder, lag, lnpos):
    nj = c4 // LANES
    njh = nj // 2
    njk = nj // 3
    nk = c // LANES
    nspill = ns - npin - ring
    dot = functools.partial(jnp.dot, preferred_element_type=F32)

    def unit_info(t, acc, lo):
        unpinned = acc + npin < ns
        u = t - lo
        slot = jnp.where(unpinned, wrap_ring(u), ring + lo)
        return unpinned, u, slot

    def wrap_ring(u):
        return u & (ring - 1)

    def step_up(acc, lo):
        acc = acc + npin
        wrap = acc >= ns
        return jnp.where(wrap, acc - ns, acc), jnp.where(wrap, lo + 1, lo)

    def step_down(acc, lo):
        acc = acc - npin
        wrap = acc < 0
        return jnp.where(wrap, acc + ns, acc), jnp.where(wrap, lo - 1, lo)

    def xwrap(v):
        return jnp.where(v >= xr, v - xr, v)

    def h_out_copy(u):
        return pltpu.make_async_copy(hs.at[wrap_ring(u)], h_hbm.at[u], sem_h.at[wrap_ring(u)])

    def h_in_copy(u):
        return pltpu.make_async_copy(h_hbm.at[u], hs.at[wrap_ring(u)], sem_h.at[wrap_ring(u)])

    def x_copy(t, slot):
        return pltpu.make_async_copy(x_hbm.at[pl.ds(t * st, st), :], xb.at[slot], sem_x.at[slot])

    def o_copy(t, slot):
        return pltpu.make_async_copy(xb.at[slot], o_hbm.at[pl.ds(t * st, st), :], sem_o.at[slot])

    w1_copy = pltpu.make_async_copy(w1_hbm, w1_ref, sem_w.at[0])
    w2_copy = pltpu.make_async_copy(w2_hbm, w2_ref, sem_w.at[1])

    hh = rbs // 2

    def strassen_lhs(xslot, rb):
        dw = dw_ref[...].astype(F32)

        def scale(ss):
            if rsq == 0:
                return _LAM * jax.lax.rsqrt(ss * (1.0 / c) + 1e-5)
            return jnp.exp2(jnp.log(ss + c * 1e-5) * (-0.5 * _LOG2E) + _RS_C)

        def layernorm(xf):
            y = xf * dw
            if lnm == 0:
                yc = y - jnp.sum(y, axis=-1, keepdims=True) * (1.0 / c)
                return yc * scale(jnp.sum(yc * yc, axis=-1, keepdims=True))
            s1 = jnp.sum(y, axis=-1, keepdims=True)
            s2 = jnp.sum(y * y, axis=-1, keepdims=True)
            m = s1 * (1.0 / c)
            return (y - m) * scale(jnp.maximum(s2 - s1 * m, 0.0))

        xu = _pack(xb[xslot, rb * rbs:(rb + 1) * rbs, :])
        a1, a2 = [layernorm(pltpu.unpack_elementwise(
            xu, index=k, packed_dtype=BF16, unpacked_dtype=F32)) for k in range(2)]
        a11, a12, a13 = (a1[:, k * LANES:(k + 1) * LANES] for k in range(3))
        a21, a22, a23 = (a2[:, k * LANES:(k + 1) * LANES] for k in range(3))
        return [a11 + a22, a21 + a22, a11, a22, a11 + a12, a21 - a11, a12 - a22, a13, a23]

    def lhs_to_scratch(xslot):
        for q, t in enumerate(strassen_lhs(xslot, 0)):
            sb0[q] = _pack(t.astype(BF16))

    look = 1 if lnpre else 0
    w1_copy.start()
    if 0 in phases:
        for k in range(nu0 + look):
            x_copy(k, k).start()
    w2_copy.start()
    w1_copy.wait()
    ssq_ref[...] = jnp.zeros_like(ssq_ref)
    for j in range(njh):
        cl = slice(j * LANES, (j + 1) * LANES)
        cr = slice((njh + j) * LANES, (njh + j + 1) * LANES)
        b11 = w1_ref[0:LANES, cl].astype(F32)
        b12 = w1_ref[0:LANES, cr].astype(F32)
        b21 = w1_ref[LANES:2 * LANES, cl].astype(F32)
        b22 = w1_ref[LANES:2 * LANES, cr].astype(F32)
        combos = [b11 + b22, b11, b12 - b22, b21 - b11, b22, b11 + b12, b21 + b22]
        for q, t in enumerate(combos):
            w1s_ref[q * njh + j] = _pack(t.astype(BF16))
        w1s_ref[7 * njh + j] = _pack(w1_ref[2 * LANES:3 * LANES, cl])
        w1s_ref[8 * njh + j] = _pack(w1_ref[2 * LANES:3 * LANES, cr])
    if 0 in phases and lnpre:
        x_copy(0, 0).wait()
        lhs_to_scratch(0)

    def gelu(b):
        t = jnp.tanh(b * (b * b + _KAP))
        return b * (1.0 + t) if gform == 0 else b + b * t

    def phase0_state(t0, acc, lo):
        infos = []
        for su in range(nu0):
            infos.append(unit_info(t0 + su, acc, lo))
            acc, lo = step_up(acc, lo)
        return tuple(infos), acc, lo

    def phase0_block(blk, carry):
        infos, bacc, blo, xs0 = carry
        jb = cn // LANES
        t0 = blk * nu0
        xslots = [xs0]
        for _ in range(2 * nu0 + look - 1):
            xslots.append(xwrap(xslots[-1] + 1))
        for su in range(nu0):
            tn = t0 + nu0 + look + su

            @pl.when(tn < ns)
            def _():
                x_copy(tn, xslots[nu0 + look + su]).start()

        for su in range(nu0):
            tw = t0 + look + su

            @pl.when(tw < ns)
            def _():
                x_copy(tw, xslots[look + su]).wait()

        for unpinned, u, _ in infos:
            @pl.when(jnp.logical_and(unpinned, u >= ring))
            def _():
                h_out_copy(u - ring).wait()

        nrb = st // rbs
        nch = njh // jb
        rbl = [(su, rb) for su in range(nu0) for rb in range(nrb)]
        lhs_cache = {}

        def get_lhs(k):
            if k not in lhs_cache:
                su, rb = rbl[k]
                if lnpre and k == 0:
                    ops = [_unpack(sb0[q]) for q in range(9)]
                else:
                    ops = [t.astype(BF16) for t in strassen_lhs(xslots[su], rb)]
                lhs_cache[k] = ops
            return lhs_cache[k]

        done = {}

        def finish(k, jc, cb, pre):
            done[(k, jc, cb)] = gelu(pre)
            for top, bot, j0 in ((0, 2, jc * jb), (1, 3, njh + jc * jb)):
                if cb in (top, bot) and (k, jc, top) in done and (k, jc, bot) in done:
                    gt, gb = done.pop((k, jc, top)), done.pop((k, jc, bot))
                    su, rb = rbl[k]
                    sq = jnp.sum((gt * gt + gb * gb).reshape(hh // 8, 8, cn), axis=0)
                    hp = pltpu.pack_elementwise([gt, gb], packed_dtype=BF16)
                    for kq in range(jb):
                        ls = slice(kq * LANES, (kq + 1) * LANES)
                        ssq_ref[j0 + kq] += sq[:, ls]
                        hs[infos[su][2], j0 + kq, rb * hh:(rb + 1) * hh, :] = hp[:, ls]

        queue = []
        for k in range(len(rbl)):
            for jc in range(nch):
                if jc == lnpos and k + 1 < len(rbl):
                    get_lhs(k + 1)
                s1, s2, s3, s4, s5, s6, s7, k1, k2 = get_lhs(k)

                def wq(q):
                    ws = [_unpack(w1s_ref[q * njh + jc * jb + kq]) for kq in range(jb)]
                    return ws[0] if jb == 1 else jnp.concatenate(ws, axis=1)

                prods = {}

                def prod(name):
                    if name not in prods:
                        if name[0] == 'm':
                            q = int(name[1]) - 1
                            prods[name] = dot((s1, s2, s3, s4, s5, s6, s7)[q], wq(q))
                        elif kkcat:
                            r = dot(jnp.concatenate([k1, k2], axis=0), wq(7 if name[1] == 'l' else 8))
                            prods[name[:2] + 't'], prods[name[:2] + 'b'] = r[:hh], r[hh:]
                        else:
                            prods[name] = dot(k1 if name[2] == 't' else k2,
                                              wq(7 if name[1] == 'l' else 8))
                    return prods[name]

                for cb in corder:
                    acc = None
                    for tok in order[cb].split():
                        v = prod(tok.lstrip('-'))
                        acc = v if acc is None else (acc - v if tok[0] == '-' else acc + v)
                    queue.append((k, jc, cb, acc))
                    if len(queue) > lag:
                        finish(*queue.pop(0))
        while queue:
            finish(*queue.pop(0))

        if lnpre:
            lhs_to_scratch(xslots[nu0])

        for unpinned, u, _ in infos:
            @pl.when(jnp.logical_and(unpinned, u < nspill))
            def _():
                h_out_copy(u).start()
        infos, bacc, blo = phase0_state(t0 + nu0, bacc, blo)
        return infos, bacc, blo, xslots[nu0]

    if 0 in phases:
        zero = jnp.int32(0)
        jax.lax.fori_loop(0, ns // nu0, phase0_block, (*phase0_state(zero, zero, zero), zero))

    if 1 in phases:
        for k in range(xd):
            x_copy(ns - 1 - k, k).start()
    w2_copy.wait()
    ssq = jnp.concatenate(
        [jnp.sum(ssq_ref[j], axis=0, keepdims=True) for j in range(nj)], axis=1)
    ssq = ssq * (_HSCALE * _HSCALE)
    gx = jnp.sqrt(ssq + 1e-6)
    nx = gx / (jnp.mean(gx, axis=-1, keepdims=True) + 1e-6)
    s = (1.0 + g_ref[...].astype(F32) * nx) * _HSCALE
    s_t = _col(s, c4)
    kb = c4 // 3
    ws = [w2_ref[:, k * LANES:(k + 1) * LANES].astype(F32) * s_t for k in range(nk)]
    bl = [ws[l][j * kb:(j + 1) * kb] for j in range(3) for l in range(3)]
    for q, (t, sg) in enumerate(_combos(_HK_V, bl)):
        if sg * _HK_USIGN[q] < 0:
            t = -t
        w2s_ref[q] = _pack(t.astype(BF16))
    b8 = jnp.broadcast_to(b_ref[...], (16, c4))
    bias_ref[...] = dot(b8, w2_ref[...])[:8]

    def phase1_state(i0, acc, lo):
        infos = []
        for su in range(nu1):
            infos.append(unit_info(ns - 1 - (i0 + su), acc, lo))
            acc, lo = step_down(acc, lo)
        return tuple(infos), acc, lo

    def phase1_block(blk, carry):
        prev, infos, bacc, blo, xs0 = carry
        hh1 = rbs1 // 2
        bias = bias_ref[0:1, :]
        i0 = blk * nu1
        xslots = [xs0]
        for _ in range(xd + nu1 - 1):
            xslots.append(xwrap(xslots[-1] + 1))
        for su in range(nu1):
            inx = i0 + su + xd

            @pl.when(jnp.logical_and(inx < ns, inx >= xr))
            def _():
                o_copy(ns - 1 - (inx - xr), xslots[su + xd]).wait()

            @pl.when(inx < ns)
            def _():
                x_copy(ns - 1 - inx, xslots[su + xd]).start()

        if not nodma:
            for unp_p, u_p, _ in prev:
                @pl.when(jnp.logical_and(unp_p, u_p >= ring))
                def _():
                    h_in_copy(u_p - ring).start()

        for su in range(nu1):
            x_copy(ns - 1 - (i0 + su), xslots[su]).wait()
            if not nodma:
                unpinned, u, _ = infos[su]

                @pl.when(jnp.logical_and(unpinned, u < nspill))
                def _():
                    h_in_copy(u).wait()

        for su in range(nu1):
            slot = infos[su][2]
            xslot = xslots[su]
            for rb in range(st // rbs1):
                r0 = rb * rbs1
                raw = [jnp.concatenate(
                    [_unpack(hs[slot, kk * njk + j,
                                (r0 + half * hh1) // 2:(r0 + (half + 1) * hh1) // 2, :])
                     for j in range(njk)], axis=1) for half in range(2) for kk in range(3)]
                flt = [_lazy(lambda a=a: a.astype(F32)) for a in raw]
                lhs = _combos(_HK_U, flt)
                ms = []
                for q, row in enumerate(_HK_U):
                    nzs = [ix for ix, cf in enumerate(row) if cf]
                    a = raw[nzs[0]] if len(nzs) == 1 else lhs[q][0].astype(BF16)
                    ms.append(dot(a, _unpack(w2s_ref[q])))
                cs = _combos([[w[o] for w in _HK_W] for o in range(6)], ms)
                for half in range(2):
                    rs = slice(r0 + half * hh1, r0 + (half + 1) * hh1)
                    for l in range(3):
                        cl = slice(l * LANES, (l + 1) * LANES)
                        val, sg = cs[half * 3 + l]
                        base = xb[xslot, rs, cl].astype(F32) + bias[:, cl]
                        xb[xslot, rs, cl] = (base + val if sg > 0 else base - val).astype(BF16)

        for su in range(nu1):
            o_copy(ns - 1 - (i0 + su), xslots[su]).start()
        nxt, bacc, blo = phase1_state(i0 + nu1, bacc, blo)
        return infos, nxt, bacc, blo, xslots[nu1]

    if 1 in phases:
        acc0, lo0 = jnp.int32(((ns - 1) * npin) % ns), jnp.int32(((ns - 1) * npin) // ns)
        first, acc0, lo0 = phase1_state(jnp.int32(0), acc0, lo0)
        none = tuple((jnp.bool_(False), jnp.int32(0), jnp.int32(0)) for _ in range(nu1))
        jax.lax.fori_loop(0, ns // nu1, phase1_block, (none, first, acc0, lo0, jnp.int32(0)))
        for i in range(ns - xr, ns):
            o_copy(ns - 1 - i, i % xr).wait()
    else:
        o_copy(0, 0).start()
        o_copy(0, 0).wait()


def _build(n, c, c4, st=1024, nu0=2, nu1=1, cn=128, ring=4, npin=34, xr=5, xd=2, vmem_mb=128,
           phases=(0, 1), rbs=128, rbs1=256, nodma=False, lnpre=True, lnm=0, rsq=1, order=_ORDER, gform=0, kkcat=True, corder=(2, 0, 3, 1), lag=0, lnpos=99,
           nobc=True):
    ns = n // st
    phases = tuple(phases)
    assert ring & (ring - 1) == 0 and xd + nu1 <= xr
    assert xr >= 2 * nu0 + (1 if lnpre else 0) and xr >= xd + 2 * nu1 and xd >= nu1
    kern = functools.partial(_kernel, st=st, nu0=nu0, nu1=nu1, ns=ns, c=c, c4=c4, cn=cn,
                             ring=ring, npin=npin, xr=xr, xd=xd, rbs=rbs, rbs1=rbs1,
                             phases=phases, nodma=nodma, lnpre=lnpre, lnm=lnm, rsq=rsq,
                             order=tuple(order), gform=gform, kkcat=kkcat,
                             corder=tuple(corder), lag=lag, lnpos=lnpos)
    nj = c4 // LANES
    hbm = pl.BlockSpec(memory_space=pl.ANY)
    vmem = pl.BlockSpec(memory_space=pltpu.VMEM)
    return pl.pallas_call(
        kern,
        in_specs=[hbm, vmem, hbm, hbm, vmem, vmem],
        out_specs=[hbm, hbm],
        out_shape=[
            jax.ShapeDtypeStruct((n, c), BF16),
            jax.ShapeDtypeStruct((ns - npin - ring, nj, st // 2, LANES), U32),
        ],
        scratch_shapes=[
            pltpu.VMEM((ring + npin, nj, st // 2, LANES), U32),
            pltpu.VMEM((xr, st, c), BF16),
            pltpu.VMEM((9, rbs // 4, LANES), U32),
            pltpu.VMEM((nj, 8, LANES), F32),
            pltpu.VMEM((9 * nj // 2, LANES // 2, LANES), U32),
            pltpu.VMEM((15, c4 // 6, LANES), U32),
            pltpu.VMEM((8, c), F32),
            pltpu.VMEM((c, c4), BF16),
            pltpu.VMEM((c4, c), BF16),
            pltpu.SemaphoreType.DMA((ring,)),
            pltpu.SemaphoreType.DMA((xr,)),
            pltpu.SemaphoreType.DMA((xr,)),
            pltpu.SemaphoreType.DMA((2,)),
        ],
        compiler_params=pltpu.CompilerParams(
            vmem_limit_bytes=vmem_mb * 1024 * 1024,
            disable_bounds_checks=nobc,
        ),
    )


def _run(x, dw, w1, w2, grn_g, grn_b, **kw):
    b, hh, ww, c = x.shape
    c4 = w1.shape[1]
    n = b * hh * ww
    assert b == 1 and dw.shape[0] == 1 and dw.shape[1] == 1
    out, _ = _build(n, c, c4, **kw)(
        x.reshape(n, c), dw.reshape(1, c), w1, w2,
        grn_g.reshape(1, c4), grn_b.reshape(1, c4))
    return out.reshape(x.shape)


@jax.jit
def pallas_standalone__modern_conv_block_slak__vision_kernel(
    x: jax.Array,
    dw: jax.Array,
    w1: jax.Array,
    w2: jax.Array,
    grn_g: jax.Array,
    grn_b: jax.Array,
):
    return _run(x, dw, w1, w2, grn_g, grn_b)
```

```python
import functools
import math

import jax
import jax.numpy as jnp
import jax.experimental.pallas as pl
import jax.experimental.pallas.tpu as pltpu

F32 = jnp.float32
BF16 = jnp.bfloat16
U32 = jnp.uint32
LANES = 128

_GELU_C0 = 0.7978845608028654
_GELU_C1 = 0.7978845608028654 * 0.044715
_LAM = _GELU_C1 ** (1.0 / 3.0)
_KAP = _GELU_C0 / _LAM
_HSCALE = 1.0 / (2.0 * _LAM)
_LOG2E = 1.4426950408889634
_RS_C = math.log2(_LAM) + 0.5 * math.log2(384.0)


_HK_U = ((0, 0, 0, 1, -1, 0), (-1, 0, 0, 0, 0, 1), (1, 0, 0, -1, 0, 0), (-1, 0, 0, 0, 0, 0),
         (0, 0, -1, 0, 0, 1), (1, 0, 0, -1, 1, 0), (0, -1, 0, 0, 0, 0), (0, -1, 1, 0, 0, -1),
         (0, 1, -1, 0, 0, 0), (1, 0, -1, 0, 0, 0), (0, 0, 0, 0, -1, 0), (0, 0, 0, -1, 0, 1),
         (0, 1, -1, 0, -1, 1), (-1, 1, 0, 1, -1, 0), (0, 0, 0, 0, 0, 1))
_HK_V = ((0, 0, 1, 0, 0, 0, 0, 0, 0), (0, -1, 0, 0, 0, 0, 1, 0, 0), (1, 1, 0, 1, 0, 0, 0, 0, 0),
         (1, 0, -1, 0, 0, 0, 1, 0, 0), (0, 0, 0, 0, 1, 0, 1, 1, 0), (0, 0, 1, 1, 0, 0, 0, 0, 0),
         (0, 0, 0, -1, 0, 1, 0, 0, 1), (0, 0, 0, 0, -1, 0, 0, 0, -1), (0, 0, 0, 0, 0, 0, 0, 0, 1),
         (0, 0, 0, 0, 0, 0, 1, 0, 0), (0, 0, 1, 0, -1, 1, 0, 0, 0), (0, -1, 0, 0, 0, 0, 0, 0, 0),
         (0, 0, 0, 0, -1, 0, 0, 0, 0), (0, 0, 0, 1, 0, 0, 0, 0, 0), (0, -1, 0, 0, 0, 0, 0, -1, 1))
_HK_W = ((1, 0, 1, 1, 0, 1), (0, 1, 0, 1, 0, 0), (0, 0, 0, -1, 0, 0), (-1, 0, 0, -1, 0, 0),
         (0, -1, 0, 0, 0, 0), (1, 0, 1, 1, 0, 0), (0, 0, -1, 0, 0, 0), (0, 1, 0, 0, 1, 1),
         (0, -1, -1, 0, -1, -1), (-1, 1, 0, 0, 0, 0), (0, 0, 0, 0, 0, -1), (0, 0, 0, -1, 1, 0),
         (0, 0, 0, 0, 1, 1), (1, 0, 1, 0, 0, 0), (0, -1, 0, 0, -1, 0))


def _combos(rows, vals, perm=None):
    vals = list(vals)
    rank = list(perm) if perm is not None else list(range(len(vals)))
    rows = [{i: c for i, c in enumerate(r) if c} for r in rows]
    while True:
        cnt = {}
        for r in rows:
            ks = sorted(r, key=lambda i: rank[i])
            for ia, a in enumerate(ks):
                for b in ks[ia + 1:]:
                    key = (a, b, r[a] * r[b])
                    cnt[key] = cnt.get(key, 0) + 1
        if not cnt or max(cnt.values()) < 2:
            break
        a, b, sg = max(sorted(cnt, key=lambda k_: (rank[k_[0]], rank[k_[1]], k_[2])),
                       key=lambda k_: cnt[k_])
        vals.append(_lazy(lambda a=a, b=b, sg=sg: (
            _force(vals[a]) + _force(vals[b]) if sg > 0 else _force(vals[a]) - _force(vals[b]))))
        rank.append(max(rank[a], rank[b]) + 0.5)
        new = len(vals) - 1
        for r in rows:
            if a in r and b in r and r[a] * r[b] == sg:
                r[new] = r.pop(a)
                del r[b]

    def total(items, sign):
        acc = _force(vals[items[0][0]])
        for idx, cf in items[1:]:
            acc = acc + _force(vals[idx]) if cf * sign > 0 else acc - _force(vals[idx])
        return acc

    out = []
    for r in rows:
        items = sorted(r.items(), key=lambda kv: rank[kv[0]])
        pos = [i for i, kv in enumerate(items) if kv[1] > 0]
        if pos and pos[0] > 0 and len(pos) < len(items):
            items.insert(0, items.pop(pos[0]))
        sign = items[0][1]
        out.append((_lazy(functools.partial(total, items, sign)), sign))
    return out


class _lazy:
    def __init__(self, fn):
        self.fn, self.val = fn, None


def _force(v):
    if isinstance(v, _lazy):
        if v.val is None:
            v.val = v.fn()
        return v.val
    return v


_HK_USIGN = tuple(sg for _, sg in _combos(_HK_U, [1.0] * 6))


def _col(row, n):
    return jnp.transpose(jnp.broadcast_to(row, (LANES, n)))


def _pack(v):
    return pltpu.bitcast(v, U32)


def _unpack(v):
    return pltpu.bitcast(v, BF16)


_ORDER = ('klt m4 -m5 m1 m7', 'krt m3 m5', 'm4 klb m2', 'm1 m3 m6 -m2 krb')


def _kernel(x_hbm, dw_ref, w1_hbm, w2_hbm, g_ref, b_ref,
            o_hbm, h_hbm,
            hs, xb, sb0, ssq_ref, w1s_ref, w2s_ref, bias_ref, w1_ref, w2_ref,
            sem_h, sem_x, sem_o, sem_w,
            *, st, nu0, nu1, ns, c, c4, cn, ring, npin, xr, xd, rbs, rbs1, phases, nodma,
            lnpre, lnm, rsq, order, gform, kkcat, corder, lag, lnpos, nocomp, hk0, perm0, corder0):
    nj = c4 // LANES
    njh = nj // 2
    njk = nj // 3
    nk = c // LANES
    nspill = ns - npin - ring
    dot = functools.partial(jnp.dot, preferred_element_type=F32)

    def unit_info(t, acc, lo):
        unpinned = acc + npin < ns
        u = t - lo
        slot = jnp.where(unpinned, wrap_ring(u), ring + lo)
        return unpinned, u, slot

    def wrap_ring(u):
        return u & (ring - 1)

    def step_up(acc, lo):
        acc = acc + npin
        wrap = acc >= ns
        return jnp.where(wrap, acc - ns, acc), jnp.where(wrap, lo + 1, lo)

    def step_down(acc, lo):
        acc = acc - npin
        wrap = acc < 0
        return jnp.where(wrap, acc + ns, acc), jnp.where(wrap, lo - 1, lo)

    def xwrap(v):
        return jnp.where(v >= xr, v - xr, v)

    def h_out_copy(u):
        return pltpu.make_async_copy(hs.at[wrap_ring(u)], h_hbm.at[u], sem_h.at[wrap_ring(u)])

    def h_in_copy(u):
        return pltpu.make_async_copy(h_hbm.at[u], hs.at[wrap_ring(u)], sem_h.at[wrap_ring(u)])

    def x_copy(t, slot):
        return pltpu.make_async_copy(x_hbm.at[pl.ds(t * st, st), :], xb.at[slot], sem_x.at[slot])

    def o_copy(t, slot):
        return pltpu.make_async_copy(xb.at[slot], o_hbm.at[pl.ds(t * st, st), :], sem_o.at[slot])

    w1_copy = pltpu.make_async_copy(w1_hbm, w1_ref, sem_w.at[0])
    w2_copy = pltpu.make_async_copy(w2_hbm, w2_ref, sem_w.at[1])

    hh = rbs // 2

    def strassen_lhs(xslot, rb):
        dw = dw_ref[...].astype(F32)

        def scale(ss):
            if rsq == 0:
                return _LAM * jax.lax.rsqrt(ss * (1.0 / c) + 1e-5)
            return jnp.exp2(jnp.log(ss + c * 1e-5) * (-0.5 * _LOG2E) + _RS_C)

        def layernorm(xf):
            y = xf * dw
            if lnm == 0:
                yc = y - jnp.sum(y, axis=-1, keepdims=True) * (1.0 / c)
                return yc * scale(jnp.sum(yc * yc, axis=-1, keepdims=True))
            s1 = jnp.sum(y, axis=-1, keepdims=True)
            s2 = jnp.sum(y * y, axis=-1, keepdims=True)
            m = s1 * (1.0 / c)
            return (y - m) * scale(jnp.maximum(s2 - s1 * m, 0.0))

        xu = _pack(xb[xslot, rb * rbs:(rb + 1) * rbs, :])
        a1, a2 = [layernorm(pltpu.unpack_elementwise(
            xu, index=k, packed_dtype=BF16, unpacked_dtype=F32)) for k in range(2)]
        a11, a12, a13 = (a1[:, k * LANES:(k + 1) * LANES] for k in range(3))
        a21, a22, a23 = (a2[:, k * LANES:(k + 1) * LANES] for k in range(3))
        if hk0:
            return [_force(v) for v, _ in _combos(_HK_U, [a11, a12, a13, a21, a22, a23])]
        return [a11 + a22, a21 + a22, a11, a22, a11 + a12, a21 - a11, a12 - a22, a13, a23]

    def lhs_to_scratch(xslot):
        for q, t in enumerate(strassen_lhs(xslot, 0)):
            sb0[q] = _pack(t.astype(BF16))

    look = 1 if lnpre else 0
    w1_copy.start()
    if 0 in phases:
        for k in range(nu0 + look):
            x_copy(k, k).start()
    w2_copy.start()
    w1_copy.wait()
    ssq_ref[...] = jnp.zeros_like(ssq_ref)
    if hk0:
        for j in range(njk):
            bl = [w1_ref[kb_ * LANES:(kb_ + 1) * LANES,
                         (l * njk + j) * LANES:(l * njk + j + 1) * LANES].astype(F32)
                  for kb_ in range(3) for l in range(3)]
            for q, (t, sg) in enumerate(_combos(_HK_V, bl)):
                t = _force(t)
                if sg * _HK_USIGN[q] < 0:
                    t = -t
                w1s_ref[q * njk + j] = _pack(t.astype(BF16))
    for j in range(0 if hk0 else njh):
        cl = slice(j * LANES, (j + 1) * LANES)
        cr = slice((njh + j) * LANES, (njh + j + 1) * LANES)
        b11 = w1_ref[0:LANES, cl].astype(F32)
        b12 = w1_ref[0:LANES, cr].astype(F32)
        b21 = w1_ref[LANES:2 * LANES, cl].astype(F32)
        b22 = w1_ref[LANES:2 * LANES, cr].astype(F32)
        combos = [b11 + b22, b11, b12 - b22, b21 - b11, b22, b11 + b12, b21 + b22]
        for q, t in enumerate(combos):
            w1s_ref[q * njh + j] = _pack(t.astype(BF16))
        w1s_ref[7 * njh + j] = _pack(w1_ref[2 * LANES:3 * LANES, cl])
        w1s_ref[8 * njh + j] = _pack(w1_ref[2 * LANES:3 * LANES, cr])
    if 0 in phases and lnpre:
        x_copy(0, 0).wait()
        lhs_to_scratch(0)

    def gelu(b):
        t = jnp.tanh(b * (b * b + _KAP))
        return b * (1.0 + t) if gform == 0 else b + b * t

    def phase0_state(t0, acc, lo):
        infos = []
        for su in range(nu0):
            infos.append(unit_info(t0 + su, acc, lo))
            acc, lo = step_up(acc, lo)
        return tuple(infos), acc, lo

    def phase0_block(blk, carry):
        infos, bacc, blo, xs0 = carry
        jb = cn // LANES
        t0 = blk * nu0
        xslots = [xs0]
        for _ in range(2 * nu0 + look - 1):
            xslots.append(xwrap(xslots[-1] + 1))
        for su in range(nu0):
            tn = t0 + nu0 + look + su

            @pl.when(tn < ns)
            def _():
                x_copy(tn, xslots[nu0 + look + su]).start()

        for su in range(nu0):
            tw = t0 + look + su

            @pl.when(tw < ns)
            def _():
                x_copy(tw, xslots[look + su]).wait()

        for unpinned, u, _ in infos:
            @pl.when(jnp.logical_and(unpinned, u >= ring))
            def _():
                h_out_copy(u - ring).wait()

        nrb = st // rbs
        nch = njh // jb
        rbl = [(su, rb) for su in range(nu0) for rb in range(nrb)]
        lhs_cache = {}

        def get_lhs(k):
            if k not in lhs_cache:
                su, rb = rbl[k]
                if lnpre and k == 0:
                    ops = [_unpack(sb0[q]) for q in range(15 if hk0 else 9)]
                else:
                    ops = [t.astype(BF16) for t in strassen_lhs(xslots[su], rb)]
                lhs_cache[k] = ops
            return lhs_cache[k]

        done = {}

        def finish(k, jc, cb, pre):
            done[(k, jc, cb)] = gelu(pre)
            for top, bot, j0 in ((0, 2, jc * jb), (1, 3, njh + jc * jb)):
                if cb in (top, bot) and (k, jc, top) in done and (k, jc, bot) in done:
                    gt, gb = done.pop((k, jc, top)), done.pop((k, jc, bot))
                    su, rb = rbl[k]
                    sq = jnp.sum((gt * gt + gb * gb).reshape(hh // 8, 8, cn), axis=0)
                    hp = pltpu.pack_elementwise([gt, gb], packed_dtype=BF16)
                    for kq in range(jb):
                        ls = slice(kq * LANES, (kq + 1) * LANES)
                        ssq_ref[j0 + kq] += sq[:, ls]
                        hs[infos[su][2], j0 + kq, rb * hh:(rb + 1) * hh, :] = hp[:, ls]

        def finish_hk(k, jc, o, pre, sg):
            done[(k, jc, o)] = gelu(pre if sg > 0 else -pre)
            l = o % 3
            if (k, jc, l) in done and (k, jc, l + 3) in done:
                gt, gb = done.pop((k, jc, l)), done.pop((k, jc, l + 3))
                su, rb = rbl[k]
                sq = jnp.sum((gt * gt + gb * gb).reshape(hh // 8, 8, LANES), axis=0)
                j0 = l * njk + jc
                ssq_ref[j0] += sq
                hs[infos[su][2], j0, rb * hh:(rb + 1) * hh, :] = pltpu.pack_elementwise(
                    [gt, gb], packed_dtype=BF16)

        for k in range(len(rbl) if hk0 else 0):
            for jc in range(njk):
                ops = get_lhs(k)
                ms = [_lazy(lambda q=q: dot(ops[q], _unpack(w1s_ref[q * njk + jc])))
                      for q in range(15)]
                cs = _combos([[w[o] for w in _HK_W] for o in range(6)], ms, perm0)
                for o in corder0:
                    finish_hk(k, jc, o, _force(cs[o][0]), cs[o][1])

        queue = []
        for k in range(0 if hk0 else len(rbl)):
            for jc in range(nch):
                if jc == lnpos and k + 1 < len(rbl):
                    get_lhs(k + 1)
                s1, s2, s3, s4, s5, s6, s7, k1, k2 = get_lhs(k)

                def wq(q):
                    ws = [_unpack(w1s_ref[q * njh + jc * jb + kq]) for kq in range(jb)]
                    return ws[0] if jb == 1 else jnp.concatenate(ws, axis=1)

                prods = {}

                def prod(name):
                    if name not in prods:
                        if name[0] == 'm':
                            q = int(name[1]) - 1
                            prods[name] = dot((s1, s2, s3, s4, s5, s6, s7)[q], wq(q))
                        elif kkcat:
                            r = dot(jnp.concatenate([k1, k2], axis=0), wq(7 if name[1] == 'l' else 8))
                            prods[name[:2] + 't'], prods[name[:2] + 'b'] = r[:hh], r[hh:]
                        else:
                            prods[name] = dot(k1 if name[2] == 't' else k2,
                                              wq(7 if name[1] == 'l' else 8))
                    return prods[name]

                for cb in corder:
                    acc = None
                    for tok in order[cb].split():
                        v = prod(tok.lstrip('-'))
                        acc = v if acc is None else (acc - v if tok[0] == '-' else acc + v)
                    queue.append((k, jc, cb, acc))
                    if len(queue) > lag:
                        finish(*queue.pop(0))
        while queue:
            finish(*queue.pop(0))

        if lnpre:
            lhs_to_scratch(xslots[nu0])

        for unpinned, u, _ in infos:
            @pl.when(jnp.logical_and(unpinned, u < nspill))
            def _():
                h_out_copy(u).start()
        infos, bacc, blo = phase0_state(t0 + nu0, bacc, blo)
        return infos, bacc, blo, xslots[nu0]

    if 0 in phases:
        zero = jnp.int32(0)
        jax.lax.fori_loop(0, ns // nu0, phase0_block, (*phase0_state(zero, zero, zero), zero))

    if 1 in phases:
        for k in range(xd):
            x_copy(ns - 1 - k, k).start()
    w2_copy.wait()
    ssq = jnp.concatenate(
        [jnp.sum(ssq_ref[j], axis=0, keepdims=True) for j in range(nj)], axis=1)
    ssq = ssq * (_HSCALE * _HSCALE)
    gx = jnp.sqrt(ssq + 1e-6)
    nx = gx / (jnp.mean(gx, axis=-1, keepdims=True) + 1e-6)
    s = (1.0 + g_ref[...].astype(F32) * nx) * _HSCALE
    s_t = _col(s, c4)
    kb = c4 // 3
    ws = [w2_ref[:, k * LANES:(k + 1) * LANES].astype(F32) * s_t for k in range(nk)]
    bl = [ws[l][j * kb:(j + 1) * kb] for j in range(3) for l in range(3)]
    for q, (t, sg) in enumerate(_combos(_HK_V, bl)):
        t = _force(t)
        if sg * _HK_USIGN[q] < 0:
            t = -t
        w2s_ref[q] = _pack(t.astype(BF16))
    b8 = jnp.broadcast_to(b_ref[...], (16, c4))
    bias_ref[...] = dot(b8, w2_ref[...])[:8]

    def phase1_state(i0, acc, lo):
        infos = []
        for su in range(nu1):
            infos.append(unit_info(ns - 1 - (i0 + su), acc, lo))
            acc, lo = step_down(acc, lo)
        return tuple(infos), acc, lo

    def phase1_block(blk, carry):
        prev, infos, bacc, blo, xs0 = carry
        hh1 = rbs1 // 2
        bias = bias_ref[0:1, :]
        i0 = blk * nu1
        xslots = [xs0]
        for _ in range(xd + nu1 - 1):
            xslots.append(xwrap(xslots[-1] + 1))
        for su in range(nu1):
            inx = i0 + su + xd

            @pl.when(jnp.logical_and(inx < ns, inx >= xr))
            def _():
                o_copy(ns - 1 - (inx - xr), xslots[su + xd]).wait()

            @pl.when(inx < ns)
            def _():
                x_copy(ns - 1 - inx, xslots[su + xd]).start()

        if not nodma:
            for unp_p, u_p, _ in prev:
                @pl.when(jnp.logical_and(unp_p, u_p >= ring))
                def _():
                    h_in_copy(u_p - ring).start()

        for su in range(nu1):
            x_copy(ns - 1 - (i0 + su), xslots[su]).wait()
            if not nodma:
                unpinned, u, _ = infos[su]

                @pl.when(jnp.logical_and(unpinned, u < nspill))
                def _():
                    h_in_copy(u).wait()

        for su in range(nu1):
            slot = infos[su][2]
            xslot = xslots[su]
            for rb in range(0 if nocomp else st // rbs1):
                r0 = rb * rbs1
                raw = [jnp.concatenate(
                    [_unpack(hs[slot, kk * njk + j,
                                (r0 + half * hh1) // 2:(r0 + (half + 1) * hh1) // 2, :])
                     for j in range(njk)], axis=1) for half in range(2) for kk in range(3)]
                flt = [_lazy(lambda a=a: a.astype(F32)) for a in raw]
                lhs = _combos(_HK_U, flt)
                ms = []
                for q, row in enumerate(_HK_U):
                    nzs = [ix for ix, cf in enumerate(row) if cf]
                    a = raw[nzs[0]] if len(nzs) == 1 else _force(lhs[q][0]).astype(BF16)
                    ms.append(dot(a, _unpack(w2s_ref[q])))
                cs = _combos([[w[o] for w in _HK_W] for o in range(6)], ms)
                for half in range(2):
                    rs = slice(r0 + half * hh1, r0 + (half + 1) * hh1)
                    for l in range(3):
                        cl = slice(l * LANES, (l + 1) * LANES)
                        val, sg = cs[half * 3 + l]
                        val = _force(val)
                        base = xb[xslot, rs, cl].astype(F32) + bias[:, cl]
                        xb[xslot, rs, cl] = (base + val if sg > 0 else base - val).astype(BF16)

        for su in range(nu1):
            o_copy(ns - 1 - (i0 + su), xslots[su]).start()
        nxt, bacc, blo = phase1_state(i0 + nu1, bacc, blo)
        return infos, nxt, bacc, blo, xslots[nu1]

    if 1 in phases:
        acc0, lo0 = jnp.int32(((ns - 1) * npin) % ns), jnp.int32(((ns - 1) * npin) // ns)
        first, acc0, lo0 = phase1_state(jnp.int32(0), acc0, lo0)
        none = tuple((jnp.bool_(False), jnp.int32(0), jnp.int32(0)) for _ in range(nu1))
        jax.lax.fori_loop(0, ns // nu1, phase1_block, (none, first, acc0, lo0, jnp.int32(0)))
        for i in range(ns - xr, ns):
            o_copy(ns - 1 - i, i % xr).wait()
    else:
        o_copy(0, 0).start()
        o_copy(0, 0).wait()


def _build(n, c, c4, st=1024, nu0=2, nu1=1, cn=128, ring=4, npin=34, xr=5, xd=2, vmem_mb=128,
           phases=(0, 1), rbs=128, rbs1=256, nodma=False, lnpre=True, lnm=0, rsq=1, order=_ORDER, gform=0, kkcat=True, corder=(2, 0, 3, 1), lag=0, lnpos=99,
           nobc=True, nocomp=False, hk0=False,
           perm0=None, corder0=(0, 3, 1, 4, 2, 5)):
    ns = n // st
    phases = tuple(phases)
    assert ring & (ring - 1) == 0 and xd + nu1 <= xr
    assert xr >= 2 * nu0 + (1 if lnpre else 0) and xr >= xd + 2 * nu1 and xd >= nu1
    kern = functools.partial(_kernel, st=st, nu0=nu0, nu1=nu1, ns=ns, c=c, c4=c4, cn=cn,
                             ring=ring, npin=npin, xr=xr, xd=xd, rbs=rbs, rbs1=rbs1,
                             phases=phases, nodma=nodma, lnpre=lnpre, lnm=lnm, rsq=rsq,
                             order=tuple(order), gform=gform, kkcat=kkcat,
                             corder=tuple(corder), lag=lag, lnpos=lnpos, nocomp=nocomp, hk0=hk0,
                             perm0=perm0, corder0=tuple(corder0))
    nj = c4 // LANES
    hbm = pl.BlockSpec(memory_space=pl.ANY)
    vmem = pl.BlockSpec(memory_space=pltpu.VMEM)
    return pl.pallas_call(
        kern,
        in_specs=[hbm, vmem, hbm, hbm, vmem, vmem],
        out_specs=[hbm, hbm],
        out_shape=[
            jax.ShapeDtypeStruct((n, c), BF16),
            jax.ShapeDtypeStruct((ns - npin - ring, nj, st // 2, LANES), U32),
        ],
        scratch_shapes=[
            pltpu.VMEM((ring + npin, nj, st // 2, LANES), U32),
            pltpu.VMEM((xr, st, c), BF16),
            pltpu.VMEM((15 if hk0 else 9, rbs // 4, LANES), U32),
            pltpu.VMEM((nj, 8, LANES), F32),
            pltpu.VMEM((5 * nj if hk0 else 9 * nj // 2, LANES // 2, LANES), U32),
            pltpu.VMEM((15, c4 // 6, LANES), U32),
            pltpu.VMEM((8, c), F32),
            pltpu.VMEM((c, c4), BF16),
            pltpu.VMEM((c4, c), BF16),
            pltpu.SemaphoreType.DMA((ring,)),
            pltpu.SemaphoreType.DMA((xr,)),
            pltpu.SemaphoreType.DMA((xr,)),
            pltpu.SemaphoreType.DMA((2,)),
        ],
        compiler_params=pltpu.CompilerParams(
            vmem_limit_bytes=vmem_mb * 1024 * 1024,
            disable_bounds_checks=nobc,
        ),
    )


def _run(x, dw, w1, w2, grn_g, grn_b, **kw):
    b, hh, ww, c = x.shape
    c4 = w1.shape[1]
    n = b * hh * ww
    assert b == 1 and dw.shape[0] == 1 and dw.shape[1] == 1
    out, _ = _build(n, c, c4, **kw)(
        x.reshape(n, c), dw.reshape(1, c), w1, w2,
        grn_g.reshape(1, c4), grn_b.reshape(1, c4))
    return out.reshape(x.shape)


@jax.jit
def pallas_standalone__modern_conv_block_slak__vision_kernel(
    x: jax.Array,
    dw: jax.Array,
    w1: jax.Array,
    w2: jax.Array,
    grn_g: jax.Array,
    grn_b: jax.Array,
):
    return _run(x, dw, w1, w2, grn_g, grn_b)
```

```python
import functools
import math

import jax
import jax.numpy as jnp
import jax.experimental.pallas as pl
import jax.experimental.pallas.tpu as pltpu

F32 = jnp.float32
BF16 = jnp.bfloat16
U32 = jnp.uint32
LANES = 128

_GELU_C0 = 0.7978845608028654
_GELU_C1 = 0.7978845608028654 * 0.044715
_LAM = _GELU_C1 ** (1.0 / 3.0)
_KAP = _GELU_C0 / _LAM
_HSCALE = 1.0 / (2.0 * _LAM)
_LOG2E = 1.4426950408889634
_RS_C = math.log2(_LAM) + 0.5 * math.log2(384.0)


_HK_U = ((0, 0, 0, 1, -1, 0), (-1, 0, 0, 0, 0, 1), (1, 0, 0, -1, 0, 0), (-1, 0, 0, 0, 0, 0),
         (0, 0, -1, 0, 0, 1), (1, 0, 0, -1, 1, 0), (0, -1, 0, 0, 0, 0), (0, -1, 1, 0, 0, -1),
         (0, 1, -1, 0, 0, 0), (1, 0, -1, 0, 0, 0), (0, 0, 0, 0, -1, 0), (0, 0, 0, -1, 0, 1),
         (0, 1, -1, 0, -1, 1), (-1, 1, 0, 1, -1, 0), (0, 0, 0, 0, 0, 1))
_HK_V = ((0, 0, 1, 0, 0, 0, 0, 0, 0), (0, -1, 0, 0, 0, 0, 1, 0, 0), (1, 1, 0, 1, 0, 0, 0, 0, 0),
         (1, 0, -1, 0, 0, 0, 1, 0, 0), (0, 0, 0, 0, 1, 0, 1, 1, 0), (0, 0, 1, 1, 0, 0, 0, 0, 0),
         (0, 0, 0, -1, 0, 1, 0, 0, 1), (0, 0, 0, 0, -1, 0, 0, 0, -1), (0, 0, 0, 0, 0, 0, 0, 0, 1),
         (0, 0, 0, 0, 0, 0, 1, 0, 0), (0, 0, 1, 0, -1, 1, 0, 0, 0), (0, -1, 0, 0, 0, 0, 0, 0, 0),
         (0, 0, 0, 0, -1, 0, 0, 0, 0), (0, 0, 0, 1, 0, 0, 0, 0, 0), (0, -1, 0, 0, 0, 0, 0, -1, 1))
_HK_W = ((1, 0, 1, 1, 0, 1), (0, 1, 0, 1, 0, 0), (0, 0, 0, -1, 0, 0), (-1, 0, 0, -1, 0, 0),
         (0, -1, 0, 0, 0, 0), (1, 0, 1, 1, 0, 0), (0, 0, -1, 0, 0, 0), (0, 1, 0, 0, 1, 1),
         (0, -1, -1, 0, -1, -1), (-1, 1, 0, 0, 0, 0), (0, 0, 0, 0, 0, -1), (0, 0, 0, -1, 1, 0),
         (0, 0, 0, 0, 1, 1), (1, 0, 1, 0, 0, 0), (0, -1, 0, 0, -1, 0))


def _combos(rows, vals, perm=None):
    vals = list(vals)
    rank = list(perm) if perm is not None else list(range(len(vals)))
    rows = [{i: c for i, c in enumerate(r) if c} for r in rows]
    while True:
        cnt = {}
        for r in rows:
            ks = sorted(r, key=lambda i: rank[i])
            for ia, a in enumerate(ks):
                for b in ks[ia + 1:]:
                    key = (a, b, r[a] * r[b])
                    cnt[key] = cnt.get(key, 0) + 1
        if not cnt or max(cnt.values()) < 2:
            break
        a, b, sg = max(sorted(cnt, key=lambda k_: (rank[k_[0]], rank[k_[1]], k_[2])),
                       key=lambda k_: cnt[k_])
        vals.append(_lazy(lambda a=a, b=b, sg=sg: (
            _force(vals[a]) + _force(vals[b]) if sg > 0 else _force(vals[a]) - _force(vals[b]))))
        rank.append(max(rank[a], rank[b]) + 0.5)
        new = len(vals) - 1
        for r in rows:
            if a in r and b in r and r[a] * r[b] == sg:
                r[new] = r.pop(a)
                del r[b]

    def total(items, sign):
        acc = _force(vals[items[0][0]])
        for idx, cf in items[1:]:
            acc = acc + _force(vals[idx]) if cf * sign > 0 else acc - _force(vals[idx])
        return acc

    out = []
    for r in rows:
        items = sorted(r.items(), key=lambda kv: rank[kv[0]])
        pos = [i for i, kv in enumerate(items) if kv[1] > 0]
        if pos and pos[0] > 0 and len(pos) < len(items):
            items.insert(0, items.pop(pos[0]))
        sign = items[0][1]
        out.append((_lazy(functools.partial(total, items, sign)), sign))
    return out


class _lazy:
    def __init__(self, fn):
        self.fn, self.val = fn, None


def _force(v):
    if isinstance(v, _lazy):
        if v.val is None:
            v.val = v.fn()
        return v.val
    return v


_HK_USIGN = tuple(sg for _, sg in _combos(_HK_U, [1.0] * 6))


def _col(row, n):
    return jnp.transpose(jnp.broadcast_to(row, (LANES, n)))


def _pack(v):
    return pltpu.bitcast(v, U32)


def _unpack(v):
    return pltpu.bitcast(v, BF16)


_ORDER = ('klt m4 -m5 m1 m7', 'krt m3 m5', 'm4 klb m2', 'm1 m3 m6 -m2 krb')


def _kernel(x_hbm, dw_ref, w1_hbm, w2_hbm, g_ref, b_ref,
            o_hbm, h_hbm,
            hs, xb, sb0, ssq_ref, w1s_ref, w2s_ref, bias_ref, w1_ref, w2_ref,
            sem_h, sem_x, sem_o, sem_w,
            *, st, nu0, nu1, ns, c, c4, cn, ring, npin, xr, xd, rbs, rbs1, phases, nodma,
            lnpre, lnm, rsq, order, gform, kkcat, corder, lag, lnpos, nocomp, hk0, perm0, corder0, perm1, corder1, eager1):
    nj = c4 // LANES
    njh = nj // 2
    njk = nj // 3
    nk = c // LANES
    nspill = ns - npin - ring
    dot = functools.partial(jnp.dot, preferred_element_type=F32)

    def unit_info(t, acc, lo):
        unpinned = acc + npin < ns
        u = t - lo
        slot = jnp.where(unpinned, wrap_ring(u), ring + lo)
        return unpinned, u, slot

    def wrap_ring(u):
        return u & (ring - 1)

    def step_up(acc, lo):
        acc = acc + npin
        wrap = acc >= ns
        return jnp.where(wrap, acc - ns, acc), jnp.where(wrap, lo + 1, lo)

    def step_down(acc, lo):
        acc = acc - npin
        wrap = acc < 0
        return jnp.where(wrap, acc + ns, acc), jnp.where(wrap, lo - 1, lo)

    def xwrap(v):
        return jnp.where(v >= xr, v - xr, v)

    def h_out_copy(u):
        return pltpu.make_async_copy(hs.at[wrap_ring(u)], h_hbm.at[u], sem_h.at[wrap_ring(u)])

    def h_in_copy(u):
        return pltpu.make_async_copy(h_hbm.at[u], hs.at[wrap_ring(u)], sem_h.at[wrap_ring(u)])

    def x_copy(t, slot):
        return pltpu.make_async_copy(x_hbm.at[pl.ds(t * st, st), :], xb.at[slot], sem_x.at[slot])

    def o_copy(t, slot):
        return pltpu.make_async_copy(xb.at[slot], o_hbm.at[pl.ds(t * st, st), :], sem_o.at[slot])

    w1_copy = pltpu.make_async_copy(w1_hbm, w1_ref, sem_w.at[0])
    w2_copy = pltpu.make_async_copy(w2_hbm, w2_ref, sem_w.at[1])

    hh = rbs // 2

    def strassen_lhs(xslot, rb):
        dw = dw_ref[...].astype(F32)

        def scale(ss):
            if rsq == 0:
                return _LAM * jax.lax.rsqrt(ss * (1.0 / c) + 1e-5)
            return jnp.exp2(jnp.log(ss + c * 1e-5) * (-0.5 * _LOG2E) + _RS_C)

        def layernorm(xf):
            y = xf * dw
            if lnm == 0:
                yc = y - jnp.sum(y, axis=-1, keepdims=True) * (1.0 / c)
                return yc * scale(jnp.sum(yc * yc, axis=-1, keepdims=True))
            s1 = jnp.sum(y, axis=-1, keepdims=True)
            s2 = jnp.sum(y * y, axis=-1, keepdims=True)
            m = s1 * (1.0 / c)
            return (y - m) * scale(jnp.maximum(s2 - s1 * m, 0.0))

        xu = _pack(xb[xslot, rb * rbs:(rb + 1) * rbs, :])
        a1, a2 = [layernorm(pltpu.unpack_elementwise(
            xu, index=k, packed_dtype=BF16, unpacked_dtype=F32)) for k in range(2)]
        a11, a12, a13 = (a1[:, k * LANES:(k + 1) * LANES] for k in range(3))
        a21, a22, a23 = (a2[:, k * LANES:(k + 1) * LANES] for k in range(3))
        if hk0:
            return [_force(v) for v, _ in _combos(_HK_U, [a11, a12, a13, a21, a22, a23])]
        return [a11 + a22, a21 + a22, a11, a22, a11 + a12, a21 - a11, a12 - a22, a13, a23]

    def lhs_to_scratch(xslot):
        for q, t in enumerate(strassen_lhs(xslot, 0)):
            sb0[q] = _pack(t.astype(BF16))

    look = 1 if lnpre else 0
    w1_copy.start()
    if 0 in phases:
        for k in range(nu0 + look):
            x_copy(k, k).start()
    w2_copy.start()
    w1_copy.wait()
    ssq_ref[...] = jnp.zeros_like(ssq_ref)
    if hk0:
        for j in range(njk):
            bl = [w1_ref[kb_ * LANES:(kb_ + 1) * LANES,
                         (l * njk + j) * LANES:(l * njk + j + 1) * LANES].astype(F32)
                  for kb_ in range(3) for l in range(3)]
            for q, (t, sg) in enumerate(_combos(_HK_V, bl)):
                t = _force(t)
                if sg * _HK_USIGN[q] < 0:
                    t = -t
                w1s_ref[q * njk + j] = _pack(t.astype(BF16))
    for j in range(0 if hk0 else njh):
        cl = slice(j * LANES, (j + 1) * LANES)
        cr = slice((njh + j) * LANES, (njh + j + 1) * LANES)
        b11 = w1_ref[0:LANES, cl].astype(F32)
        b12 = w1_ref[0:LANES, cr].astype(F32)
        b21 = w1_ref[LANES:2 * LANES, cl].astype(F32)
        b22 = w1_ref[LANES:2 * LANES, cr].astype(F32)
        combos = [b11 + b22, b11, b12 - b22, b21 - b11, b22, b11 + b12, b21 + b22]
        for q, t in enumerate(combos):
            w1s_ref[q * njh + j] = _pack(t.astype(BF16))
        w1s_ref[7 * njh + j] = _pack(w1_ref[2 * LANES:3 * LANES, cl])
        w1s_ref[8 * njh + j] = _pack(w1_ref[2 * LANES:3 * LANES, cr])
    if 0 in phases and lnpre:
        x_copy(0, 0).wait()
        lhs_to_scratch(0)

    def gelu(b):
        t = jnp.tanh(b * (b * b + _KAP))
        return b * (1.0 + t) if gform == 0 else b + b * t

    def phase0_state(t0, acc, lo):
        infos = []
        for su in range(nu0):
            infos.append(unit_info(t0 + su, acc, lo))
            acc, lo = step_up(acc, lo)
        return tuple(infos), acc, lo

    def phase0_block(blk, carry):
        infos, bacc, blo, xs0 = carry
        jb = cn // LANES
        t0 = blk * nu0
        xslots = [xs0]
        for _ in range(2 * nu0 + look - 1):
            xslots.append(xwrap(xslots[-1] + 1))
        for su in range(nu0):
            tn = t0 + nu0 + look + su

            @pl.when(tn < ns)
            def _():
                x_copy(tn, xslots[nu0 + look + su]).start()

        for su in range(nu0):
            tw = t0 + look + su

            @pl.when(tw < ns)
            def _():
                x_copy(tw, xslots[look + su]).wait()

        for unpinned, u, _ in infos:
            @pl.when(jnp.logical_and(unpinned, u >= ring))
            def _():
                h_out_copy(u - ring).wait()

        nrb = st // rbs
        nch = njh // jb
        rbl = [(su, rb) for su in range(nu0) for rb in range(nrb)]
        lhs_cache = {}

        def get_lhs(k):
            if k not in lhs_cache:
                su, rb = rbl[k]
                if lnpre and k == 0:
                    ops = [_unpack(sb0[q]) for q in range(15 if hk0 else 9)]
                else:
                    ops = [t.astype(BF16) for t in strassen_lhs(xslots[su], rb)]
                lhs_cache[k] = ops
            return lhs_cache[k]

        done = {}

        def finish(k, jc, cb, pre):
            done[(k, jc, cb)] = gelu(pre)
            for top, bot, j0 in ((0, 2, jc * jb), (1, 3, njh + jc * jb)):
                if cb in (top, bot) and (k, jc, top) in done and (k, jc, bot) in done:
                    gt, gb = done.pop((k, jc, top)), done.pop((k, jc, bot))
                    su, rb = rbl[k]
                    sq = jnp.sum((gt * gt + gb * gb).reshape(hh // 8, 8, cn), axis=0)
                    hp = pltpu.pack_elementwise([gt, gb], packed_dtype=BF16)
                    for kq in range(jb):
                        ls = slice(kq * LANES, (kq + 1) * LANES)
                        ssq_ref[j0 + kq] += sq[:, ls]
                        hs[infos[su][2], j0 + kq, rb * hh:(rb + 1) * hh, :] = hp[:, ls]

        def finish_hk(k, jc, o, pre, sg):
            done[(k, jc, o)] = gelu(pre if sg > 0 else -pre)
            l = o % 3
            if (k, jc, l) in done and (k, jc, l + 3) in done:
                gt, gb = done.pop((k, jc, l)), done.pop((k, jc, l + 3))
                su, rb = rbl[k]
                sq = jnp.sum((gt * gt + gb * gb).reshape(hh // 8, 8, LANES), axis=0)
                j0 = l * njk + jc
                ssq_ref[j0] += sq
                hs[infos[su][2], j0, rb * hh:(rb + 1) * hh, :] = pltpu.pack_elementwise(
                    [gt, gb], packed_dtype=BF16)

        for k in range(len(rbl) if hk0 else 0):
            for jc in range(njk):
                ops = get_lhs(k)
                ms = [_lazy(lambda q=q: dot(ops[q], _unpack(w1s_ref[q * njk + jc])))
                      for q in range(15)]
                cs = _combos([[w[o] for w in _HK_W] for o in range(6)], ms, perm0)
                for o in corder0:
                    finish_hk(k, jc, o, _force(cs[o][0]), cs[o][1])

        queue = []
        for k in range(0 if hk0 else len(rbl)):
            for jc in range(nch):
                if jc == lnpos and k + 1 < len(rbl):
                    get_lhs(k + 1)
                s1, s2, s3, s4, s5, s6, s7, k1, k2 = get_lhs(k)

                def wq(q):
                    ws = [_unpack(w1s_ref[q * njh + jc * jb + kq]) for kq in range(jb)]
                    return ws[0] if jb == 1 else jnp.concatenate(ws, axis=1)

                prods = {}

                def prod(name):
                    if name not in prods:
                        if name[0] == 'm':
                            q = int(name[1]) - 1
                            prods[name] = dot((s1, s2, s3, s4, s5, s6, s7)[q], wq(q))
                        elif kkcat:
                            r = dot(jnp.concatenate([k1, k2], axis=0), wq(7 if name[1] == 'l' else 8))
                            prods[name[:2] + 't'], prods[name[:2] + 'b'] = r[:hh], r[hh:]
                        else:
                            prods[name] = dot(k1 if name[2] == 't' else k2,
                                              wq(7 if name[1] == 'l' else 8))
                    return prods[name]

                for cb in corder:
                    acc = None
                    for tok in order[cb].split():
                        v = prod(tok.lstrip('-'))
                        acc = v if acc is None else (acc - v if tok[0] == '-' else acc + v)
                    queue.append((k, jc, cb, acc))
                    if len(queue) > lag:
                        finish(*queue.pop(0))
        while queue:
            finish(*queue.pop(0))

        if lnpre:
            lhs_to_scratch(xslots[nu0])

        for unpinned, u, _ in infos:
            @pl.when(jnp.logical_and(unpinned, u < nspill))
            def _():
                h_out_copy(u).start()
        infos, bacc, blo = phase0_state(t0 + nu0, bacc, blo)
        return infos, bacc, blo, xslots[nu0]

    if 0 in phases:
        zero = jnp.int32(0)
        jax.lax.fori_loop(0, ns // nu0, phase0_block, (*phase0_state(zero, zero, zero), zero))

    if 1 in phases:
        for k in range(xd):
            x_copy(ns - 1 - k, k).start()
    w2_copy.wait()
    ssq = jnp.concatenate(
        [jnp.sum(ssq_ref[j], axis=0, keepdims=True) for j in range(nj)], axis=1)
    ssq = ssq * (_HSCALE * _HSCALE)
    gx = jnp.sqrt(ssq + 1e-6)
    nx = gx / (jnp.mean(gx, axis=-1, keepdims=True) + 1e-6)
    s = (1.0 + g_ref[...].astype(F32) * nx) * _HSCALE
    s_t = _col(s, c4)
    kb = c4 // 3
    ws = [w2_ref[:, k * LANES:(k + 1) * LANES].astype(F32) * s_t for k in range(nk)]
    bl = [ws[l][j * kb:(j + 1) * kb] for j in range(3) for l in range(3)]
    for q, (t, sg) in enumerate(_combos(_HK_V, bl)):
        t = _force(t)
        if sg * _HK_USIGN[q] < 0:
            t = -t
        w2s_ref[q] = _pack(t.astype(BF16))
    b8 = jnp.broadcast_to(b_ref[...], (16, c4))
    bias_ref[...] = dot(b8, w2_ref[...])[:8]

    def phase1_state(i0, acc, lo):
        infos = []
        for su in range(nu1):
            infos.append(unit_info(ns - 1 - (i0 + su), acc, lo))
            acc, lo = step_down(acc, lo)
        return tuple(infos), acc, lo

    def phase1_block(blk, carry):
        prev, infos, bacc, blo, xs0 = carry
        hh1 = rbs1 // 2
        bias = bias_ref[0:1, :]
        i0 = blk * nu1
        xslots = [xs0]
        for _ in range(xd + nu1 - 1):
            xslots.append(xwrap(xslots[-1] + 1))
        for su in range(nu1):
            inx = i0 + su + xd

            @pl.when(jnp.logical_and(inx < ns, inx >= xr))
            def _():
                o_copy(ns - 1 - (inx - xr), xslots[su + xd]).wait()

            @pl.when(inx < ns)
            def _():
                x_copy(ns - 1 - inx, xslots[su + xd]).start()

        if not nodma:
            for unp_p, u_p, _ in prev:
                @pl.when(jnp.logical_and(unp_p, u_p >= ring))
                def _():
                    h_in_copy(u_p - ring).start()

        for su in range(nu1):
            x_copy(ns - 1 - (i0 + su), xslots[su]).wait()
            if not nodma:
                unpinned, u, _ = infos[su]

                @pl.when(jnp.logical_and(unpinned, u < nspill))
                def _():
                    h_in_copy(u).wait()

        for su in range(nu1):
            slot = infos[su][2]
            xslot = xslots[su]
            for rb in range(0 if nocomp else st // rbs1):
                r0 = rb * rbs1
                raw = [jnp.concatenate(
                    [_unpack(hs[slot, kk * njk + j,
                                (r0 + half * hh1) // 2:(r0 + (half + 1) * hh1) // 2, :])
                     for j in range(njk)], axis=1) for half in range(2) for kk in range(3)]
                flt = [_lazy(lambda a=a: a.astype(F32)) for a in raw]
                lhs = _combos(_HK_U, flt)

                def product(q):
                    nzs = [ix for ix, cf in enumerate(_HK_U[q]) if cf]
                    a = raw[nzs[0]] if len(nzs) == 1 else _force(lhs[q][0]).astype(BF16)
                    return dot(a, _unpack(w2s_ref[q]))

                ms = [_lazy(functools.partial(product, q)) for q in range(15)]
                if eager1:
                    for q in (perm1 or range(15)):
                        pass
                    for q in sorted(range(15), key=lambda q_: (perm1 or range(15))[q_]):
                        _force(ms[q])
                cs = _combos([[w[o] for w in _HK_W] for o in range(6)], ms, perm1)
                for o in corder1:
                    half, l = divmod(o, 3)
                    rs = slice(r0 + half * hh1, r0 + (half + 1) * hh1)
                    cl = slice(l * LANES, (l + 1) * LANES)
                    val, sg = cs[o]
                    val = _force(val)
                    base = xb[xslot, rs, cl].astype(F32) + bias[:, cl]
                    xb[xslot, rs, cl] = (base + val if sg > 0 else base - val).astype(BF16)

        for su in range(nu1):
            o_copy(ns - 1 - (i0 + su), xslots[su]).start()
        nxt, bacc, blo = phase1_state(i0 + nu1, bacc, blo)
        return infos, nxt, bacc, blo, xslots[nu1]

    if 1 in phases:
        acc0, lo0 = jnp.int32(((ns - 1) * npin) % ns), jnp.int32(((ns - 1) * npin) // ns)
        first, acc0, lo0 = phase1_state(jnp.int32(0), acc0, lo0)
        none = tuple((jnp.bool_(False), jnp.int32(0), jnp.int32(0)) for _ in range(nu1))
        jax.lax.fori_loop(0, ns // nu1, phase1_block, (none, first, acc0, lo0, jnp.int32(0)))
        for i in range(ns - xr, ns):
            o_copy(ns - 1 - i, i % xr).wait()
    else:
        o_copy(0, 0).start()
        o_copy(0, 0).wait()


def _build(n, c, c4, st=1024, nu0=2, nu1=1, cn=128, ring=4, npin=33, xr=5, xd=2, vmem_mb=128,
           phases=(0, 1), rbs=128, rbs1=256, nodma=False, lnpre=True, lnm=0, rsq=1, order=_ORDER, gform=0, kkcat=True, corder=(2, 0, 3, 1), lag=0, lnpos=99,
           nobc=True, nocomp=False, hk0=True,
           perm0=(13, 2, 10, 0, 11, 7, 6, 4, 9, 5, 14, 1, 8, 3, 12), corder0=(3, 2, 1, 4, 0, 5),
           perm1=(6, 4, 5, 8, 9, 7, 10, 13, 0, 11, 12, 3, 2, 14, 1), corder1=(1, 4, 2, 3, 5, 0),
           eager1=False):
    ns = n // st
    phases = tuple(phases)
    assert ring & (ring - 1) == 0 and xd + nu1 <= xr
    assert xr >= 2 * nu0 + (1 if lnpre else 0) and xr >= xd + 2 * nu1 and xd >= nu1
    kern = functools.partial(_kernel, st=st, nu0=nu0, nu1=nu1, ns=ns, c=c, c4=c4, cn=cn,
                             ring=ring, npin=npin, xr=xr, xd=xd, rbs=rbs, rbs1=rbs1,
                             phases=phases, nodma=nodma, lnpre=lnpre, lnm=lnm, rsq=rsq,
                             order=tuple(order), gform=gform, kkcat=kkcat,
                             corder=tuple(corder), lag=lag, lnpos=lnpos, nocomp=nocomp, hk0=hk0,
                             perm0=perm0, corder0=tuple(corder0), perm1=perm1,
                             corder1=tuple(corder1), eager1=eager1)
    nj = c4 // LANES
    hbm = pl.BlockSpec(memory_space=pl.ANY)
    vmem = pl.BlockSpec(memory_space=pltpu.VMEM)
    return pl.pallas_call(
        kern,
        in_specs=[hbm, vmem, hbm, hbm, vmem, vmem],
        out_specs=[hbm, hbm],
        out_shape=[
            jax.ShapeDtypeStruct((n, c), BF16),
            jax.ShapeDtypeStruct((ns - npin - ring, nj, st // 2, LANES), U32),
        ],
        scratch_shapes=[
            pltpu.VMEM((ring + npin, nj, st // 2, LANES), U32),
            pltpu.VMEM((xr, st, c), BF16),
            pltpu.VMEM((15 if hk0 else 9, rbs // 4, LANES), U32),
            pltpu.VMEM((nj, 8, LANES), F32),
            pltpu.VMEM((5 * nj if hk0 else 9 * nj // 2, LANES // 2, LANES), U32),
            pltpu.VMEM((15, c4 // 6, LANES), U32),
            pltpu.VMEM((8, c), F32),
            pltpu.VMEM((c, c4), BF16),
            pltpu.VMEM((c4, c), BF16),
            pltpu.SemaphoreType.DMA((ring,)),
            pltpu.SemaphoreType.DMA((xr,)),
            pltpu.SemaphoreType.DMA((xr,)),
            pltpu.SemaphoreType.DMA((2,)),
        ],
        compiler_params=pltpu.CompilerParams(
            vmem_limit_bytes=vmem_mb * 1024 * 1024,
            disable_bounds_checks=nobc,
        ),
    )


def _run(x, dw, w1, w2, grn_g, grn_b, **kw):
    b, hh, ww, c = x.shape
    c4 = w1.shape[1]
    n = b * hh * ww
    assert b == 1 and dw.shape[0] == 1 and dw.shape[1] == 1
    out, _ = _build(n, c, c4, **kw)(
        x.reshape(n, c), dw.reshape(1, c), w1, w2,
        grn_g.reshape(1, c4), grn_b.reshape(1, c4))
    return out.reshape(x.shape)


@jax.jit
def pallas_standalone__modern_conv_block_slak__vision_kernel(
    x: jax.Array,
    dw: jax.Array,
    w1: jax.Array,
    w2: jax.Array,
    grn_g: jax.Array,
    grn_b: jax.Array,
):
    return _run(x, dw, w1, w2, grn_g, grn_b)
```

```python
import functools
import math

import jax
import jax.numpy as jnp
import jax.experimental.pallas as pl
import jax.experimental.pallas.tpu as pltpu

F32 = jnp.float32
BF16 = jnp.bfloat16
U32 = jnp.uint32
LANES = 128

_GELU_C0 = math.sqrt(2.0 / math.pi)
_GELU_C1 = _GELU_C0 * 0.044715
_LAM = _GELU_C1 ** (1.0 / 3.0)
_KAP = _GELU_C0 / _LAM
_HSCALE = 1.0 / (2.0 * _LAM)
_LN_EPS = 1e-5
_GRN_EPS = 1e-6

_HK_U = ((0, 0, 0, 1, -1, 0), (-1, 0, 0, 0, 0, 1), (1, 0, 0, -1, 0, 0), (-1, 0, 0, 0, 0, 0),
         (0, 0, -1, 0, 0, 1), (1, 0, 0, -1, 1, 0), (0, -1, 0, 0, 0, 0), (0, -1, 1, 0, 0, -1),
         (0, 1, -1, 0, 0, 0), (1, 0, -1, 0, 0, 0), (0, 0, 0, 0, -1, 0), (0, 0, 0, -1, 0, 1),
         (0, 1, -1, 0, -1, 1), (-1, 1, 0, 1, -1, 0), (0, 0, 0, 0, 0, 1))
_HK_V = ((0, 0, 1, 0, 0, 0, 0, 0, 0), (0, -1, 0, 0, 0, 0, 1, 0, 0), (1, 1, 0, 1, 0, 0, 0, 0, 0),
         (1, 0, -1, 0, 0, 0, 1, 0, 0), (0, 0, 0, 0, 1, 0, 1, 1, 0), (0, 0, 1, 1, 0, 0, 0, 0, 0),
         (0, 0, 0, -1, 0, 1, 0, 0, 1), (0, 0, 0, 0, -1, 0, 0, 0, -1), (0, 0, 0, 0, 0, 0, 0, 0, 1),
         (0, 0, 0, 0, 0, 0, 1, 0, 0), (0, 0, 1, 0, -1, 1, 0, 0, 0), (0, -1, 0, 0, 0, 0, 0, 0, 0),
         (0, 0, 0, 0, -1, 0, 0, 0, 0), (0, 0, 0, 1, 0, 0, 0, 0, 0), (0, -1, 0, 0, 0, 0, 0, -1, 1))
_HK_W = ((1, 0, 1, 1, 0, 1), (0, 1, 0, 1, 0, 0), (0, 0, 0, -1, 0, 0), (-1, 0, 0, -1, 0, 0),
         (0, -1, 0, 0, 0, 0), (1, 0, 1, 1, 0, 0), (0, 0, -1, 0, 0, 0), (0, 1, 0, 0, 1, 1),
         (0, -1, -1, 0, -1, -1), (-1, 1, 0, 0, 0, 0), (0, 0, 0, 0, 0, -1), (0, 0, 0, -1, 1, 0),
         (0, 0, 0, 0, 1, 1), (1, 0, 1, 0, 0, 0), (0, -1, 0, 0, -1, 0))
_HK_WT = tuple(tuple(w[o] for w in _HK_W) for o in range(6))
_NPROD = len(_HK_U)


class _lazy:
    def __init__(self, fn):
        self.fn, self.val = fn, None


def _force(v):
    if isinstance(v, _lazy):
        if v.val is None:
            v.val = v.fn()
        return v.val
    return v


def _combos(rows, vals, perm=None):
    vals = list(vals)
    rank = list(perm) if perm is not None else list(range(len(vals)))
    rows = [{i: c for i, c in enumerate(r) if c} for r in rows]
    while True:
        cnt = {}
        for r in rows:
            ks = sorted(r, key=lambda i: rank[i])
            for ia, a in enumerate(ks):
                for b in ks[ia + 1:]:
                    key = (a, b, r[a] * r[b])
                    cnt[key] = cnt.get(key, 0) + 1
        if not cnt or max(cnt.values()) < 2:
            break
        a, b, sg = max(sorted(cnt, key=lambda k_: (rank[k_[0]], rank[k_[1]], k_[2])),
                       key=lambda k_: cnt[k_])
        vals.append(_lazy(lambda a=a, b=b, sg=sg: (
            _force(vals[a]) + _force(vals[b]) if sg > 0 else _force(vals[a]) - _force(vals[b]))))
        rank.append(max(rank[a], rank[b]) + 0.5)
        new = len(vals) - 1
        for r in rows:
            if a in r and b in r and r[a] * r[b] == sg:
                r[new] = r.pop(a)
                del r[b]

    def total(items, sign):
        acc = _force(vals[items[0][0]])
        for idx, cf in items[1:]:
            acc = acc + _force(vals[idx]) if cf * sign > 0 else acc - _force(vals[idx])
        return acc

    out = []
    for r in rows:
        items = sorted(r.items(), key=lambda kv: rank[kv[0]])
        pos = [i for i, kv in enumerate(items) if kv[1] > 0]
        if pos and pos[0] > 0:
            items.insert(0, items.pop(pos[0]))
        sign = items[0][1]
        out.append((_lazy(functools.partial(total, items, sign)), sign))
    return out


_HK_USIGN = tuple(sg for _, sg in _combos(_HK_U, [1.0] * 6))


def _weight_sums(blocks):
    res = []
    for q, (t, sg) in enumerate(_combos(_HK_V, blocks)):
        t = _force(t)
        res.append(_pack((t if sg * _HK_USIGN[q] > 0 else -t).astype(BF16)))
    return res


def _col(row, n):
    return jnp.transpose(jnp.broadcast_to(row, (LANES, n)))


def _pack(v):
    return pltpu.bitcast(v, U32)


def _unpack(v):
    return pltpu.bitcast(v, BF16)


def _kernel(x_hbm, dw_ref, w1_hbm, w2_hbm, g_ref, b_ref,
            o_hbm, h_hbm,
            hs, xb, sb0, ssq_ref, ws_ref, bias_ref, w1_ref, w2_ref,
            sem_h, sem_x, sem_o, sem_w,
            *, st, nu0, nu1, ns, c, c4, ring, npin, xr, xd, rbs0, rbs1,
            perm0, corder0, perm1, corder1, phases, nodma, nocomp):
    nj = c4 // LANES
    njk = nj // 3
    nspill = ns - npin - ring
    dot = functools.partial(jnp.dot, preferred_element_type=F32)

    def wrap_ring(u):
        return u & (ring - 1)

    def unit_info(t, acc, lo):
        unpinned = acc + npin < ns
        u = t - lo
        return unpinned, u, jnp.where(unpinned, wrap_ring(u), ring + lo)

    def step_up(acc, lo):
        acc = acc + npin
        wrap = acc >= ns
        return jnp.where(wrap, acc - ns, acc), jnp.where(wrap, lo + 1, lo)

    def step_down(acc, lo):
        acc = acc - npin
        wrap = acc < 0
        return jnp.where(wrap, acc + ns, acc), jnp.where(wrap, lo - 1, lo)

    def x_slots(first, n):
        res = [first]
        for _ in range(n - 1):
            nxt = res[-1] + 1
            res.append(jnp.where(nxt >= xr, nxt - xr, nxt))
        return res

    def h_out_copy(u):
        return pltpu.make_async_copy(hs.at[wrap_ring(u)], h_hbm.at[u], sem_h.at[wrap_ring(u)])

    def h_in_copy(u):
        return pltpu.make_async_copy(h_hbm.at[u], hs.at[wrap_ring(u)], sem_h.at[wrap_ring(u)])

    def x_copy(t, slot):
        return pltpu.make_async_copy(x_hbm.at[pl.ds(t * st, st), :], xb.at[slot], sem_x.at[slot])

    def o_copy(t, slot):
        return pltpu.make_async_copy(xb.at[slot], o_hbm.at[pl.ds(t * st, st), :], sem_o.at[slot])

    w1_copy = pltpu.make_async_copy(w1_hbm, w1_ref, sem_w.at[0])
    w2_copy = pltpu.make_async_copy(w2_hbm, w2_ref, sem_w.at[1])

    hh = rbs0 // 2

    def phase0_lhs(xslot, rb):
        dw = dw_ref[...].astype(F32)

        def layernorm(xf):
            y = xf * dw
            yc = y - jnp.sum(y, axis=-1, keepdims=True) * (1.0 / c)
            ss = jnp.sum(yc * yc, axis=-1, keepdims=True)
            return yc * jnp.exp2(jnp.log(ss + c * _LN_EPS) * (-0.5 / math.log(2.0)))

        xu = _pack(xb[xslot, rb * rbs0:(rb + 1) * rbs0, :])
        halves = [layernorm(pltpu.unpack_elementwise(
            xu, index=k, packed_dtype=BF16, unpacked_dtype=F32)) for k in range(2)]
        blocks = [a[:, k * LANES:(k + 1) * LANES] for a in halves for k in range(3)]
        return [_force(v).astype(BF16) for v, _ in _combos(_HK_U, blocks)]

    def lhs_to_scratch(xslot):
        for q, t in enumerate(phase0_lhs(xslot, 0)):
            sb0[q] = _pack(t)

    w1_copy.start()
    if 0 in phases:
        for k in range(nu0 + 1):
            x_copy(k, k).start()
    w2_copy.start()
    ssq_ref[...] = jnp.zeros_like(ssq_ref)
    w1_copy.wait()
    for j in range(njk):
        blocks = [w1_ref[kb * LANES:(kb + 1) * LANES,
                         (l * njk + j) * LANES:(l * njk + j + 1) * LANES].astype(F32)
                  * (_LAM * math.sqrt(c))
                  for kb in range(3) for l in range(3)]
        for q, t in enumerate(_weight_sums(blocks)):
            ws_ref[q, j * (LANES // 2):(j + 1) * (LANES // 2), :] = t
    if 0 in phases:
        x_copy(0, 0).wait()
        lhs_to_scratch(0)

    def phase0_state(t0, acc, lo):
        infos = []
        for su in range(nu0):
            infos.append(unit_info(t0 + su, acc, lo))
            acc, lo = step_up(acc, lo)
        return tuple(infos), acc, lo

    def phase0_block(blk, carry):
        infos, bacc, blo, xs0 = carry
        t0 = blk * nu0
        xslots = x_slots(xs0, 2 * nu0 + 1)
        for su in range(nu0):
            tn = t0 + nu0 + 1 + su

            @pl.when(tn < ns)
            def _():
                x_copy(tn, xslots[nu0 + 1 + su]).start()

        for su in range(nu0):
            tw = t0 + 1 + su

            @pl.when(tw < ns)
            def _():
                x_copy(tw, xslots[1 + su]).wait()

        for unpinned, u, _ in infos:
            @pl.when(jnp.logical_and(unpinned, u >= ring))
            def _():
                h_out_copy(u - ring).wait()

        for su in range(nu0):
            slot = infos[su][2]
            for rb in range(st // rbs0):
                if su == 0 and rb == 0:
                    ops = [_unpack(sb0[q]) for q in range(_NPROD)]
                else:
                    ops = phase0_lhs(xslots[su], rb)
                for jc in range(njk):
                    wrows = slice(jc * (LANES // 2), (jc + 1) * (LANES // 2))
                    ms = [_lazy(lambda q=q: dot(ops[q], _unpack(ws_ref[q, wrows, :])))
                          for q in range(_NPROD)]
                    cs = _combos(_HK_WT, ms, perm0)
                    done = {}
                    for o in corder0:
                        b = _force(cs[o][0])
                        if cs[o][1] < 0:
                            b = -b
                        done[o] = b * (1.0 + jnp.tanh(b * (b * b + _KAP)))
                        l = o % 3
                        if l in done and l + 3 in done:
                            gt, gb = done[l], done[l + 3]
                            j = l * njk + jc
                            ssq_ref[j] += jnp.sum(
                                (gt * gt + gb * gb).reshape(hh // 8, 8, LANES), axis=0)
                            hs[slot, j, rb * hh:(rb + 1) * hh, :] = pltpu.pack_elementwise(
                                [gt, gb], packed_dtype=BF16)
        lhs_to_scratch(xslots[nu0])

        for unpinned, u, _ in infos:
            @pl.when(jnp.logical_and(unpinned, u < nspill))
            def _():
                h_out_copy(u).start()
        infos, bacc, blo = phase0_state(t0 + nu0, bacc, blo)
        return infos, bacc, blo, xslots[nu0]

    if 0 in phases:
        zero = jnp.int32(0)
        jax.lax.fori_loop(0, ns // nu0, phase0_block, (*phase0_state(zero, zero, zero), zero))

    if 1 in phases:
        for k in range(xd):
            x_copy(ns - 1 - k, k).start()
    w2_copy.wait()
    ssq = jnp.concatenate(
        [jnp.sum(ssq_ref[j], axis=0, keepdims=True) for j in range(nj)], axis=1)
    gx = jnp.sqrt(ssq * (_HSCALE * _HSCALE) + _GRN_EPS)
    nx = gx / (jnp.mean(gx, axis=-1, keepdims=True) + _GRN_EPS)
    s = (1.0 + g_ref[...].astype(F32) * nx) * _HSCALE
    s_t = _col(s, c4)
    kb = c4 // 3
    w2s = [w2_ref[:, l * LANES:(l + 1) * LANES].astype(F32) * s_t for l in range(3)]
    for q, t in enumerate(_weight_sums(
            [w2s[l][j * kb:(j + 1) * kb] for j in range(3) for l in range(3)])):
        ws_ref[q] = t
    bias_ref[...] = dot(jnp.broadcast_to(b_ref[...], (16, c4)), w2_ref[...])[:8]

    def phase1_state(i0, acc, lo):
        infos = []
        for su in range(nu1):
            infos.append(unit_info(ns - 1 - (i0 + su), acc, lo))
            acc, lo = step_down(acc, lo)
        return tuple(infos), acc, lo

    def phase1_block(blk, carry):
        prev, infos, bacc, blo, xs0 = carry
        hh1 = rbs1 // 2
        bias = bias_ref[0:1, :]
        i0 = blk * nu1
        xslots = x_slots(xs0, xd + nu1)
        for su in range(nu1):
            inx = i0 + su + xd

            @pl.when(jnp.logical_and(inx < ns, inx >= xr))
            def _():
                o_copy(ns - 1 - (inx - xr), xslots[su + xd]).wait()

            @pl.when(inx < ns)
            def _():
                x_copy(ns - 1 - inx, xslots[su + xd]).start()

        if not nodma:
            for unp_p, u_p, _ in prev:
                @pl.when(jnp.logical_and(unp_p, u_p >= ring))
                def _():
                    h_in_copy(u_p - ring).start()

        for su in range(nu1):
            x_copy(ns - 1 - (i0 + su), xslots[su]).wait()
            if not nodma:
                unpinned, u, _ = infos[su]

                @pl.when(jnp.logical_and(unpinned, u < nspill))
                def _():
                    h_in_copy(u).wait()

        for su in range(nu1):
            slot = infos[su][2]
            xslot = xslots[su]
            for rb in range(0 if nocomp else st // rbs1):
                r0 = rb * rbs1
                raw = [jnp.concatenate(
                    [_unpack(hs[slot, kk * njk + j,
                                (r0 + half * hh1) // 2:(r0 + (half + 1) * hh1) // 2, :])
                     for j in range(njk)], axis=1) for half in range(2) for kk in range(3)]
                lhs = _combos(_HK_U, [_lazy(lambda a=a: a.astype(F32)) for a in raw])

                def product(q):
                    nzs = [ix for ix, cf in enumerate(_HK_U[q]) if cf]
                    a = raw[nzs[0]] if len(nzs) == 1 else _force(lhs[q][0]).astype(BF16)
                    return dot(a, _unpack(ws_ref[q]))

                ms = [_lazy(functools.partial(product, q)) for q in range(_NPROD)]
                cs = _combos(_HK_WT, ms, perm1)
                for o in corder1:
                    half, l = divmod(o, 3)
                    rs = slice(r0 + half * hh1, r0 + (half + 1) * hh1)
                    cl = slice(l * LANES, (l + 1) * LANES)
                    val, sg = _force(cs[o][0]), cs[o][1]
                    base = xb[xslot, rs, cl].astype(F32) + bias[:, cl]
                    xb[xslot, rs, cl] = (base + val if sg > 0 else base - val).astype(BF16)

        for su in range(nu1):
            o_copy(ns - 1 - (i0 + su), xslots[su]).start()
        nxt, bacc, blo = phase1_state(i0 + nu1, bacc, blo)
        return infos, nxt, bacc, blo, xslots[nu1]

    if 1 in phases:
        acc0, lo0 = jnp.int32(((ns - 1) * npin) % ns), jnp.int32(((ns - 1) * npin) // ns)
        first, acc0, lo0 = phase1_state(jnp.int32(0), acc0, lo0)
        none = tuple((jnp.bool_(False), jnp.int32(0), jnp.int32(0)) for _ in range(nu1))
        jax.lax.fori_loop(0, ns // nu1, phase1_block, (none, first, acc0, lo0, jnp.int32(0)))
        for i in range(ns - xr, ns):
            o_copy(ns - 1 - i, i % xr).wait()
    else:
        o_copy(0, 0).start()
        o_copy(0, 0).wait()


def _build(n, c, c4, st=1024, nu0=2, nu1=1, ring=4, npin=35, xr=5, xd=3, vmem_mb=128,
           rbs0=128, rbs1=256,
           perm0=(6, 7, 9, 11, 3, 12, 4, 10, 13, 2, 0, 1, 5, 14, 8), corder0=(3, 0, 2, 1, 4, 5),
           perm1=(6, 4, 5, 8, 9, 7, 10, 13, 0, 11, 12, 3, 2, 14, 1), corder1=(1, 4, 2, 3, 5, 0),
           phases=(0, 1), nodma=False, nocomp=False):
    ns = n // st
    assert n % st == 0 and ns % nu0 == 0 and ns % nu1 == 0 and c == 3 * LANES and c4 % (3 * LANES) == 0
    assert ring & (ring - 1) == 0 and ring >= 2 * nu0
    assert xr >= 2 * nu0 + 1 and xr >= xd + 2 * nu1 and xd >= nu1
    kern = functools.partial(
        _kernel, st=st, nu0=nu0, nu1=nu1, ns=ns, c=c, c4=c4, ring=ring, npin=npin, xr=xr, xd=xd,
        rbs0=rbs0, rbs1=rbs1, perm0=perm0, corder0=tuple(corder0), perm1=perm1,
        corder1=tuple(corder1), phases=tuple(phases), nodma=nodma, nocomp=nocomp)
    nj = c4 // LANES
    hbm = pl.BlockSpec(memory_space=pl.ANY)
    vmem = pl.BlockSpec(memory_space=pltpu.VMEM)
    return pl.pallas_call(
        kern,
        in_specs=[hbm, vmem, hbm, hbm, vmem, vmem],
        out_specs=[hbm, hbm],
        out_shape=[
            jax.ShapeDtypeStruct((n, c), BF16),
            jax.ShapeDtypeStruct((ns - npin - ring, nj, st // 2, LANES), U32),
        ],
        scratch_shapes=[
            pltpu.VMEM((ring + npin, nj, st // 2, LANES), U32),
            pltpu.VMEM((xr, st, c), BF16),
            pltpu.VMEM((_NPROD, rbs0 // 4, LANES), U32),
            pltpu.VMEM((nj, 8, LANES), F32),
            pltpu.VMEM((_NPROD, c4 // 6, LANES), U32),
            pltpu.VMEM((8, c), F32),
            pltpu.VMEM((c, c4), BF16),
            pltpu.VMEM((c4, c), BF16),
            pltpu.SemaphoreType.DMA((ring,)),
            pltpu.SemaphoreType.DMA((xr,)),
            pltpu.SemaphoreType.DMA((xr,)),
            pltpu.SemaphoreType.DMA((2,)),
        ],
        compiler_params=pltpu.CompilerParams(
            vmem_limit_bytes=vmem_mb * 1024 * 1024,
            disable_bounds_checks=True,
        ),
    )


def _run(x, dw, w1, w2, grn_g, grn_b, **kw):
    b, hh, ww, c = x.shape
    c4 = w1.shape[1]
    n = b * hh * ww
    assert b == 1 and dw.shape[0] == 1 and dw.shape[1] == 1
    out, _ = _build(n, c, c4, **kw)(
        x.reshape(n, c), dw.reshape(1, c), w1, w2,
        grn_g.reshape(1, c4), grn_b.reshape(1, c4))
    return out.reshape(x.shape)


@jax.jit
def pallas_standalone__modern_conv_block_slak__vision_kernel(
    x: jax.Array,
    dw: jax.Array,
    w1: jax.Array,
    w2: jax.Array,
    grn_g: jax.Array,
    grn_b: jax.Array,
):
    return _run(x, dw, w1, w2, grn_g, grn_b)
```

```python
import functools
import math

import jax
import jax.numpy as jnp
import jax.experimental.pallas as pl
import jax.experimental.pallas.tpu as pltpu

F32 = jnp.float32
BF16 = jnp.bfloat16
U32 = jnp.uint32
LANES = 128

_GELU_C0 = math.sqrt(2.0 / math.pi)
_GELU_C1 = _GELU_C0 * 0.044715
_LAM = _GELU_C1 ** (1.0 / 3.0)
_KAP = _GELU_C0 / _LAM
_HSCALE = 1.0 / (2.0 * _LAM)
_LN_EPS = 1e-5
_GRN_EPS = 1e-6

_HK_U = ((0, 0, 0, 1, -1, 0), (-1, 0, 0, 0, 0, 1), (1, 0, 0, -1, 0, 0), (-1, 0, 0, 0, 0, 0),
         (0, 0, -1, 0, 0, 1), (1, 0, 0, -1, 1, 0), (0, -1, 0, 0, 0, 0), (0, -1, 1, 0, 0, -1),
         (0, 1, -1, 0, 0, 0), (1, 0, -1, 0, 0, 0), (0, 0, 0, 0, -1, 0), (0, 0, 0, -1, 0, 1),
         (0, 1, -1, 0, -1, 1), (-1, 1, 0, 1, -1, 0), (0, 0, 0, 0, 0, 1))
_HK_V = ((0, 0, 1, 0, 0, 0, 0, 0, 0), (0, -1, 0, 0, 0, 0, 1, 0, 0), (1, 1, 0, 1, 0, 0, 0, 0, 0),
         (1, 0, -1, 0, 0, 0, 1, 0, 0), (0, 0, 0, 0, 1, 0, 1, 1, 0), (0, 0, 1, 1, 0, 0, 0, 0, 0),
         (0, 0, 0, -1, 0, 1, 0, 0, 1), (0, 0, 0, 0, -1, 0, 0, 0, -1), (0, 0, 0, 0, 0, 0, 0, 0, 1),
         (0, 0, 0, 0, 0, 0, 1, 0, 0), (0, 0, 1, 0, -1, 1, 0, 0, 0), (0, -1, 0, 0, 0, 0, 0, 0, 0),
         (0, 0, 0, 0, -1, 0, 0, 0, 0), (0, 0, 0, 1, 0, 0, 0, 0, 0), (0, -1, 0, 0, 0, 0, 0, -1, 1))
_HK_W = ((1, 0, 1, 1, 0, 1), (0, 1, 0, 1, 0, 0), (0, 0, 0, -1, 0, 0), (-1, 0, 0, -1, 0, 0),
         (0, -1, 0, 0, 0, 0), (1, 0, 1, 1, 0, 0), (0, 0, -1, 0, 0, 0), (0, 1, 0, 0, 1, 1),
         (0, -1, -1, 0, -1, -1), (-1, 1, 0, 0, 0, 0), (0, 0, 0, 0, 0, -1), (0, 0, 0, -1, 1, 0),
         (0, 0, 0, 0, 1, 1), (1, 0, 1, 0, 0, 0), (0, -1, 0, 0, -1, 0))
_HK_WT = tuple(tuple(w[o] for w in _HK_W) for o in range(6))
_NPROD = len(_HK_U)


class _lazy:
    def __init__(self, fn):
        self.fn, self.val = fn, None


def _force(v):
    if isinstance(v, _lazy):
        if v.val is None:
            v.val = v.fn()
        return v.val
    return v


def _combos(rows, vals, perm=None):
    vals = list(vals)
    rank = list(perm) if perm is not None else list(range(len(vals)))
    rows = [{i: c for i, c in enumerate(r) if c} for r in rows]
    while True:
        cnt = {}
        for r in rows:
            ks = sorted(r, key=lambda i: rank[i])
            for ia, a in enumerate(ks):
                for b in ks[ia + 1:]:
                    key = (a, b, r[a] * r[b])
                    cnt[key] = cnt.get(key, 0) + 1
        if not cnt or max(cnt.values()) < 2:
            break
        a, b, sg = max(sorted(cnt, key=lambda k_: (rank[k_[0]], rank[k_[1]], k_[2])),
                       key=lambda k_: cnt[k_])
        vals.append(_lazy(lambda a=a, b=b, sg=sg: (
            _force(vals[a]) + _force(vals[b]) if sg > 0 else _force(vals[a]) - _force(vals[b]))))
        rank.append(max(rank[a], rank[b]) + 0.5)
        new = len(vals) - 1
        for r in rows:
            if a in r and b in r and r[a] * r[b] == sg:
                r[new] = r.pop(a)
                del r[b]

    def total(items, sign):
        acc = _force(vals[items[0][0]])
        for idx, cf in items[1:]:
            acc = acc + _force(vals[idx]) if cf * sign > 0 else acc - _force(vals[idx])
        return acc

    out = []
    for r in rows:
        items = sorted(r.items(), key=lambda kv: rank[kv[0]])
        pos = [i for i, kv in enumerate(items) if kv[1] > 0]
        if pos and pos[0] > 0:
            items.insert(0, items.pop(pos[0]))
        sign = items[0][1]
        out.append((_lazy(functools.partial(total, items, sign)), sign))
    return out


_HK_USIGN = tuple(sg for _, sg in _combos(_HK_U, [1.0] * 6))


def _weight_sums(blocks):
    res = []
    for q, (t, sg) in enumerate(_combos(_HK_V, blocks)):
        t = _force(t)
        res.append(_pack((t if sg * _HK_USIGN[q] > 0 else -t).astype(BF16)))
    return res


def _col(row, n):
    return jnp.transpose(jnp.broadcast_to(row, (LANES, n)))


def _pack(v):
    return pltpu.bitcast(v, U32)


def _unpack(v):
    return pltpu.bitcast(v, BF16)


def _kernel(x_hbm, dw_ref, w1_hbm, w2_hbm, g_ref, b_ref,
            o_hbm, h_hbm,
            hs, xb, sb0, ssq_ref, ws_ref, bias_ref, w1_ref, w2_ref,
            sem_h, sem_x, sem_o, sem_w,
            *, st, nu0, nu1, ns, c, c4, ring, npin, xr, xd, rbs0, rbs1,
            perm0, corder0, perm1, corder1, phases, nodma, nocomp, aoff):
    nj = c4 // LANES
    njk = nj // 3
    nspill = ns - npin - ring
    dot = functools.partial(jnp.dot, preferred_element_type=F32)

    def wrap_ring(u):
        return u & (ring - 1)

    def unit_info(t, acc, lo):
        unpinned = acc + npin < ns
        u = t - lo
        return unpinned, u, jnp.where(unpinned, wrap_ring(u), ring + lo)

    def step_up(acc, lo):
        acc = acc + npin
        wrap = acc >= ns
        return jnp.where(wrap, acc - ns, acc), jnp.where(wrap, lo + 1, lo)

    def step_down(acc, lo):
        acc = acc - npin
        wrap = acc < 0
        return jnp.where(wrap, acc + ns, acc), jnp.where(wrap, lo - 1, lo)

    def x_slots(first, n, step):
        res = [first]
        for _ in range(n - 1):
            nxt = res[-1] + step
            res.append(jnp.where(nxt >= xr, nxt - xr, jnp.where(nxt < 0, nxt + xr, nxt)))
        return res

    def h_out_copy(u):
        return pltpu.make_async_copy(hs.at[wrap_ring(u)], h_hbm.at[u], sem_h.at[wrap_ring(u)])

    def h_in_copy(u):
        return pltpu.make_async_copy(h_hbm.at[u], hs.at[wrap_ring(u)], sem_h.at[wrap_ring(u)])

    def x_copy(t, slot):
        return pltpu.make_async_copy(x_hbm.at[pl.ds(t * st, st), :], xb.at[slot], sem_x.at[slot])

    def o_copy(t, slot):
        return pltpu.make_async_copy(xb.at[slot], o_hbm.at[pl.ds(t * st, st), :], sem_o.at[slot])

    w1_copy = pltpu.make_async_copy(w1_hbm, w1_ref, sem_w.at[0])
    w2_copy = pltpu.make_async_copy(w2_hbm, w2_ref, sem_w.at[1])

    hh = rbs0 // 2

    def phase0_lhs(xslot, rb):
        dw = dw_ref[...].astype(F32)

        def layernorm(xf):
            y = xf * dw
            yc = y - jnp.sum(y, axis=-1, keepdims=True) * (1.0 / c)
            ss = jnp.sum(yc * yc, axis=-1, keepdims=True)
            return yc * jnp.exp2(jnp.log(ss + c * _LN_EPS) * (-0.5 / math.log(2.0)))

        xu = _pack(xb[xslot, rb * rbs0:(rb + 1) * rbs0, :])
        halves = [layernorm(pltpu.unpack_elementwise(
            xu, index=k, packed_dtype=BF16, unpacked_dtype=F32)) for k in range(2)]
        blocks = [a[:, k * LANES:(k + 1) * LANES] for a in halves for k in range(3)]
        return [_force(v).astype(BF16) for v, _ in _combos(_HK_U, blocks)]

    def lhs_to_scratch(xslot):
        for q, t in enumerate(phase0_lhs(xslot, 0)):
            sb0[q] = _pack(t)

    w1_copy.start()
    if 0 in phases:
        for k in range(nu0 + 1):
            x_copy(k, k).start()
    w2_copy.start()
    ssq_ref[...] = jnp.zeros_like(ssq_ref)
    w1_copy.wait()
    for j in range(njk):
        blocks = [w1_ref[kb * LANES:(kb + 1) * LANES,
                         (l * njk + j) * LANES:(l * njk + j + 1) * LANES].astype(F32)
                  * (_LAM * math.sqrt(c))
                  for kb in range(3) for l in range(3)]
        for q, t in enumerate(_weight_sums(blocks)):
            ws_ref[q, j * (LANES // 2):(j + 1) * (LANES // 2), :] = t
    if 0 in phases:
        x_copy(0, 0).wait()
        lhs_to_scratch(0)

    def phase0_state(t0, acc, lo):
        infos = []
        for su in range(nu0):
            infos.append(unit_info(t0 + su, acc, lo))
            acc, lo = step_up(acc, lo)
        return tuple(infos), acc, lo

    def phase0_block(blk, carry):
        infos, bacc, blo, xs0 = carry
        t0 = blk * nu0
        xslots = x_slots(xs0, 2 * nu0 + 1, 1)
        for su in range(nu0):
            tn = t0 + nu0 + 1 + su

            @pl.when(tn < ns)
            def _():
                x_copy(tn, xslots[nu0 + 1 + su]).start()

        for su in range(nu0):
            tw = t0 + 1 + su

            @pl.when(tw < ns)
            def _():
                x_copy(tw, xslots[1 + su]).wait()

        for unpinned, u, _ in infos:
            @pl.when(jnp.logical_and(unpinned, u >= ring))
            def _():
                h_out_copy(u - ring).wait()

        for su in range(nu0):
            slot = infos[su][2]
            for rb in range(st // rbs0):
                if su == 0 and rb == 0:
                    ops = [_unpack(sb0[q]) for q in range(_NPROD)]
                else:
                    ops = phase0_lhs(xslots[su], rb)
                for jc in range(njk):
                    wrows = slice(jc * (LANES // 2), (jc + 1) * (LANES // 2))
                    ms = [_lazy(lambda q=q: dot(ops[q], _unpack(ws_ref[q, wrows, :])))
                          for q in range(_NPROD)]
                    cs = _combos(_HK_WT, ms, perm0)
                    done = {}
                    for o in corder0:
                        b = _force(cs[o][0])
                        if cs[o][1] < 0:
                            b = -b
                        done[o] = b * (1.0 + jnp.tanh(b * (b * b + _KAP)))
                        l = o % 3
                        if l in done and l + 3 in done:
                            gt, gb = done[l], done[l + 3]
                            j = l * njk + jc
                            ssq_ref[j] += jnp.sum(
                                (gt * gt + gb * gb).reshape(hh // 8, 8, LANES), axis=0)
                            hs[slot, j, rb * hh:(rb + 1) * hh, :] = pltpu.pack_elementwise(
                                [gt, gb], packed_dtype=BF16)
        lhs_to_scratch(xslots[nu0])

        for unpinned, u, _ in infos:
            @pl.when(jnp.logical_and(unpinned, u < nspill))
            def _():
                h_out_copy(u).start()
        infos, bacc, blo = phase0_state(t0 + nu0, bacc, blo)
        return infos, bacc, blo, xslots[nu0]

    if 0 in phases:
        zero = jnp.int32(0)
        jax.lax.fori_loop(0, ns // nu0, phase0_block,
                          (*phase0_state(zero, jnp.int32(aoff), zero), zero))

    if phases == (1,):
        for t in range(ns - xr, ns):
            x_copy(t, t % xr).start()
            x_copy(t, t % xr).wait()
    w2_copy.wait()
    ssq = jnp.concatenate(
        [jnp.sum(ssq_ref[j], axis=0, keepdims=True) for j in range(nj)], axis=1)
    gx = jnp.sqrt(ssq * (_HSCALE * _HSCALE) + _GRN_EPS)
    nx = gx / (jnp.mean(gx, axis=-1, keepdims=True) + _GRN_EPS)
    s = (1.0 + g_ref[...].astype(F32) * nx) * _HSCALE
    s_t = _col(s, c4)
    kb = c4 // 3
    w2s = [w2_ref[:, l * LANES:(l + 1) * LANES].astype(F32) * s_t for l in range(3)]
    for q, t in enumerate(_weight_sums(
            [w2s[l][j * kb:(j + 1) * kb] for j in range(3) for l in range(3)])):
        ws_ref[q] = t
    bias_ref[...] = dot(jnp.broadcast_to(b_ref[...], (16, c4)), w2_ref[...])[:8]

    def phase1_state(i0, acc, lo):
        infos = []
        for su in range(nu1):
            infos.append(unit_info(ns - 1 - (i0 + su), acc, lo))
            acc, lo = step_down(acc, lo)
        return tuple(infos), acc, lo

    def phase1_block(blk, carry):
        prev, infos, bacc, blo, xs0 = carry
        hh1 = rbs1 // 2
        bias = bias_ref[0:1, :]
        i0 = blk * nu1
        xslots = x_slots(xs0, xd + nu1, -1)
        for su in range(nu1):
            inx = i0 + su + xd

            @pl.when(jnp.logical_and(inx < ns, inx >= xr))
            def _():
                o_copy(ns - 1 - (inx - xr), xslots[su + xd]).wait()
                x_copy(ns - 1 - inx, xslots[su + xd]).start()

        if not nodma:
            for unp_p, u_p, _ in prev:
                @pl.when(jnp.logical_and(unp_p, u_p >= ring))
                def _():
                    h_in_copy(u_p - ring).start()

        for su in range(nu1):
            @pl.when(i0 + su >= xr)
            def _():
                x_copy(ns - 1 - (i0 + su), xslots[su]).wait()

            if not nodma:
                unpinned, u, _ = infos[su]

                @pl.when(jnp.logical_and(unpinned, u < nspill))
                def _():
                    h_in_copy(u).wait()

        for su in range(nu1):
            slot = infos[su][2]
            xslot = xslots[su]
            for rb in range(0 if nocomp else st // rbs1):
                r0 = rb * rbs1
                raw = [jnp.concatenate(
                    [_unpack(hs[slot, kk * njk + j,
                                (r0 + half * hh1) // 2:(r0 + (half + 1) * hh1) // 2, :])
                     for j in range(njk)], axis=1) for half in range(2) for kk in range(3)]
                lhs = _combos(_HK_U, [_lazy(lambda a=a: a.astype(F32)) for a in raw])

                def product(q):
                    nzs = [ix for ix, cf in enumerate(_HK_U[q]) if cf]
                    a = raw[nzs[0]] if len(nzs) == 1 else _force(lhs[q][0]).astype(BF16)
                    return dot(a, _unpack(ws_ref[q]))

                ms = [_lazy(functools.partial(product, q)) for q in range(_NPROD)]
                cs = _combos(_HK_WT, ms, perm1)
                for o in corder1:
                    half, l = divmod(o, 3)
                    rs = slice(r0 + half * hh1, r0 + (half + 1) * hh1)
                    cl = slice(l * LANES, (l + 1) * LANES)
                    val, sg = _force(cs[o][0]), cs[o][1]
                    base = xb[xslot, rs, cl].astype(F32) + bias[:, cl]
                    xb[xslot, rs, cl] = (base + val if sg > 0 else base - val).astype(BF16)

        for su in range(nu1):
            o_copy(ns - 1 - (i0 + su), xslots[su]).start()
        nxt, bacc, blo = phase1_state(i0 + nu1, bacc, blo)
        return infos, nxt, bacc, blo, xslots[nu1]

    if 1 in phases:
        acc0, lo0 = (jnp.int32(v) for v in divmod((ns - 1) * npin + aoff, ns)[::-1])
        first, acc0, lo0 = phase1_state(jnp.int32(0), acc0, lo0)
        none = tuple((jnp.bool_(False), jnp.int32(0), jnp.int32(0)) for _ in range(nu1))
        jax.lax.fori_loop(0, ns // nu1, phase1_block,
                          (none, first, acc0, lo0, jnp.int32((ns - 1) % xr)))
        for t in range(xr):
            o_copy(t, t % xr).wait()
    else:
        o_copy(0, 0).start()
        o_copy(0, 0).wait()


def _build(n, c, c4, st=1024, nu0=2, nu1=1, ring=4, npin=35, xr=5, xd=3, vmem_mb=128,
           rbs0=128, rbs1=256,
           perm0=(6, 7, 9, 11, 3, 12, 4, 10, 13, 2, 0, 1, 5, 14, 8), corder0=(3, 0, 2, 1, 4, 5),
           perm1=(6, 4, 5, 8, 9, 7, 10, 13, 0, 11, 12, 3, 2, 14, 1), corder1=(1, 4, 2, 3, 5, 0),
           phases=(0, 1), nodma=False, nocomp=False, aoff=72):
    ns = n // st
    assert n % st == 0 and ns % nu0 == 0 and ns % nu1 == 0 and c == 3 * LANES and c4 % (3 * LANES) == 0
    assert ring & (ring - 1) == 0 and ring >= 2 * nu0
    assert xr >= 2 * nu0 + 1 and xr >= xd + 2 * nu1 and xd >= nu1
    kern = functools.partial(
        _kernel, st=st, nu0=nu0, nu1=nu1, ns=ns, c=c, c4=c4, ring=ring, npin=npin, xr=xr, xd=xd,
        rbs0=rbs0, rbs1=rbs1, perm0=perm0, corder0=tuple(corder0), perm1=perm1,
        corder1=tuple(corder1), phases=tuple(phases), nodma=nodma, nocomp=nocomp, aoff=aoff)
    nj = c4 // LANES
    hbm = pl.BlockSpec(memory_space=pl.ANY)
    vmem = pl.BlockSpec(memory_space=pltpu.VMEM)
    return pl.pallas_call(
        kern,
        in_specs=[hbm, vmem, hbm, hbm, vmem, vmem],
        out_specs=[hbm, hbm],
        out_shape=[
            jax.ShapeDtypeStruct((n, c), BF16),
            jax.ShapeDtypeStruct((ns - npin - ring, nj, st // 2, LANES), U32),
        ],
        scratch_shapes=[
            pltpu.VMEM((ring + npin, nj, st // 2, LANES), U32),
            pltpu.VMEM((xr, st, c), BF16),
            pltpu.VMEM((_NPROD, rbs0 // 4, LANES), U32),
            pltpu.VMEM((nj, 8, LANES), F32),
            pltpu.VMEM((_NPROD, c4 // 6, LANES), U32),
            pltpu.VMEM((8, c), F32),
            pltpu.VMEM((c, c4), BF16),
            pltpu.VMEM((c4, c), BF16),
            pltpu.SemaphoreType.DMA((ring,)),
            pltpu.SemaphoreType.DMA((xr,)),
            pltpu.SemaphoreType.DMA((xr,)),
            pltpu.SemaphoreType.DMA((2,)),
        ],
        compiler_params=pltpu.CompilerParams(
            vmem_limit_bytes=vmem_mb * 1024 * 1024,
            disable_bounds_checks=True,
        ),
    )


def _run(x, dw, w1, w2, grn_g, grn_b, **kw):
    b, hh, ww, c = x.shape
    c4 = w1.shape[1]
    n = b * hh * ww
    assert b == 1 and dw.shape[0] == 1 and dw.shape[1] == 1
    out, _ = _build(n, c, c4, **kw)(
        x.reshape(n, c), dw.reshape(1, c), w1, w2,
        grn_g.reshape(1, c4), grn_b.reshape(1, c4))
    return out.reshape(x.shape)


@jax.jit
def pallas_standalone__modern_conv_block_slak__vision_kernel(
    x: jax.Array,
    dw: jax.Array,
    w1: jax.Array,
    w2: jax.Array,
    grn_g: jax.Array,
    grn_b: jax.Array,
):
    return _run(x, dw, w1, w2, grn_g, grn_b)
```

```python
import functools
import math

import jax
import jax.numpy as jnp
import jax.experimental.pallas as pl
import jax.experimental.pallas.tpu as pltpu

F32 = jnp.float32
BF16 = jnp.bfloat16
U32 = jnp.uint32
LANES = 128

_GELU_C0 = math.sqrt(2.0 / math.pi)
_GELU_C1 = _GELU_C0 * 0.044715
_LAM = _GELU_C1 ** (1.0 / 3.0)
_KAP = _GELU_C0 / _LAM
_HSCALE = 1.0 / (2.0 * _LAM)
_LN_EPS = 1e-5
_GRN_EPS = 1e-6

_HK_U = ((0, 0, 0, 1, -1, 0), (-1, 0, 0, 0, 0, 1), (1, 0, 0, -1, 0, 0), (-1, 0, 0, 0, 0, 0),
         (0, 0, -1, 0, 0, 1), (1, 0, 0, -1, 1, 0), (0, -1, 0, 0, 0, 0), (0, -1, 1, 0, 0, -1),
         (0, 1, -1, 0, 0, 0), (1, 0, -1, 0, 0, 0), (0, 0, 0, 0, -1, 0), (0, 0, 0, -1, 0, 1),
         (0, 1, -1, 0, -1, 1), (-1, 1, 0, 1, -1, 0), (0, 0, 0, 0, 0, 1))
_HK_V = ((0, 0, 1, 0, 0, 0, 0, 0, 0), (0, -1, 0, 0, 0, 0, 1, 0, 0), (1, 1, 0, 1, 0, 0, 0, 0, 0),
         (1, 0, -1, 0, 0, 0, 1, 0, 0), (0, 0, 0, 0, 1, 0, 1, 1, 0), (0, 0, 1, 1, 0, 0, 0, 0, 0),
         (0, 0, 0, -1, 0, 1, 0, 0, 1), (0, 0, 0, 0, -1, 0, 0, 0, -1), (0, 0, 0, 0, 0, 0, 0, 0, 1),
         (0, 0, 0, 0, 0, 0, 1, 0, 0), (0, 0, 1, 0, -1, 1, 0, 0, 0), (0, -1, 0, 0, 0, 0, 0, 0, 0),
         (0, 0, 0, 0, -1, 0, 0, 0, 0), (0, 0, 0, 1, 0, 0, 0, 0, 0), (0, -1, 0, 0, 0, 0, 0, -1, 1))
_HK_W = ((1, 0, 1, 1, 0, 1), (0, 1, 0, 1, 0, 0), (0, 0, 0, -1, 0, 0), (-1, 0, 0, -1, 0, 0),
         (0, -1, 0, 0, 0, 0), (1, 0, 1, 1, 0, 0), (0, 0, -1, 0, 0, 0), (0, 1, 0, 0, 1, 1),
         (0, -1, -1, 0, -1, -1), (-1, 1, 0, 0, 0, 0), (0, 0, 0, 0, 0, -1), (0, 0, 0, -1, 1, 0),
         (0, 0, 0, 0, 1, 1), (1, 0, 1, 0, 0, 0), (0, -1, 0, 0, -1, 0))
_HK_WT = tuple(tuple(w[o] for w in _HK_W) for o in range(6))
_NPROD = len(_HK_U)


class _lazy:
    def __init__(self, fn):
        self.fn, self.val = fn, None


def _force(v):
    if isinstance(v, _lazy):
        if v.val is None:
            v.val = v.fn()
        return v.val
    return v


def _combos(rows, vals, perm=None):
    vals = list(vals)
    rank = list(perm) if perm is not None else list(range(len(vals)))
    rows = [{i: c for i, c in enumerate(r) if c} for r in rows]
    while True:
        cnt = {}
        for r in rows:
            ks = sorted(r, key=lambda i: rank[i])
            for ia, a in enumerate(ks):
                for b in ks[ia + 1:]:
                    key = (a, b, r[a] * r[b])
                    cnt[key] = cnt.get(key, 0) + 1
        if not cnt or max(cnt.values()) < 2:
            break
        a, b, sg = max(sorted(cnt, key=lambda k_: (rank[k_[0]], rank[k_[1]], k_[2])),
                       key=lambda k_: cnt[k_])
        vals.append(_lazy(lambda a=a, b=b, sg=sg: (
            _force(vals[a]) + _force(vals[b]) if sg > 0 else _force(vals[a]) - _force(vals[b]))))
        rank.append(max(rank[a], rank[b]) + 0.5)
        new = len(vals) - 1
        for r in rows:
            if a in r and b in r and r[a] * r[b] == sg:
                r[new] = r.pop(a)
                del r[b]

    def total(items, sign):
        acc = _force(vals[items[0][0]])
        for idx, cf in items[1:]:
            acc = acc + _force(vals[idx]) if cf * sign > 0 else acc - _force(vals[idx])
        return acc

    out = []
    for r in rows:
        items = sorted(r.items(), key=lambda kv: rank[kv[0]])
        pos = [i for i, kv in enumerate(items) if kv[1] > 0]
        if pos and pos[0] > 0:
            items.insert(0, items.pop(pos[0]))
        sign = items[0][1]
        out.append((_lazy(functools.partial(total, items, sign)), sign))
    return out


_HK_USIGN = tuple(sg for _, sg in _combos(_HK_U, [1.0] * 6))


def _weight_sums(blocks):
    res = []
    for q, (t, sg) in enumerate(_combos(_HK_V, blocks)):
        t = _force(t)
        res.append(_pack((t if sg * _HK_USIGN[q] > 0 else -t).astype(BF16)))
    return res


def _col(row, n):
    return jnp.transpose(jnp.broadcast_to(row, (LANES, n)))


def _pack(v):
    return pltpu.bitcast(v, U32)


def _unpack(v):
    return pltpu.bitcast(v, BF16)


def _kernel(x_hbm, dw_ref, w1_hbm, w2_hbm, g_ref, b_ref,
            o_hbm, h_hbm,
            hs, xb, sb0, ssq_ref, ws_ref, bias_ref, w1_ref, w2_ref,
            sem_h, sem_x, sem_o, sem_w,
            *, st, nu0, nu1, ns, c, c4, ring, npin, xr, xd, rbs0, rbs1,
            perm0, corder0, perm1, corder1, phases, nodma, nocomp, aoff):
    nj = c4 // LANES
    njk = nj // 3
    nspill = ns - npin - ring
    dot = functools.partial(jnp.dot, preferred_element_type=F32)

    def wrap_ring(u):
        return u & (ring - 1)

    def unit_info(t, acc, lo):
        unpinned = acc + npin < ns
        u = t - lo
        return unpinned, u, jnp.where(unpinned, wrap_ring(u), ring + lo)

    def step_up(acc, lo):
        acc = acc + npin
        wrap = acc >= ns
        return jnp.where(wrap, acc - ns, acc), jnp.where(wrap, lo + 1, lo)

    def step_down(acc, lo):
        acc = acc - npin
        wrap = acc < 0
        return jnp.where(wrap, acc + ns, acc), jnp.where(wrap, lo - 1, lo)

    def x_slots(first, n, step):
        res = [first]
        for _ in range(n - 1):
            nxt = res[-1] + step
            res.append(jnp.where(nxt >= xr, nxt - xr, jnp.where(nxt < 0, nxt + xr, nxt)))
        return res

    def h_out_copy(u):
        return pltpu.make_async_copy(hs.at[wrap_ring(u)], h_hbm.at[u], sem_h.at[wrap_ring(u)])

    def h_in_copy(u):
        return pltpu.make_async_copy(h_hbm.at[u], hs.at[wrap_ring(u)], sem_h.at[wrap_ring(u)])

    def x_copy(t, slot):
        return pltpu.make_async_copy(x_hbm.at[pl.ds(t * st, st), :], xb.at[slot], sem_x.at[slot])

    def o_copy(t, slot):
        return pltpu.make_async_copy(xb.at[slot], o_hbm.at[pl.ds(t * st, st), :], sem_o.at[slot])

    w1_copy = pltpu.make_async_copy(w1_hbm, w1_ref, sem_w.at[0])
    w2_copy = pltpu.make_async_copy(w2_hbm, w2_ref, sem_w.at[1])

    hh = rbs0 // 2

    def phase0_lhs(xslot, rb):
        dw = dw_ref[...].astype(F32)

        def layernorm(xf):
            y = xf * dw
            yc = y - jnp.sum(y, axis=-1, keepdims=True) * (1.0 / c)
            ss = jnp.sum(yc * yc, axis=-1, keepdims=True)
            return yc * jnp.exp2(jnp.log(ss + c * _LN_EPS) * (-0.5 / math.log(2.0)))

        xu = _pack(xb[xslot, rb * rbs0:(rb + 1) * rbs0, :])
        halves = [layernorm(pltpu.unpack_elementwise(
            xu, index=k, packed_dtype=BF16, unpacked_dtype=F32)) for k in range(2)]
        blocks = [a[:, k * LANES:(k + 1) * LANES] for a in halves for k in range(3)]
        return [_force(v).astype(BF16) for v, _ in _combos(_HK_U, blocks)]

    def lhs_to_scratch(xslot):
        for q, t in enumerate(phase0_lhs(xslot, 0)):
            sb0[q] = _pack(t)

    w1_copy.start()
    if 0 in phases:
        for k in range(nu0 + 1):
            x_copy(k, k).start()
    w2_copy.start()
    ssq_ref[...] = jnp.zeros_like(ssq_ref)
    w1_copy.wait()
    for j in range(njk):
        blocks = [w1_ref[kb * LANES:(kb + 1) * LANES,
                         (l * njk + j) * LANES:(l * njk + j + 1) * LANES].astype(F32)
                  * (_LAM * math.sqrt(c))
                  for kb in range(3) for l in range(3)]
        for q, t in enumerate(_weight_sums(blocks)):
            ws_ref[q, j * (LANES // 2):(j + 1) * (LANES // 2), :] = t
    if 0 in phases:
        x_copy(0, 0).wait()
        lhs_to_scratch(0)

    def phase0_state(t0, acc, lo):
        infos = []
        for su in range(nu0):
            infos.append(unit_info(t0 + su, acc, lo))
            acc, lo = step_up(acc, lo)
        return tuple(infos), acc, lo

    def phase0_block(blk, carry):
        infos, bacc, blo, xs0 = carry
        t0 = blk * nu0
        xslots = x_slots(xs0, 2 * nu0 + 1, 1)
        for su in range(nu0):
            tn = t0 + nu0 + 1 + su

            @pl.when(tn < ns)
            def _():
                x_copy(tn, xslots[nu0 + 1 + su]).start()

        for su in range(nu0):
            tw = t0 + 1 + su

            @pl.when(tw < ns)
            def _():
                x_copy(tw, xslots[1 + su]).wait()

        for unpinned, u, _ in infos:
            @pl.when(jnp.logical_and(unpinned, u >= ring))
            def _():
                h_out_copy(u - ring).wait()

        for su in range(nu0):
            slot = infos[su][2]
            for rb in range(st // rbs0):
                if su == 0 and rb == 0:
                    ops = [_unpack(sb0[q]) for q in range(_NPROD)]
                else:
                    ops = phase0_lhs(xslots[su], rb)
                for jc in range(njk):
                    wrows = slice(jc * (LANES // 2), (jc + 1) * (LANES // 2))
                    ms = [_lazy(lambda q=q: dot(ops[q], _unpack(ws_ref[q, wrows, :])))
                          for q in range(_NPROD)]
                    cs = _combos(_HK_WT, ms, perm0)
                    done = {}
                    for o in corder0:
                        b = _force(cs[o][0])
                        if cs[o][1] < 0:
                            b = -b
                        done[o] = b * (1.0 + jnp.tanh(b * (b * b + _KAP)))
                        l = o % 3
                        if l in done and l + 3 in done:
                            gt, gb = done[l], done[l + 3]
                            j = l * njk + jc
                            ssq_ref[j] += jnp.sum(
                                (gt * gt + gb * gb).reshape(hh // 8, 8, LANES), axis=0)
                            hs[slot, j, rb * hh:(rb + 1) * hh, :] = pltpu.pack_elementwise(
                                [gt, gb], packed_dtype=BF16)
        lhs_to_scratch(xslots[nu0])

        for unpinned, u, _ in infos:
            @pl.when(jnp.logical_and(unpinned, u < nspill))
            def _():
                h_out_copy(u).start()
        infos, bacc, blo = phase0_state(t0 + nu0, bacc, blo)
        return infos, bacc, blo, xslots[nu0]

    if 0 in phases:
        zero = jnp.int32(0)
        jax.lax.fori_loop(0, ns // nu0, phase0_block,
                          (*phase0_state(zero, jnp.int32(aoff), zero), zero))

    if phases == (1,):
        for t in range(ns - xr, ns):
            x_copy(t, t % xr).start()
            x_copy(t, t % xr).wait()
    w2_copy.wait()
    ssq = jnp.concatenate(
        [jnp.sum(ssq_ref[j], axis=0, keepdims=True) for j in range(nj)], axis=1)
    gx = jnp.sqrt(ssq * (_HSCALE * _HSCALE) + _GRN_EPS)
    nx = gx / (jnp.mean(gx, axis=-1, keepdims=True) + _GRN_EPS)
    s = (1.0 + g_ref[...].astype(F32).reshape(1, c4) * nx) * _HSCALE
    s_t = _col(s, c4)
    kb = c4 // 3
    w2s = [w2_ref[:, l * LANES:(l + 1) * LANES].astype(F32) * s_t for l in range(3)]
    for q, t in enumerate(_weight_sums(
            [w2s[l][j * kb:(j + 1) * kb] for j in range(3) for l in range(3)])):
        ws_ref[q] = t
    grn_b = b_ref[...].astype(F32).reshape(1, c4)
    bias_ref[...] = dot(jnp.broadcast_to(grn_b, (16, c4)).astype(BF16), w2_ref[...])[:8]

    def phase1_state(i0, acc, lo):
        infos = []
        for su in range(nu1):
            infos.append(unit_info(ns - 1 - (i0 + su), acc, lo))
            acc, lo = step_down(acc, lo)
        return tuple(infos), acc, lo

    def phase1_block(blk, carry):
        prev, infos, bacc, blo, xs0 = carry
        hh1 = rbs1 // 2
        bias = bias_ref[0:1, :]
        i0 = blk * nu1
        xslots = x_slots(xs0, xd + nu1, -1)
        for su in range(nu1):
            inx = i0 + su + xd

            @pl.when(jnp.logical_and(inx < ns, inx >= xr))
            def _():
                o_copy(ns - 1 - (inx - xr), xslots[su + xd]).wait()
                x_copy(ns - 1 - inx, xslots[su + xd]).start()

        if not nodma:
            for unp_p, u_p, _ in prev:
                @pl.when(jnp.logical_and(unp_p, u_p >= ring))
                def _():
                    h_in_copy(u_p - ring).start()

        for su in range(nu1):
            @pl.when(i0 + su >= xr)
            def _():
                x_copy(ns - 1 - (i0 + su), xslots[su]).wait()

            if not nodma:
                unpinned, u, _ = infos[su]

                @pl.when(jnp.logical_and(unpinned, u < nspill))
                def _():
                    h_in_copy(u).wait()

        for su in range(nu1):
            slot = infos[su][2]
            xslot = xslots[su]
            for rb in range(0 if nocomp else st // rbs1):
                r0 = rb * rbs1
                raw = [jnp.concatenate(
                    [_unpack(hs[slot, kk * njk + j,
                                (r0 + half * hh1) // 2:(r0 + (half + 1) * hh1) // 2, :])
                     for j in range(njk)], axis=1) for half in range(2) for kk in range(3)]
                lhs = _combos(_HK_U, [_lazy(lambda a=a: a.astype(F32)) for a in raw])

                def product(q):
                    nzs = [ix for ix, cf in enumerate(_HK_U[q]) if cf]
                    a = raw[nzs[0]] if len(nzs) == 1 else _force(lhs[q][0]).astype(BF16)
                    return dot(a, _unpack(ws_ref[q]))

                ms = [_lazy(functools.partial(product, q)) for q in range(_NPROD)]
                cs = _combos(_HK_WT, ms, perm1)
                for o in corder1:
                    half, l = divmod(o, 3)
                    rs = slice(r0 + half * hh1, r0 + (half + 1) * hh1)
                    cl = slice(l * LANES, (l + 1) * LANES)
                    val, sg = _force(cs[o][0]), cs[o][1]
                    base = xb[xslot, rs, cl].astype(F32) + bias[:, cl]
                    xb[xslot, rs, cl] = (base + val if sg > 0 else base - val).astype(BF16)

        for su in range(nu1):
            o_copy(ns - 1 - (i0 + su), xslots[su]).start()
        nxt, bacc, blo = phase1_state(i0 + nu1, bacc, blo)
        return infos, nxt, bacc, blo, xslots[nu1]

    if 1 in phases:
        acc0, lo0 = (jnp.int32(v) for v in divmod((ns - 1) * npin + aoff, ns)[::-1])
        first, acc0, lo0 = phase1_state(jnp.int32(0), acc0, lo0)
        none = tuple((jnp.bool_(False), jnp.int32(0), jnp.int32(0)) for _ in range(nu1))
        jax.lax.fori_loop(0, ns // nu1, phase1_block,
                          (none, first, acc0, lo0, jnp.int32((ns - 1) % xr)))
        for t in range(xr):
            o_copy(t, t % xr).wait()
    else:
        o_copy(0, 0).start()
        o_copy(0, 0).wait()


def _build(n, c, c4, st=1024, nu0=2, nu1=1, ring=4, npin=35, xr=5, xd=3, vmem_mb=128,
           rbs0=128, rbs1=256,
           perm0=(6, 7, 9, 11, 3, 12, 4, 10, 13, 2, 0, 1, 5, 14, 8), corder0=(3, 0, 2, 1, 4, 5),
           perm1=(6, 4, 5, 8, 9, 7, 10, 13, 0, 11, 12, 3, 2, 14, 1), corder1=(1, 4, 2, 3, 5, 0),
           phases=(0, 1), nodma=False, nocomp=False, aoff=72):
    ns = n // st
    assert n % st == 0 and ns % nu0 == 0 and ns % nu1 == 0 and c == 3 * LANES and c4 % (3 * LANES) == 0
    assert ring & (ring - 1) == 0 and ring >= 2 * nu0
    assert xr >= 2 * nu0 + 1 and xr >= xd + 2 * nu1 and xd >= nu1
    kern = functools.partial(
        _kernel, st=st, nu0=nu0, nu1=nu1, ns=ns, c=c, c4=c4, ring=ring, npin=npin, xr=xr, xd=xd,
        rbs0=rbs0, rbs1=rbs1, perm0=perm0, corder0=tuple(corder0), perm1=perm1,
        corder1=tuple(corder1), phases=tuple(phases), nodma=nodma, nocomp=nocomp, aoff=aoff)
    nj = c4 // LANES
    hbm = pl.BlockSpec(memory_space=pl.ANY)
    vmem = pl.BlockSpec(memory_space=pltpu.VMEM)
    return pl.pallas_call(
        kern,
        in_specs=[hbm, vmem, hbm, hbm, vmem, vmem],
        out_specs=[hbm, hbm],
        out_shape=[
            jax.ShapeDtypeStruct((n, c), BF16),
            jax.ShapeDtypeStruct((ns - npin - ring, nj, st // 2, LANES), U32),
        ],
        scratch_shapes=[
            pltpu.VMEM((ring + npin, nj, st // 2, LANES), U32),
            pltpu.VMEM((xr, st, c), BF16),
            pltpu.VMEM((_NPROD, rbs0 // 4, LANES), U32),
            pltpu.VMEM((nj, 8, LANES), F32),
            pltpu.VMEM((_NPROD, c4 // 6, LANES), U32),
            pltpu.VMEM((8, c), F32),
            pltpu.VMEM((c, c4), BF16),
            pltpu.VMEM((c4, c), BF16),
            pltpu.SemaphoreType.DMA((ring,)),
            pltpu.SemaphoreType.DMA((xr,)),
            pltpu.SemaphoreType.DMA((xr,)),
            pltpu.SemaphoreType.DMA((2,)),
        ],
        compiler_params=pltpu.CompilerParams(
            vmem_limit_bytes=vmem_mb * 1024 * 1024,
            disable_bounds_checks=True,
        ),
    )


def _run(x, dw, w1, w2, grn_g, grn_b, **kw):
    b, hh, ww, c = x.shape
    c4 = w1.shape[1]
    n = b * hh * ww
    assert b == 1 and dw.shape[0] == 1 and dw.shape[1] == 1
    out, _ = _build(n, c, c4, **kw)(
        x.reshape(n, c), dw.reshape(1, c), w1, w2, grn_g, grn_b)
    return out.reshape(x.shape)


@jax.jit
def pallas_standalone__modern_conv_block_slak__vision_kernel(
    x: jax.Array,
    dw: jax.Array,
    w1: jax.Array,
    w2: jax.Array,
    grn_g: jax.Array,
    grn_b: jax.Array,
):
    return _run(x, dw, w1, w2, grn_g, grn_b)
```

```python
import functools
import math

import jax
import jax.numpy as jnp
import jax.experimental.pallas as pl
import jax.experimental.pallas.tpu as pltpu

F32 = jnp.float32
BF16 = jnp.bfloat16
U32 = jnp.uint32
LANES = 128

_GELU_C0 = math.sqrt(2.0 / math.pi)
_GELU_C1 = _GELU_C0 * 0.044715
_LAM = _GELU_C1 ** (1.0 / 3.0)
_KAP = _GELU_C0 / _LAM
_HSCALE = 1.0 / (2.0 * _LAM)
_LN_EPS = 1e-5
_GRN_EPS = 1e-6

_HK_U = ((0, 0, 0, 1, -1, 0), (-1, 0, 0, 0, 0, 1), (1, 0, 0, -1, 0, 0), (-1, 0, 0, 0, 0, 0),
         (0, 0, -1, 0, 0, 1), (1, 0, 0, -1, 1, 0), (0, -1, 0, 0, 0, 0), (0, -1, 1, 0, 0, -1),
         (0, 1, -1, 0, 0, 0), (1, 0, -1, 0, 0, 0), (0, 0, 0, 0, -1, 0), (0, 0, 0, -1, 0, 1),
         (0, 1, -1, 0, -1, 1), (-1, 1, 0, 1, -1, 0), (0, 0, 0, 0, 0, 1))
_HK_V = ((0, 0, 1, 0, 0, 0, 0, 0, 0), (0, -1, 0, 0, 0, 0, 1, 0, 0), (1, 1, 0, 1, 0, 0, 0, 0, 0),
         (1, 0, -1, 0, 0, 0, 1, 0, 0), (0, 0, 0, 0, 1, 0, 1, 1, 0), (0, 0, 1, 1, 0, 0, 0, 0, 0),
         (0, 0, 0, -1, 0, 1, 0, 0, 1), (0, 0, 0, 0, -1, 0, 0, 0, -1), (0, 0, 0, 0, 0, 0, 0, 0, 1),
         (0, 0, 0, 0, 0, 0, 1, 0, 0), (0, 0, 1, 0, -1, 1, 0, 0, 0), (0, -1, 0, 0, 0, 0, 0, 0, 0),
         (0, 0, 0, 0, -1, 0, 0, 0, 0), (0, 0, 0, 1, 0, 0, 0, 0, 0), (0, -1, 0, 0, 0, 0, 0, -1, 1))
_HK_W = ((1, 0, 1, 1, 0, 1), (0, 1, 0, 1, 0, 0), (0, 0, 0, -1, 0, 0), (-1, 0, 0, -1, 0, 0),
         (0, -1, 0, 0, 0, 0), (1, 0, 1, 1, 0, 0), (0, 0, -1, 0, 0, 0), (0, 1, 0, 0, 1, 1),
         (0, -1, -1, 0, -1, -1), (-1, 1, 0, 0, 0, 0), (0, 0, 0, 0, 0, -1), (0, 0, 0, -1, 1, 0),
         (0, 0, 0, 0, 1, 1), (1, 0, 1, 0, 0, 0), (0, -1, 0, 0, -1, 0))
_HK = (_HK_U, _HK_V, tuple(tuple(w[o] for w in _HK_W) for o in range(6)))
_NPROD = len(_HK_U)


class _lazy:
    def __init__(self, fn):
        self.fn, self.val = fn, None


def _force(v):
    if isinstance(v, _lazy):
        if v.val is None:
            v.val = v.fn()
        return v.val
    return v


def _combos(rows, vals, perm=None):
    vals = list(vals)
    rank = list(perm) if perm is not None else list(range(len(vals)))
    rows = [{i: c for i, c in enumerate(r) if c} for r in rows]
    while True:
        cnt = {}
        for r in rows:
            ks = sorted(r, key=lambda i: rank[i])
            for ia, a in enumerate(ks):
                for b in ks[ia + 1:]:
                    key = (a, b, r[a] * r[b])
                    cnt[key] = cnt.get(key, 0) + 1
        if not cnt or max(cnt.values()) < 2:
            break
        a, b, sg = max(sorted(cnt, key=lambda k_: (rank[k_[0]], rank[k_[1]], k_[2])),
                       key=lambda k_: cnt[k_])
        vals.append(_lazy(lambda a=a, b=b, sg=sg: (
            _force(vals[a]) + _force(vals[b]) if sg > 0 else _force(vals[a]) - _force(vals[b]))))
        rank.append(max(rank[a], rank[b]) + 0.5)
        new = len(vals) - 1
        for r in rows:
            if a in r and b in r and r[a] * r[b] == sg:
                r[new] = r.pop(a)
                del r[b]

    def total(items, sign):
        acc = _force(vals[items[0][0]])
        for idx, cf in items[1:]:
            acc = acc + _force(vals[idx]) if cf * sign > 0 else acc - _force(vals[idx])
        return acc

    out = []
    for r in rows:
        items = sorted(r.items(), key=lambda kv: rank[kv[0]])
        pos = [i for i, kv in enumerate(items) if kv[1] > 0]
        if pos and pos[0] > 0:
            items.insert(0, items.pop(pos[0]))
        sign = items[0][1]
        out.append((_lazy(functools.partial(total, items, sign)), sign))
    return out


def _weight_sums(sch, blocks):
    usign = [sg for _, sg in _combos(sch[0], [1.0] * 6)]
    res = []
    for q, (t, sg) in enumerate(_combos(sch[1], blocks)):
        t = _force(t)
        res.append(_pack((t if sg * usign[q] > 0 else -t).astype(BF16)))
    return res


def _col(row, n):
    return jnp.transpose(jnp.broadcast_to(row, (LANES, n)))


def _pack(v):
    return pltpu.bitcast(v, U32)


def _unpack(v):
    return pltpu.bitcast(v, BF16)


def _kernel(x_hbm, dw_ref, w1_hbm, w2_hbm, g_ref, b_ref,
            o_hbm, h_hbm,
            hs, xb, sb0, ssq_ref, ws_ref, bias_ref, w1_ref, w2_ref,
            sem_h, sem_x, sem_o, sem_w,
            *, st, nu0, nu1, ns, c, c4, ring, npin, xr, xd, rbs0, rbs1,
            perm0, corder0, perm1, corder1, phases, nodma, nocomp, aoff, prepos, sch0, sch1):
    nj = c4 // LANES
    njk = nj // 3
    nspill = ns - npin - ring
    dot = functools.partial(jnp.dot, preferred_element_type=F32)

    def wrap_ring(u):
        return u & (ring - 1)

    def unit_info(t, acc, lo):
        unpinned = acc + npin < ns
        u = t - lo
        return unpinned, u, jnp.where(unpinned, wrap_ring(u), ring + lo)

    def step_up(acc, lo):
        acc = acc + npin
        wrap = acc >= ns
        return jnp.where(wrap, acc - ns, acc), jnp.where(wrap, lo + 1, lo)

    def step_down(acc, lo):
        acc = acc - npin
        wrap = acc < 0
        return jnp.where(wrap, acc + ns, acc), jnp.where(wrap, lo - 1, lo)

    def x_slots(first, n, step):
        res = [first]
        for _ in range(n - 1):
            nxt = res[-1] + step
            res.append(jnp.where(nxt >= xr, nxt - xr, jnp.where(nxt < 0, nxt + xr, nxt)))
        return res

    def h_out_copy(u):
        return pltpu.make_async_copy(hs.at[wrap_ring(u)], h_hbm.at[u], sem_h.at[wrap_ring(u)])

    def h_in_copy(u):
        return pltpu.make_async_copy(h_hbm.at[u], hs.at[wrap_ring(u)], sem_h.at[wrap_ring(u)])

    def x_copy(t, slot):
        return pltpu.make_async_copy(x_hbm.at[pl.ds(t * st, st), :], xb.at[slot], sem_x.at[slot])

    def o_copy(t, slot):
        return pltpu.make_async_copy(xb.at[slot], o_hbm.at[pl.ds(t * st, st), :], sem_o.at[slot])

    w1_copy = pltpu.make_async_copy(w1_hbm, w1_ref, sem_w.at[0])
    w2_copy = pltpu.make_async_copy(w2_hbm, w2_ref, sem_w.at[1])

    hh = rbs0 // 2

    def phase0_lhs(xslot, rb):
        dw = dw_ref[...].astype(F32)

        def layernorm(xf):
            y = xf * dw
            yc = y - jnp.sum(y, axis=-1, keepdims=True) * (1.0 / c)
            ss = jnp.sum(yc * yc, axis=-1, keepdims=True)
            return yc * jnp.exp2(jnp.log(ss + c * _LN_EPS) * (-0.5 / math.log(2.0)))

        xu = _pack(xb[xslot, rb * rbs0:(rb + 1) * rbs0, :])
        halves = [layernorm(pltpu.unpack_elementwise(
            xu, index=k, packed_dtype=BF16, unpacked_dtype=F32)) for k in range(2)]
        blocks = [a[:, k * LANES:(k + 1) * LANES] for a in halves for k in range(3)]
        return [_force(v).astype(BF16) for v, _ in _combos(sch0[0], blocks)]

    def lhs_to_scratch(xslot):
        for q, t in enumerate(phase0_lhs(xslot, 0)):
            sb0[q] = t

    w1_copy.start()
    if 0 in phases:
        for k in range(nu0 + 1):
            x_copy(k, k).start()
    w2_copy.start()
    ssq_ref[...] = jnp.zeros_like(ssq_ref)
    w1_copy.wait()
    for j in range(njk):
        blocks = [w1_ref[kb * LANES:(kb + 1) * LANES,
                         (l * njk + j) * LANES:(l * njk + j + 1) * LANES].astype(F32)
                  * (_LAM * math.sqrt(c))
                  for kb in range(3) for l in range(3)]
        for q, t in enumerate(_weight_sums(sch0, blocks)):
            ws_ref[q, j * (LANES // 2):(j + 1) * (LANES // 2), :] = t
    if 0 in phases:
        x_copy(0, 0).wait()
        lhs_to_scratch(0)

    def phase0_state(t0, acc, lo):
        infos = []
        for su in range(nu0):
            infos.append(unit_info(t0 + su, acc, lo))
            acc, lo = step_up(acc, lo)
        return tuple(infos), acc, lo

    def phase0_block(blk, carry):
        infos, bacc, blo, xs0 = carry
        t0 = blk * nu0
        xslots = x_slots(xs0, 2 * nu0 + 1, 1)
        for su in range(nu0):
            tn = t0 + nu0 + 1 + su

            @pl.when(tn < ns)
            def _():
                x_copy(tn, xslots[nu0 + 1 + su]).start()

        for su in range(nu0):
            tw = t0 + 1 + su

            @pl.when(tw < ns)
            def _():
                x_copy(tw, xslots[1 + su]).wait()

        for unpinned, u, _ in infos:
            @pl.when(jnp.logical_and(unpinned, u >= ring))
            def _():
                h_out_copy(u - ring).wait()

        for su in range(nu0):
            slot = infos[su][2]
            for rb in range(st // rbs0):
                if su == 0 and rb == 0:
                    ops = [sb0[q] for q in range(_NPROD)]
                else:
                    ops = phase0_lhs(xslots[su], rb)
                if su * (st // rbs0) + rb == prepos:
                    lhs_to_scratch(xslots[nu0])
                for jc in range(njk):
                    wrows = slice(jc * (LANES // 2), (jc + 1) * (LANES // 2))
                    ms = [_lazy(lambda q=q: dot(ops[q], _unpack(ws_ref[q, wrows, :])))
                          for q in range(_NPROD)]
                    cs = _combos(sch0[2], ms, perm0)
                    done = {}
                    for o in corder0:
                        b = _force(cs[o][0])
                        if cs[o][1] < 0:
                            b = -b
                        done[o] = b * (1.0 + jnp.tanh(b * (b * b + _KAP)))
                        l = o % 3
                        if l in done and l + 3 in done:
                            gt, gb = done[l], done[l + 3]
                            j = l * njk + jc
                            ssq_ref[j] += jnp.sum(
                                (gt * gt + gb * gb).reshape(hh // 8, 8, LANES), axis=0)
                            hs[slot, j, rb * hh:(rb + 1) * hh, :] = pltpu.pack_elementwise(
                                [gt, gb], packed_dtype=BF16)
        if prepos >= nu0 * (st // rbs0):
            lhs_to_scratch(xslots[nu0])

        for unpinned, u, _ in infos:
            @pl.when(jnp.logical_and(unpinned, u < nspill))
            def _():
                h_out_copy(u).start()
        infos, bacc, blo = phase0_state(t0 + nu0, bacc, blo)
        return infos, bacc, blo, xslots[nu0]

    if 0 in phases:
        zero = jnp.int32(0)
        jax.lax.fori_loop(0, ns // nu0, phase0_block,
                          (*phase0_state(zero, jnp.int32(aoff), zero), zero))

    if phases == (1,):
        for t in range(ns - xr, ns):
            x_copy(t, t % xr).start()
            x_copy(t, t % xr).wait()
    w2_copy.wait()
    ssq = jnp.concatenate(
        [jnp.sum(ssq_ref[j], axis=0, keepdims=True) for j in range(nj)], axis=1)
    gx = jnp.sqrt(ssq * (_HSCALE * _HSCALE) + _GRN_EPS)
    nx = gx / (jnp.mean(gx, axis=-1, keepdims=True) + _GRN_EPS)
    s = (1.0 + g_ref[...].astype(F32).reshape(1, c4) * nx) * _HSCALE
    s_t = _col(s, c4)
    kb = c4 // 3
    w2s = [w2_ref[:, l * LANES:(l + 1) * LANES].astype(F32) * s_t for l in range(3)]
    for q, t in enumerate(_weight_sums(
            sch1, [w2s[l][j * kb:(j + 1) * kb] for j in range(3) for l in range(3)])):
        ws_ref[q] = t
    grn_b = b_ref[...].astype(F32).reshape(1, c4)
    bias_ref[...] = dot(jnp.broadcast_to(grn_b, (16, c4)).astype(BF16), w2_ref[...])[:8]

    def phase1_state(i0, acc, lo):
        infos = []
        for su in range(nu1):
            infos.append(unit_info(ns - 1 - (i0 + su), acc, lo))
            acc, lo = step_down(acc, lo)
        return tuple(infos), acc, lo

    def phase1_block(blk, carry):
        prev, infos, bacc, blo, xs0 = carry
        hh1 = rbs1 // 2
        bias = bias_ref[0:1, :]
        i0 = blk * nu1
        xslots = x_slots(xs0, xd + nu1, -1)
        for su in range(nu1):
            inx = i0 + su + xd

            @pl.when(jnp.logical_and(inx < ns, inx >= xr))
            def _():
                o_copy(ns - 1 - (inx - xr), xslots[su + xd]).wait()
                x_copy(ns - 1 - inx, xslots[su + xd]).start()

        if not nodma:
            for unp_p, u_p, _ in prev:
                @pl.when(jnp.logical_and(unp_p, u_p >= ring))
                def _():
                    h_in_copy(u_p - ring).start()

        for su in range(nu1):
            @pl.when(i0 + su >= xr)
            def _():
                x_copy(ns - 1 - (i0 + su), xslots[su]).wait()

            if not nodma:
                unpinned, u, _ = infos[su]

                @pl.when(jnp.logical_and(unpinned, u < nspill))
                def _():
                    h_in_copy(u).wait()

        for su in range(nu1):
            slot = infos[su][2]
            xslot = xslots[su]
            for rb in range(0 if nocomp else st // rbs1):
                r0 = rb * rbs1
                raw = [jnp.concatenate(
                    [_unpack(hs[slot, kk * njk + j,
                                (r0 + half * hh1) // 2:(r0 + (half + 1) * hh1) // 2, :])
                     for j in range(njk)], axis=1) for half in range(2) for kk in range(3)]
                lhs = _combos(sch1[0], [_lazy(lambda a=a: a.astype(F32)) for a in raw])

                def product(q):
                    nzs = [ix for ix, cf in enumerate(sch1[0][q]) if cf]
                    a = raw[nzs[0]] if len(nzs) == 1 else _force(lhs[q][0]).astype(BF16)
                    return dot(a, _unpack(ws_ref[q]))

                ms = [_lazy(functools.partial(product, q)) for q in range(_NPROD)]
                cs = _combos(sch1[2], ms, perm1)
                for o in corder1:
                    half, l = divmod(o, 3)
                    rs = slice(r0 + half * hh1, r0 + (half + 1) * hh1)
                    cl = slice(l * LANES, (l + 1) * LANES)
                    val, sg = _force(cs[o][0]), cs[o][1]
                    base = xb[xslot, rs, cl].astype(F32) + bias[:, cl]
                    xb[xslot, rs, cl] = (base + val if sg > 0 else base - val).astype(BF16)

        for su in range(nu1):
            o_copy(ns - 1 - (i0 + su), xslots[su]).start()
        nxt, bacc, blo = phase1_state(i0 + nu1, bacc, blo)
        return infos, nxt, bacc, blo, xslots[nu1]

    if 1 in phases:
        acc0, lo0 = (jnp.int32(v) for v in divmod((ns - 1) * npin + aoff, ns)[::-1])
        first, acc0, lo0 = phase1_state(jnp.int32(0), acc0, lo0)
        none = tuple((jnp.bool_(False), jnp.int32(0), jnp.int32(0)) for _ in range(nu1))
        jax.lax.fori_loop(0, ns // nu1, phase1_block,
                          (none, first, acc0, lo0, jnp.int32((ns - 1) % xr)))
        for t in range(xr):
            o_copy(t, t % xr).wait()
    else:
        o_copy(0, 0).start()
        o_copy(0, 0).wait()


def _mk(s):
    if s is None:
        return _HK
    return (tuple(tuple(t[0]) for t in s), tuple(tuple(t[1]) for t in s),
            tuple(tuple(t[2][o] for t in s) for o in range(6)))


def _build(n, c, c4, st=1024, nu0=2, nu1=1, ring=4, npin=35, xr=5, xd=3, vmem_mb=128,
           rbs0=128, rbs1=256,
           perm0=(6, 7, 9, 11, 3, 12, 4, 10, 13, 2, 0, 1, 5, 14, 8), corder0=(3, 0, 2, 1, 4, 5),
           perm1=(5, 14, 1, 7, 8, 11, 10, 12, 6, 0, 3, 2, 13, 4, 9), corder1=(1, 4, 3, 0, 5, 2),
           phases=(0, 1), nodma=False, nocomp=False, aoff=72, prepos=99, sch0=None, sch1=None):
    ns = n // st
    assert n % st == 0 and ns % nu0 == 0 and ns % nu1 == 0 and c == 3 * LANES and c4 % (3 * LANES) == 0
    assert ring & (ring - 1) == 0 and ring >= 2 * nu0
    assert xr >= 2 * nu0 + 1 and xr >= xd + 2 * nu1 and xd >= nu1
    kern = functools.partial(
        _kernel, st=st, nu0=nu0, nu1=nu1, ns=ns, c=c, c4=c4, ring=ring, npin=npin, xr=xr, xd=xd,
        rbs0=rbs0, rbs1=rbs1, perm0=perm0, corder0=tuple(corder0), perm1=perm1,
        corder1=tuple(corder1), phases=tuple(phases), nodma=nodma, nocomp=nocomp, aoff=aoff, prepos=prepos,
        sch0=_mk(sch0), sch1=_mk(sch1))
    nj = c4 // LANES
    hbm = pl.BlockSpec(memory_space=pl.ANY)
    vmem = pl.BlockSpec(memory_space=pltpu.VMEM)
    return pl.pallas_call(
        kern,
        in_specs=[hbm, vmem, hbm, hbm, vmem, vmem],
        out_specs=[hbm, hbm],
        out_shape=[
            jax.ShapeDtypeStruct((n, c), BF16),
            jax.ShapeDtypeStruct((ns - npin - ring, nj, st // 2, LANES), U32),
        ],
        scratch_shapes=[
            pltpu.VMEM((ring + npin, nj, st // 2, LANES), U32),
            pltpu.VMEM((xr, st, c), BF16),
            pltpu.VMEM((_NPROD, rbs0 // 2, LANES), BF16),
            pltpu.VMEM((nj, 8, LANES), F32),
            pltpu.VMEM((_NPROD, c4 // 6, LANES), U32),
            pltpu.VMEM((8, c), F32),
            pltpu.VMEM((c, c4), BF16),
            pltpu.VMEM((c4, c), BF16),
            pltpu.SemaphoreType.DMA((ring,)),
            pltpu.SemaphoreType.DMA((xr,)),
            pltpu.SemaphoreType.DMA((xr,)),
            pltpu.SemaphoreType.DMA((2,)),
        ],
        compiler_params=pltpu.CompilerParams(
            vmem_limit_bytes=vmem_mb * 1024 * 1024,
            disable_bounds_checks=True,
        ),
    )


def _run(x, dw, w1, w2, grn_g, grn_b, **kw):
    b, hh, ww, c = x.shape
    c4 = w1.shape[1]
    n = b * hh * ww
    assert b == 1 and dw.shape[0] == 1 and dw.shape[1] == 1
    out, _ = _build(n, c, c4, **kw)(
        x.reshape(n, c), dw.reshape(1, c), w1, w2, grn_g, grn_b)
    return out.reshape(x.shape)


@jax.jit
def pallas_standalone__modern_conv_block_slak__vision_kernel(
    x: jax.Array,
    dw: jax.Array,
    w1: jax.Array,
    w2: jax.Array,
    grn_g: jax.Array,
    grn_b: jax.Array,
):
    return _run(x, dw, w1, w2, grn_g, grn_b)
```

```python
import functools
import math

import jax
import jax.numpy as jnp
import jax.experimental.pallas as pl
import jax.experimental.pallas.tpu as pltpu

F32 = jnp.float32
BF16 = jnp.bfloat16
U32 = jnp.uint32
LANES = 128

_GELU_C0 = math.sqrt(2.0 / math.pi)
_GELU_C1 = _GELU_C0 * 0.044715
_LAM = _GELU_C1 ** (1.0 / 3.0)
_KAP = _GELU_C0 / _LAM
_HSCALE = 1.0 / (2.0 * _LAM)
_LN_EPS = 1e-5
_GRN_EPS = 1e-6

_HK_U = ((0, 0, 0, 1, -1, 0), (-1, 0, 0, 0, 0, 1), (1, 0, 0, -1, 0, 0), (-1, 0, 0, 0, 0, 0),
         (0, 0, -1, 0, 0, 1), (1, 0, 0, -1, 1, 0), (0, -1, 0, 0, 0, 0), (0, -1, 1, 0, 0, -1),
         (0, 1, -1, 0, 0, 0), (1, 0, -1, 0, 0, 0), (0, 0, 0, 0, -1, 0), (0, 0, 0, -1, 0, 1),
         (0, 1, -1, 0, -1, 1), (-1, 1, 0, 1, -1, 0), (0, 0, 0, 0, 0, 1))
_HK_V = ((0, 0, 1, 0, 0, 0, 0, 0, 0), (0, -1, 0, 0, 0, 0, 1, 0, 0), (1, 1, 0, 1, 0, 0, 0, 0, 0),
         (1, 0, -1, 0, 0, 0, 1, 0, 0), (0, 0, 0, 0, 1, 0, 1, 1, 0), (0, 0, 1, 1, 0, 0, 0, 0, 0),
         (0, 0, 0, -1, 0, 1, 0, 0, 1), (0, 0, 0, 0, -1, 0, 0, 0, -1), (0, 0, 0, 0, 0, 0, 0, 0, 1),
         (0, 0, 0, 0, 0, 0, 1, 0, 0), (0, 0, 1, 0, -1, 1, 0, 0, 0), (0, -1, 0, 0, 0, 0, 0, 0, 0),
         (0, 0, 0, 0, -1, 0, 0, 0, 0), (0, 0, 0, 1, 0, 0, 0, 0, 0), (0, -1, 0, 0, 0, 0, 0, -1, 1))
_HK_W = ((1, 0, 1, 1, 0, 1), (0, 1, 0, 1, 0, 0), (0, 0, 0, -1, 0, 0), (-1, 0, 0, -1, 0, 0),
         (0, -1, 0, 0, 0, 0), (1, 0, 1, 1, 0, 0), (0, 0, -1, 0, 0, 0), (0, 1, 0, 0, 1, 1),
         (0, -1, -1, 0, -1, -1), (-1, 1, 0, 0, 0, 0), (0, 0, 0, 0, 0, -1), (0, 0, 0, -1, 1, 0),
         (0, 0, 0, 0, 1, 1), (1, 0, 1, 0, 0, 0), (0, -1, 0, 0, -1, 0))
_HK = (_HK_U, _HK_V, tuple(tuple(w[o] for w in _HK_W) for o in range(6)))
_NPROD = len(_HK_U)


class _lazy:
    def __init__(self, fn):
        self.fn, self.val = fn, None


def _force(v):
    if isinstance(v, _lazy):
        if v.val is None:
            v.val = v.fn()
        return v.val
    return v


def _combos(rows, vals, perm=None):
    vals = list(vals)
    rank = list(perm) if perm is not None else list(range(len(vals)))
    rows = [{i: c for i, c in enumerate(r) if c} for r in rows]
    while True:
        cnt = {}
        for r in rows:
            ks = sorted(r, key=lambda i: rank[i])
            for ia, a in enumerate(ks):
                for b in ks[ia + 1:]:
                    key = (a, b, r[a] * r[b])
                    cnt[key] = cnt.get(key, 0) + 1
        if not cnt or max(cnt.values()) < 2:
            break
        a, b, sg = max(sorted(cnt, key=lambda k_: (rank[k_[0]], rank[k_[1]], k_[2])),
                       key=lambda k_: cnt[k_])
        vals.append(_lazy(lambda a=a, b=b, sg=sg: (
            _force(vals[a]) + _force(vals[b]) if sg > 0 else _force(vals[a]) - _force(vals[b]))))
        rank.append(max(rank[a], rank[b]) + 0.5)
        new = len(vals) - 1
        for r in rows:
            if a in r and b in r and r[a] * r[b] == sg:
                r[new] = r.pop(a)
                del r[b]

    def total(items, sign):
        acc = _force(vals[items[0][0]])
        for idx, cf in items[1:]:
            acc = acc + _force(vals[idx]) if cf * sign > 0 else acc - _force(vals[idx])
        return acc

    out = []
    for r in rows:
        items = sorted(r.items(), key=lambda kv: rank[kv[0]])
        pos = [i for i, kv in enumerate(items) if kv[1] > 0]
        if pos and pos[0] > 0:
            items.insert(0, items.pop(pos[0]))
        sign = items[0][1]
        out.append((_lazy(functools.partial(total, items, sign)), sign))
    return out


def _weight_sums(sch, blocks):
    usign = [sg for _, sg in _combos(sch[0], [1.0] * 6)]
    res = []
    for q, (t, sg) in enumerate(_combos(sch[1], blocks)):
        t = _force(t)
        res.append(_pack((t if sg * usign[q] > 0 else -t).astype(BF16)))
    return res


def _col(row, n):
    return jnp.transpose(jnp.broadcast_to(row, (LANES, n)))


def _pack(v):
    return pltpu.bitcast(v, U32)


def _unpack(v):
    return pltpu.bitcast(v, BF16)


def _kernel(x_hbm, dw_ref, w1_hbm, w2_hbm, g_ref, b_ref,
            o_hbm, h_hbm,
            hs, xb, sb0, ssq_ref, ws_ref, bias_ref,
            sem_h, sem_x, sem_o, sem_w,
            *, st, nu0, nu1, ns, c, c4, ring, npin, xr, xd, rbs0, rbs1,
            perm0, corder0, perm1, corder1, phases, nodma, nocomp, aoff, sch0, sch1):
    nj = c4 // LANES
    njk = nj // 3
    nspill = ns - npin - ring
    dot = functools.partial(jnp.dot, preferred_element_type=F32)

    def wrap_ring(u):
        return u & (ring - 1)

    def unit_info(t, acc, lo):
        unpinned = acc + npin < ns
        u = t - lo
        return unpinned, u, jnp.where(unpinned, wrap_ring(u), ring + lo)

    def step_up(acc, lo):
        acc = acc + npin
        wrap = acc >= ns
        return jnp.where(wrap, acc - ns, acc), jnp.where(wrap, lo + 1, lo)

    def step_down(acc, lo):
        acc = acc - npin
        wrap = acc < 0
        return jnp.where(wrap, acc + ns, acc), jnp.where(wrap, lo - 1, lo)

    def x_slots(first, n, step):
        res = [first]
        for _ in range(n - 1):
            nxt = res[-1] + step
            res.append(jnp.where(nxt >= xr, nxt - xr, jnp.where(nxt < 0, nxt + xr, nxt)))
        return res

    def h_out_copy(u):
        return pltpu.make_async_copy(hs.at[wrap_ring(u)], h_hbm.at[u], sem_h.at[wrap_ring(u)])

    def h_in_copy(u):
        return pltpu.make_async_copy(h_hbm.at[u], hs.at[wrap_ring(u)], sem_h.at[wrap_ring(u)])

    def x_copy(t, slot):
        return pltpu.make_async_copy(x_hbm.at[pl.ds(t * st, st), :], xb.at[slot], sem_x.at[slot])

    def o_copy(t, slot):
        return pltpu.make_async_copy(xb.at[slot], o_hbm.at[pl.ds(t * st, st), :], sem_o.at[slot])

    w1_slot = nu0 + 1
    w1_copies = [pltpu.make_async_copy(
        w1_hbm.at[:, pl.ds(k * c, c)],
        xb.at[w1_slot + k // 2, pl.ds((k % 2) * c, c), :], sem_w.at[k]) for k in range(4)]
    w2_slots = ((ns - xr) % xr, (ns - xr + 1) % xr)
    w2_copies = [
        pltpu.make_async_copy(w2_hbm.at[pl.ds(0, st), :], xb.at[w2_slots[0]], sem_w.at[4]),
        pltpu.make_async_copy(w2_hbm.at[pl.ds(st, c4 - st), :],
                              xb.at[w2_slots[1], pl.ds(0, c4 - st), :], sem_w.at[5])]
    nres = xr - 2

    def w1_block(kb, cb):
        k, off = divmod(cb, 3)
        r0 = (k % 2) * c + kb * LANES
        return xb[w1_slot + k // 2, r0:r0 + LANES, off * LANES:(off + 1) * LANES]

    def w2_rows(r0, n_rows, cols):
        slot, r0 = (w2_slots[0], r0) if r0 < st else (w2_slots[1], r0 - st)
        return xb[slot, r0:r0 + n_rows, cols]

    hh = rbs0 // 2

    def phase0_lhs(xslot, rb):
        dw = dw_ref[...].astype(F32)

        def layernorm(xf):
            y = xf * dw
            yc = y - jnp.sum(y, axis=-1, keepdims=True) * (1.0 / c)
            ss = jnp.sum(yc * yc, axis=-1, keepdims=True)
            return yc * jnp.exp2(jnp.log(ss + c * _LN_EPS) * (-0.5 / math.log(2.0)))

        xu = _pack(xb[xslot, rb * rbs0:(rb + 1) * rbs0, :])
        halves = [layernorm(pltpu.unpack_elementwise(
            xu, index=k, packed_dtype=BF16, unpacked_dtype=F32)) for k in range(2)]
        blocks = [a[:, k * LANES:(k + 1) * LANES] for a in halves for k in range(3)]
        return [_force(v).astype(BF16) for v, _ in _combos(sch0[0], blocks)]

    def lhs_to_scratch(xslot):
        for q, t in enumerate(phase0_lhs(xslot, 0)):
            sb0[q] = t

    for cp in w1_copies:
        cp.start()
    if 0 in phases:
        for k in range(nu0 + 1):
            x_copy(k, k).start()
    else:
        for cp in w2_copies:
            cp.start()
    ssq_ref[...] = jnp.zeros_like(ssq_ref)
    for cp in w1_copies:
        cp.wait()
    for j in range(njk):
        blocks = [w1_block(kb, l * njk + j).astype(F32) * (_LAM * math.sqrt(c))
                  for kb in range(3) for l in range(3)]
        for q, t in enumerate(_weight_sums(sch0, blocks)):
            ws_ref[q, j * (LANES // 2):(j + 1) * (LANES // 2), :] = t
    if 0 in phases:
        x_copy(0, 0).wait()
        lhs_to_scratch(0)

    def phase0_state(t0, acc, lo):
        infos = []
        for su in range(nu0):
            infos.append(unit_info(t0 + su, acc, lo))
            acc, lo = step_up(acc, lo)
        return tuple(infos), acc, lo

    def phase0_block(blk, carry):
        infos, bacc, blo, xs0 = carry
        t0 = blk * nu0
        xslots = x_slots(xs0, 2 * nu0 + 1, 1)
        for su in range(nu0):
            tn = t0 + nu0 + 1 + su

            @pl.when(tn < ns)
            def _():
                x_copy(tn, xslots[nu0 + 1 + su]).start()

        @pl.when(t0 + nu0 == ns)
        def _():
            for cp in w2_copies:
                cp.start()

        for su in range(nu0):
            tw = t0 + 1 + su

            @pl.when(tw < ns)
            def _():
                x_copy(tw, xslots[1 + su]).wait()

        for unpinned, u, _ in infos:
            @pl.when(jnp.logical_and(unpinned, u >= ring))
            def _():
                h_out_copy(u - ring).wait()

        for su in range(nu0):
            slot = infos[su][2]
            for rb in range(st // rbs0):
                if su == 0 and rb == 0:
                    ops = [sb0[q] for q in range(_NPROD)]
                else:
                    ops = phase0_lhs(xslots[su], rb)
                for jc in range(njk):
                    wrows = slice(jc * (LANES // 2), (jc + 1) * (LANES // 2))
                    ms = [_lazy(lambda q=q: dot(ops[q], _unpack(ws_ref[q, wrows, :])))
                          for q in range(_NPROD)]
                    cs = _combos(sch0[2], ms, perm0)
                    done = {}
                    for o in corder0:
                        b = _force(cs[o][0])
                        if cs[o][1] < 0:
                            b = -b
                        done[o] = b * (1.0 + jnp.tanh(b * (b * b + _KAP)))
                        l = o % 3
                        if l in done and l + 3 in done:
                            gt, gb = done[l], done[l + 3]
                            j = l * njk + jc
                            ssq_ref[j] += jnp.sum(
                                (gt * gt + gb * gb).reshape(hh // 8, 8, LANES), axis=0)
                            hs[slot, j, rb * hh:(rb + 1) * hh, :] = pltpu.pack_elementwise(
                                [gt, gb], packed_dtype=BF16)
        lhs_to_scratch(jnp.where(t0 + nu0 == ns, xs0, xslots[nu0]))

        for unpinned, u, _ in infos:
            @pl.when(jnp.logical_and(unpinned, u < nspill))
            def _():
                h_out_copy(u).start()
        infos, bacc, blo = phase0_state(t0 + nu0, bacc, blo)
        return infos, bacc, blo, xslots[nu0]

    if 0 in phases:
        zero = jnp.int32(0)
        jax.lax.fori_loop(0, ns // nu0, phase0_block,
                          (*phase0_state(zero, jnp.int32(aoff), zero), zero))

    if phases == (1,):
        for t in range(ns - nres, ns):
            x_copy(t, t % xr).start()
            x_copy(t, t % xr).wait()
    for cp in w2_copies:
        cp.wait()
    ssq = jnp.concatenate(
        [jnp.sum(ssq_ref[j], axis=0, keepdims=True) for j in range(nj)], axis=1)
    gx = jnp.sqrt(ssq * (_HSCALE * _HSCALE) + _GRN_EPS)
    nx = gx / (jnp.mean(gx, axis=-1, keepdims=True) + _GRN_EPS)
    s = (1.0 + g_ref[...].astype(F32).reshape(1, c4) * nx) * _HSCALE
    s_t = _col(s, c4)
    kb = c4 // 3
    for q, t in enumerate(_weight_sums(
            sch1, [w2_rows(j * kb, kb, slice(l * LANES, (l + 1) * LANES)).astype(F32)
                   * s_t[j * kb:(j + 1) * kb] for j in range(3) for l in range(3)])):
        ws_ref[q] = t
    grn_b = jnp.broadcast_to(b_ref[...].astype(F32).reshape(1, c4), (16, c4)).astype(BF16)
    w2 = jnp.concatenate([w2_rows(0, st, slice(None)), w2_rows(st, c4 - st, slice(None))], axis=0)
    bias_ref[...] = dot(grn_b, w2)[:8]
    if 1 in phases:
        for inx in range(nres, xd):
            x_copy(ns - 1 - inx, (ns - 1 - inx) % xr).start()

    def phase1_state(i0, acc, lo):
        infos = []
        for su in range(nu1):
            infos.append(unit_info(ns - 1 - (i0 + su), acc, lo))
            acc, lo = step_down(acc, lo)
        return tuple(infos), acc, lo

    def phase1_block(blk, carry):
        prev, infos, bacc, blo, xs0 = carry
        hh1 = rbs1 // 2
        bias = bias_ref[0:1, :]
        i0 = blk * nu1
        xslots = x_slots(xs0, xd + nu1, -1)
        for su in range(nu1):
            inx = i0 + su + xd

            @pl.when(jnp.logical_and(inx < ns, inx >= xr))
            def _():
                o_copy(ns - 1 - (inx - xr), xslots[su + xd]).wait()

            @pl.when(jnp.logical_and(inx < ns, inx >= nres))
            def _():
                x_copy(ns - 1 - inx, xslots[su + xd]).start()

        if not nodma:
            for unp_p, u_p, _ in prev:
                @pl.when(jnp.logical_and(unp_p, u_p >= ring))
                def _():
                    h_in_copy(u_p - ring).start()

        for su in range(nu1):
            @pl.when(i0 + su >= nres)
            def _():
                x_copy(ns - 1 - (i0 + su), xslots[su]).wait()

            if not nodma:
                unpinned, u, _ = infos[su]

                @pl.when(jnp.logical_and(unpinned, u < nspill))
                def _():
                    h_in_copy(u).wait()

        for su in range(nu1):
            slot = infos[su][2]
            xslot = xslots[su]
            for rb in range(0 if nocomp else st // rbs1):
                r0 = rb * rbs1
                raw = [jnp.concatenate(
                    [_unpack(hs[slot, kk * njk + j,
                                (r0 + half * hh1) // 2:(r0 + (half + 1) * hh1) // 2, :])
                     for j in range(njk)], axis=1) for half in range(2) for kk in range(3)]
                lhs = _combos(sch1[0], [_lazy(lambda a=a: a.astype(F32)) for a in raw])

                def product(q):
                    nzs = [ix for ix, cf in enumerate(sch1[0][q]) if cf]
                    a = raw[nzs[0]] if len(nzs) == 1 else _force(lhs[q][0]).astype(BF16)
                    return dot(a, _unpack(ws_ref[q]))

                ms = [_lazy(functools.partial(product, q)) for q in range(_NPROD)]
                cs = _combos(sch1[2], ms, perm1)
                for o in corder1:
                    half, l = divmod(o, 3)
                    rs = slice(r0 + half * hh1, r0 + (half + 1) * hh1)
                    cl = slice(l * LANES, (l + 1) * LANES)
                    val, sg = _force(cs[o][0]), cs[o][1]
                    base = xb[xslot, rs, cl].astype(F32) + bias[:, cl]
                    xb[xslot, rs, cl] = (base + val if sg > 0 else base - val).astype(BF16)

        for su in range(nu1):
            o_copy(ns - 1 - (i0 + su), xslots[su]).start()
        nxt, bacc, blo = phase1_state(i0 + nu1, bacc, blo)
        return infos, nxt, bacc, blo, xslots[nu1]

    if 1 in phases:
        acc0, lo0 = (jnp.int32(v) for v in divmod((ns - 1) * npin + aoff, ns)[::-1])
        first, acc0, lo0 = phase1_state(jnp.int32(0), acc0, lo0)
        none = tuple((jnp.bool_(False), jnp.int32(0), jnp.int32(0)) for _ in range(nu1))
        jax.lax.fori_loop(0, ns // nu1, phase1_block,
                          (none, first, acc0, lo0, jnp.int32((ns - 1) % xr)))
        for t in range(xr):
            o_copy(t, t % xr).wait()
    else:
        o_copy(0, 0).start()
        o_copy(0, 0).wait()


def _mk(s):
    if s is None:
        return _HK
    return (tuple(tuple(t[0]) for t in s), tuple(tuple(t[1]) for t in s),
            tuple(tuple(t[2][o] for t in s) for o in range(6)))


def _build(n, c, c4, st=1024, nu0=2, nu1=1, ring=4, npin=35, xr=6, xd=4, vmem_mb=128,
           rbs0=128, rbs1=128,
           perm0=(6, 7, 9, 11, 3, 12, 4, 10, 13, 2, 0, 1, 5, 14, 8), corder0=(3, 0, 2, 1, 4, 5),
           perm1=(5, 14, 1, 7, 8, 11, 10, 12, 6, 0, 3, 2, 13, 4, 9), corder1=(1, 4, 3, 0, 5, 2),
           phases=(0, 1), nodma=False, nocomp=False, aoff=72, sch0=None, sch1=None):
    ns = n // st
    assert n % st == 0 and ns % nu0 == 0 and ns % nu1 == 0 and c == 3 * LANES and c4 % (3 * LANES) == 0
    assert ring & (ring - 1) == 0 and ring >= 2 * nu0
    assert xr >= 2 * nu0 + 1 and xr >= nu0 + 3 and xr >= xd + 2 * nu1 and xd >= nu1
    assert c4 == 4 * c and 2 * c <= st < c4 <= 2 * st and st % (c4 // 3) == 0
    kern = functools.partial(
        _kernel, st=st, nu0=nu0, nu1=nu1, ns=ns, c=c, c4=c4, ring=ring, npin=npin, xr=xr, xd=xd,
        rbs0=rbs0, rbs1=rbs1, perm0=perm0, corder0=tuple(corder0), perm1=perm1,
        corder1=tuple(corder1), phases=tuple(phases), nodma=nodma, nocomp=nocomp, aoff=aoff,
        sch0=_mk(sch0), sch1=_mk(sch1))
    nj = c4 // LANES
    hbm = pl.BlockSpec(memory_space=pl.ANY)
    vmem = pl.BlockSpec(memory_space=pltpu.VMEM)
    return pl.pallas_call(
        kern,
        in_specs=[hbm, vmem, hbm, hbm, vmem, vmem],
        out_specs=[hbm, hbm],
        out_shape=[
            jax.ShapeDtypeStruct((n, c), BF16),
            jax.ShapeDtypeStruct((ns - npin - ring, nj, st // 2, LANES), U32),
        ],
        scratch_shapes=[
            pltpu.VMEM((ring + npin, nj, st // 2, LANES), U32),
            pltpu.VMEM((xr, st, c), BF16),
            pltpu.VMEM((_NPROD, rbs0 // 2, LANES), BF16),
            pltpu.VMEM((nj, 8, LANES), F32),
            pltpu.VMEM((_NPROD, c4 // 6, LANES), U32),
            pltpu.VMEM((8, c), F32),
            pltpu.SemaphoreType.DMA((ring,)),
            pltpu.SemaphoreType.DMA((xr,)),
            pltpu.SemaphoreType.DMA((xr,)),
            pltpu.SemaphoreType.DMA((6,)),
        ],
        compiler_params=pltpu.CompilerParams(
            vmem_limit_bytes=vmem_mb * 1024 * 1024,
            disable_bounds_checks=True,
        ),
    )


def _run(x, dw, w1, w2, grn_g, grn_b, **kw):
    b, hh, ww, c = x.shape
    c4 = w1.shape[1]
    n = b * hh * ww
    assert b == 1 and dw.shape[0] == 1 and dw.shape[1] == 1
    out, _ = _build(n, c, c4, **kw)(
        x.reshape(n, c), dw.reshape(1, c), w1, w2, grn_g, grn_b)
    return out.reshape(x.shape)


@jax.jit
def pallas_standalone__modern_conv_block_slak__vision_kernel(
    x: jax.Array,
    dw: jax.Array,
    w1: jax.Array,
    w2: jax.Array,
    grn_g: jax.Array,
    grn_b: jax.Array,
):
    return _run(x, dw, w1, w2, grn_g, grn_b)
```
